```python
import jax
import jax.numpy as jnp

def _softmax(x, axis=-1):
    return jax.nn.softmax(x, axis=axis)

def _gelu(x):
    return jax.nn.gelu(x, approximate=True)

def _silu(x):
    return jax.nn.silu(x)

def _sigmoid(x):
    return jax.nn.sigmoid(x)

def _layernorm(x, axis=-1, eps=1e-05):
    m = jnp.mean(x, axis=axis, keepdims=True)
    v = jnp.var(x, axis=axis, keepdims=True)
    return (x - m) / jnp.sqrt(v + eps)

def _scatter_add(tgt, idx, src, axis=0):
    return tgt.at[idx].add(src)

def _segment_sum(src, seg, n):
    return jax.ops.segment_sum(src, seg, n)

class _Rng:

    def __init__(self, key):
        self._k = key

    def _next(self):
        self._k, sub = jax.random.split(self._k)
        return sub

    def normal(self, shape):
        return jax.random.normal(self._next(), shape, dtype=jnp.bfloat16)

    def randint(self, lo, hi, shape):
        return jax.random.randint(self._next(), shape, lo, hi, dtype=jnp.int32)

    def uniform(self, shape, lo=0.0, hi=1.0):
        return jax.random.uniform(self._next(), shape, jnp.bfloat16, lo, hi)

    def permutation(self, n):
        return jax.random.permutation(self._next(), n)
kernel_name = 'adaLN_cond__spectral_gfnet__mixer_token_mlp__prompt'

def setup_inputs():
    _rng = _Rng(jax.random.key(int.from_bytes(__import__("os").urandom(4), "little")))
    _w = lambda a: (lambda t: t.astype(jnp.bfloat16) if jnp.issubdtype(t.dtype, jnp.floating) else t)(jnp.asarray(a))

    def _A_setup():
        B, S, D = (1, 2048, 576)
        Df = D // 2 + 1
        return {'x': _w((lambda *s: _rng.normal(s) * 0.05)(B, S, D)), 'w_r': _w((lambda *s: _rng.normal(s) * 0.05)(S, Df) * 0.02), 'w_i': _w((lambda *s: _rng.normal(s) * 0.05)(S, Df) * 0.02)}
    _A_in = _A_setup()

    def _B_setup():
        B, S, D, F = (1, 2048, 576, 4608)
        return {'x': _w((lambda *s: _rng.normal(s) * 0.05)(B, S, D)), 'w1': _w((lambda *s: _rng.normal(s) * 0.05)(S, F) * S ** (-0.5)), 'b1': _w((lambda *s: _rng.normal(s) * 0.05)(F) * 0.02), 'w2': _w((lambda *s: _rng.normal(s) * 0.05)(F, S) * F ** (-0.5)), 'b2': _w((lambda *s: _rng.normal(s) * 0.05)(S) * 0.02)}
    _B_in = _B_setup()
    return {'A_x': _A_in['x'], 'A_w_r': _A_in['w_r'], 'A_w_i': _A_in['w_i'], 'B_x': _B_in['x'], 'B_w1': _B_in['w1'], 'B_b1': _B_in['b1'], 'B_w2': _B_in['w2'], 'B_b2': _B_in['b2'], 'c': _w((lambda *s: _rng.normal(s) * 0.05)(1, 576)), 'w_mod': _w((lambda *s: _rng.normal(s) * 0.05)(576, 6 * 576) * 576 ** (-0.5))}

def reference(A_x, A_w_r, A_w_i, B_x, B_w1, B_b1, B_w2, B_b2, c, w_mod):

    def _A_ref(x, w_r, w_i):
        B, S, D = x.shape
        X = (lambda x, axes=(-2, -1): jnp.fft.rfft2(x.astype(jnp.float32), axes=axes))(x, axes=(-2, -1))
        W = w_r + 1j * w_i
        X = X * W
        y = (lambda x, s, axes=(-2, -1): jnp.fft.irfft2(x, s=s, axes=axes).astype(jnp.bfloat16))(X, (S, D), axes=(-2, -1))
        return y

    def _B_ref(x, w1, b1, w2, b2):
        B, S, D = x.shape
        h = _layernorm(x, axis=-1)
        u = jnp.einsum('bsd,sf->bdf', h, w1) + b1
        u = _gelu(u)
        y = jnp.einsum('bdf,fs->bds', u, w2) + b2
        return (lambda x, *d: x.transpose(*d))(y, 0, 2, 1)
    x = A_x
    mod = (_silu(c) @ w_mod).reshape(c.shape[0], 6, 1, -1)
    sa, ca, ga, sb, cb, gb = (mod[:, 0].copy(), mod[:, 1].copy(), mod[:, 2].copy(), mod[:, 3].copy(), mod[:, 4].copy(), mod[:, 5].copy())
    h = _layernorm(x, axis=-1) * (1 + ca) + sa
    x = x + ga * _A_ref(h, A_w_r, A_w_i)
    h = _layernorm(x, axis=-1) * (1 + cb) + sb
    x = x + gb * _B_ref(h, B_w1, B_b1, B_w2, B_b2)
    return x
```

```python
import functools

import jax
import jax.numpy as jnp
import numpy as np
import ml_dtypes
import jax.experimental.pallas as pl
import jax.experimental.pallas.tpu as pltpu

S, D, F = 2048, 576, 4608
NT = S // 128
NQ = 37
NR = NQ * 16
H = D // 2
f32, bf16, u32 = jnp.float32, jnp.bfloat16, jnp.uint32
EPS = 1e-5

_TH = 2 * np.pi / 9
C1, C2, C4 = float(np.cos(_TH)), float(np.cos(2 * _TH)), float(np.cos(4 * _TH))
S1, S3, S4 = float(np.sin(_TH)), float(np.sin(3 * _TH)), float(np.sin(4 * _TH))


def _row_groups():
    gs = []
    for g in range(1, 5):
        for c in (g, g + 9, 9 - g, 18 - g):
            for mh in range(2):
                gs.append((g, c, mh))
    for c in (0, 9):
        for mh in range(2):
            gs.append((0, c, mh))
    gs.append((0, 288, 0))
    return gs


_GROUPS = _row_groups()


def _d_mats():
    d2 = np.arange(64)
    fwd = np.zeros((5, 128, 128))
    inv = np.zeros((5, 128, 128))
    sc = {1: S1, 2: S1, 4: S1, 3: S3}
    kcol = 16 * (d2 // 8) + 2 * (d2 % 8)
    for g in range(5):
        loc = [x for x in _GROUPS if x[0] == g]
        for ql, (_, c0, mh) in enumerate(loc):
            kxs = [288] if c0 == 288 else [c0 + 18 * (8 * mh + i) for i in range(8)]
            for i, kx in enumerate(kxs):
                ph = 2 * np.pi * ((kx * d2) % D) / D
                c, s = np.cos(ph), np.sin(ph)
                if kx % 288 == 0:
                    s = np.zeros_like(s)
                sg = 1.0 if kx % 9 == g else -1.0
                rr, ri = 16 * ql + i, 16 * ql + 8 + i
                fwd[g, rr, kcol] = c
                fwd[g, ri, kcol] = -s
                w = (1.0 if kx % 288 == 0 else 2.0) / (S * D)
                kr, ki = 16 * ql + 2 * i, 16 * ql + 2 * i + 1
                inv[g, d2, kr] = w * c
                inv[g, d2, ki] = -w * s
                if g:
                    fwd[g, rr, kcol + 1] = -sg * s * sc[g]
                    fwd[g, ri, kcol + 1] = -sg * c * sc[g]
                    inv[g, 64 + d2, kr] = sg * w * s * sc[g]
                    inv[g, 64 + d2, ki] = sg * w * c * sc[g]
    return np.concatenate([fwd, inv], 0).astype(ml_dtypes.bfloat16)


def _s_mats():
    m = np.zeros((NT, 2, 128, 128))
    lane = np.arange(128)
    for b in range(NT):
        a = (lane - b) % 16
        k = 128 * a + (lane - a) % 128
        ph = 2 * np.pi * ((lane[:, None] * k[None, :]) % S) / S
        m[b, 0] = np.cos(ph)
        m[b, 1] = -np.sin(ph)
    return m.astype(ml_dtypes.bfloat16)


_DMAT = _d_mats()
_SMAT = _s_mats()


def _dot(a, b):
    return jnp.dot(a, b, preferred_element_type=f32)


def _dot_t(a, b):
    return jax.lax.dot_general(a, b, (((1,), (1,)), ((), ())), preferred_element_type=f32)


def _pack(a, b):
    return pltpu.pack_elementwise([a, b], packed_dtype=bf16)


def _unpack(x, i):
    return pltpu.unpack_elementwise(x, index=i, packed_dtype=bf16, unpacked_dtype=f32)


def _radix9_fwd(a):
    p = [None] + [a[n] + a[9 - n] for n in range(1, 5)]
    m = [None] + [a[n] - a[9 - n] for n in range(1, 5)]
    t = p[1] + p[2] + p[4]
    u = a[0] + p[3]
    b = a[0] - 0.5 * p[3]
    e1 = p[1] - p[4]
    e2 = p[2] - p[4]
    r1 = C1 * e1 + C2 * e2
    r2 = C2 * e1 + C4 * e2
    f1 = m[1] + m[2]
    f2 = m[2] + m[4]
    f3 = m[1] - m[4]
    q1 = f1 + (S4 / S1) * f2
    q2 = f3 + (S4 / S1) * f1
    n3 = (S3 / S1) * m[3]
    return u + t, [(b + r1, q1 + n3), (b + r2, q2 - n3), (u - 0.5 * t, m[1] - m[2] + m[4]),
                   (b - (r1 + r2), (q2 - q1) + n3)]


def _radix9_inv(v0, v):
    (r1_, i1), (r2_, i2), (r3_, i3), (r4_, i4) = v
    t = r1_ + r2_ + r4_
    u = v0 + r3_
    b = v0 - 0.5 * r3_
    e1 = r1_ - r4_
    e2 = r2_ - r4_
    r1 = C1 * e1 + C2 * e2
    r2 = C2 * e1 + C4 * e2
    a1, a2, a3, a4 = b + r1, b + r2, u - 0.5 * t, b - (r1 + r2)
    f1 = i1 + i2
    f2 = i2 + i4
    f3 = i1 - i4
    q1 = f1 + (S4 / S1) * f2
    q2 = f3 + (S4 / S1) * f1
    b1, b2, b4 = q1 + i3, q2 - i3, (q2 - q1) + i3
    b3 = (S3 / S1) * (i1 - i2 + i4)
    return [u + t, a1 - b1, a2 - b2, a3 - b3, a4 - b4, a4 + b4, a3 + b3, a2 + b2, a1 + b1]


def _bfly4(a, b, c, d, sgn, c_rot=False):
    if c_rot:
        if sgn < 0:
            t0 = (a[0] + c[1], a[1] - c[0])
            t1 = (a[0] - c[1], a[1] + c[0])
        else:
            t0 = (a[0] - c[1], a[1] + c[0])
            t1 = (a[0] + c[1], a[1] - c[0])
    else:
        t0 = (a[0] + c[0], a[1] + c[1])
        t1 = (a[0] - c[0], a[1] - c[1])
    t2 = (b[0] + d[0], b[1] + d[1])
    t3 = (b[0] - d[0], b[1] - d[1])
    x0 = (t0[0] + t2[0], t0[1] + t2[1])
    x2 = (t0[0] - t2[0], t0[1] - t2[1])
    xm = (t1[0] + t3[1], t1[1] - t3[0])
    xp = (t1[0] - t3[1], t1[1] + t3[0])
    return [x0, xm, x2, xp] if sgn < 0 else [x0, xp, x2, xm]


def _tw16(z, e, sgn):
    c = float(np.cos(2 * np.pi * e / 16))
    s = float(sgn * np.sin(2 * np.pi * e / 16))
    x, y = z
    if e % 2 == 0:
        if (c > 0) == (s > 0):
            return ((x - y) * c, (x + y) * c)
        return ((x + y) * c, (y - x) * c)
    return (x * c - y * s, x * s + y * c)


def _radix16(x, sgn):
    u = [_bfly4(x[n2], x[4 + n2], x[8 + n2], x[12 + n2], sgn) for n2 in range(4)]
    out = [None] * 16
    for k1 in range(4):
        v = []
        for n2 in range(4):
            e = k1 * n2
            v.append(u[n2][k1] if e % 4 == 0 else _tw16(u[n2][k1], e, sgn))
        y = _bfly4(v[0], v[1], v[2], v[3], sgn, c_rot=(k1 == 2))
        for k2 in range(4):
            out[k1 + 4 * k2] = y[k2]
    return out


def _a_ops(a11, a12, a21, a22):
    return [a11 + a22, a21 + a22, a11, a22, a11 + a12, a21 - a11, a12 - a22]


def _b_ops(b11, b12, b21, b22):
    c = lambda v: v.astype(f32)
    p = lambda v: v.astype(bf16)
    return [p(c(b11) + c(b22)), b11, p(c(b12) - c(b22)), p(c(b21) - c(b11)), b22,
            p(c(b11) + c(b12)), p(c(b21) + c(b22))]


def _c_ops(m):
    m1, m2, m3, m4, m5, m6, m7 = m
    return m1 + m4 - m5 + m7, m3 + m5, m2 + m4, m1 - m2 + m3 + m6


def _gelu2(u):
    k0 = 0.7978845608028654
    z = u * (k0 + (k0 * 0.044715) * (u * u))
    return u * jnp.tanh(z) + u


def _colsum(vs):
    acc = vs[0]
    for v in vs[1:]:
        acc = acc + v
    return jnp.sum(acc, axis=0, keepdims=True)


FC = 512
NF = F // FC
SC = 512
NS = S // SC
XC = 4


def _kernel(xT_h, wr_h, wi_h, w1_h, b1_h, w2_h, b2_h, c_h, wm_h, dm_h, sm_h, out_h,
            xT, wraw_r, wraw_i, wp, w1v, w2v, b1v, b2v, cv, wm, dm, sm, tbl, ybuf, xbuf, cbuf,
            x1, aop, gop, obuf, sem, osem, *, stop):
    n = [0]

    def cp(src, dst):
        d = pltpu.make_async_copy(src, dst, sem.at[n[0]])
        n[0] += 1
        return d

    cp_c = cp(c_h, cv)
    cp_wm0 = cp(wm_h.at[:, 0:1152], wm.at[:, 0:1152])
    xw = S // XC
    cp_x = [cp(xT_h.at[:, i * xw:(i + 1) * xw], xT.at[:, i * xw:(i + 1) * xw]) for i in range(XC)]
    cp_dm = cp(dm_h, dm)
    cp_wr = cp(wr_h, wraw_r)
    cp_wi = cp(wi_h, wraw_i)
    cp_sm = cp(sm_h, sm)
    cp_wm1 = cp(wm_h.at[:, 1152:6 * D], wm.at[:, 1152:6 * D])
    cp_b1 = cp(b1_h, b1v)
    cp_b2 = cp(b2_h, b2v)
    cp_w1 = [cp(w1_h.at[:, i * FC:(i + 1) * FC], w1v.at[i]) for i in range(NF)]
    cp_w2 = [cp(w2_h.at[:, i * SC:(i + 1) * SC], w2v.at[i]) for i in range(NS)]
    w1sem = n[0] - NS - NF
    w2sem = n[0] - NS

    for d in [cp_c, cp_wm0] + cp_x + [cp_dm, cp_wr, cp_wi, cp_sm, cp_wm1, cp_b1, cp_b2]:
        d.start()

    cp_c.wait()
    cc = cv[...].astype(f32)
    sc = jnp.broadcast_to(cc * jax.nn.sigmoid(cc), (16, D)).astype(bf16)

    def mod_part(lo, hi):
        mod = _dot(sc, wm[:, lo:hi])
        for j in range((hi - lo) // 128):
            row = jnp.broadcast_to(mod[0:1, j * 128:(j + 1) * 128], (128, 128))
            tbl[lo + j * 128:lo + (j + 1) * 128, :] = row.T

    cp_wm0.wait()
    mod_part(0, 1152)
    tbl[D:2 * D, :] = tbl[D:2 * D, :] + 1.0

    cp_dm.wait()

    def phase_b(t):
        ln = pl.ds(pl.multiple_of(t * 128, 128), 128)
        xs = [xT[8 * r:8 * r + 8, ln].astype(f32) for r in range(D // 8)]
        mean = _colsum(xs) * (1.0 / D)
        xc = [v - mean for v in xs]
        var = _colsum([v * v for v in xc]) * (1.0 / D)
        rs = jax.lax.rsqrt(var + EPS)
        for j in range(8):
            a = []
            for n9 in range(9):
                r = 8 * n9 + j
                a.append(xc[r] * rs * tbl[D + 8 * r:D + 8 * r + 8, :] + tbl[8 * r:8 * r + 8, :])
            y0, ys = _radix9_fwd(a)
            ybuf[t, 4, 8 * j:8 * j + 8, :] = _pack(y0, jnp.zeros_like(y0))
            for g in range(4):
                ybuf[t, g, 8 * j:8 * j + 8, :] = _pack(*ys[g])
        for g in range(4):
            xbuf[t, 128 * g:128 * (g + 1), :] = _dot(dm[g + 1], pltpu.bitcast(ybuf[t, g], bf16))
        xbuf[t, 512:NR, :] = _dot(dm[0, 0:80, :], pltpu.bitcast(ybuf[t, 4], bf16))

    for i in range(XC):
        cp_x[i].wait()
        if i == 1:
            for d in cp_w1:
                d.start()
        jax.lax.fori_loop(i * (NT // XC), (i + 1) * (NT // XC), lambda t, _: phase_b(t), None)

    cp_wr.wait()
    cp_wi.wait()
    lane = jax.lax.broadcasted_iota(jnp.int32, (8, 128), 1)
    masks = [(lane & (1 << b)) != 0 for b in range(4)]

    def shuffle(vals):
        vals = [pltpu.roll(v, a, 1) if a else v for a, v in enumerate(vals)]
        vals = [vals[(-b) % 16] for b in range(16)]
        for b in range(4):
            vals = [jnp.where(masks[b], vals[(i - (1 << b)) % 16], vals[i]) for i in range(16)]
        return vals

    def w_rows(r, _):
        for p, raw in enumerate((wraw_r, wraw_i)):
            rows = pl.ds(pl.multiple_of(r * 16, 16), 16)
            vals = shuffle([pltpu.bitcast(raw[rows, a * 128:(a + 1) * 128], u32) for a in range(16)])
            for b in range(16):
                wp[p, b, pl.ds(pl.multiple_of(r * 8, 8), 8), :] = vals[b]

    jax.lax.fori_loop(0, 18, w_rows, None)
    for p, raw in enumerate((wraw_r, wraw_i)):
        last = jnp.broadcast_to(raw[288:289, :].astype(f32), (8, S))
        vals = shuffle([last[:, a * 128:(a + 1) * 128] for a in range(16)])
        for b in range(16):
            wp[p, b, 144:152, :] = pltpu.bitcast(vals[b], u32)

    def phase_c(q, _):
        r0 = pl.multiple_of(q * 16, 16)
        y = _radix16([(xbuf[t, pl.ds(r0, 8), :], xbuf[t, pl.ds(r0 + 8, 8), :]) for t in range(NT)], -1)
        for b in range(NT):
            cbuf[b, pl.ds(r0, 16), :] = jnp.concatenate(y[b], axis=0).astype(bf16)

    jax.lax.fori_loop(0, NQ, phase_c, None)

    cp_sm.wait()

    def w_group(p, b, grp):
        _, c0, mh = grp
        if c0 == 288:
            return pltpu.bitcast(wp[p, b, 144:152, :], f32)
        return _unpack(wp[p, b, pl.ds(c0 // 2 + 72 * mh, 8, stride=9), :], c0 % 2)

    def phase_d(b, _):
        fr, fi = sm[b, 0], sm[b, 1]
        pp = _dot(cbuf[b], jnp.concatenate([fr, fi], axis=1))
        zs = []
        for q, grp in enumerate(_GROUPS):
            re, im = pp[16 * q:16 * q + 8], pp[16 * q + 8:16 * q + 16]
            xr = re[:, :128] - im[:, 128:]
            xi = re[:, 128:] + im[:, :128]
            wr, wi = w_group(0, b, grp), w_group(1, b, grp)
            zs += [xr * wr - xi * wi, xr * wi + xi * wr]
        z = jnp.concatenate(zs, axis=0).astype(bf16)
        qq = _dot_t(z, jnp.concatenate([fr, fi], axis=0))
        for q in range(NQ):
            re, im = qq[16 * q:16 * q + 8], qq[16 * q + 8:16 * q + 16]
            xbuf[b, 16 * q:16 * q + 8, :] = re[:, :128] + im[:, 128:]
            xbuf[b, 16 * q + 8:16 * q + 16, :] = im[:, :128] - re[:, 128:]

    jax.lax.fori_loop(0, NT, phase_d, None, unroll=2)

    for d in cp_w2:
        d.start()

    def phase_e(q, _):
        r0 = pl.multiple_of(q * 16, 16)
        y = _radix16([(xbuf[b, pl.ds(r0, 8), :], xbuf[b, pl.ds(r0 + 8, 8), :]) for b in range(NT)], 1)
        for t in range(NT):
            ybuf[t, q // 8, pl.ds(pl.multiple_of((q % 8) * 8, 8), 8), :] = _pack(*y[t])

    jax.lax.fori_loop(0, NQ, phase_e, None)

    cp_wm1.wait()
    mod_part(1152, 6 * D)
    tbl[4 * D:5 * D, :] = tbl[4 * D:5 * D, :] + 1.0

    def tile_f(t):
        ln = pl.ds(pl.multiple_of(t * 128, 128), 128)
        v = [_dot(dm[6 + g], pltpu.bitcast(ybuf[t, g], bf16)) for g in range(4)]
        v0 = _dot(dm[5, 0:64, 0:80], pltpu.bitcast(ybuf[t, 4, 0:40, :], bf16))
        xs = [None] * (D // 8)
        for j in range(8):
            sl = slice(8 * j, 8 * j + 8)
            sh = slice(64 + 8 * j, 64 + 8 * j + 8)
            ys = _radix9_inv(v0[sl], [(vg[sl], vg[sh]) for vg in v])
            for n9 in range(9):
                r = 8 * n9 + j
                xs[r] = xT[8 * r:8 * r + 8, ln].astype(f32) + ys[n9] * tbl[2 * D + 8 * r:2 * D + 8 * r + 8, :]
                x1[t, 8 * r:8 * r + 8, :] = xs[r]
        mean = _colsum(xs) * (1.0 / D)
        xc = [x - mean for x in xs]
        rs = jax.lax.rsqrt(_colsum([x * x for x in xc]) * (1.0 / D) + EPS)
        hs = [x * rs * tbl[4 * D + 8 * r:4 * D + 8 * r + 8, :] + tbl[3 * D + 8 * r:3 * D + 8 * r + 8, :]
              for r, x in enumerate(xc)]
        mean = _colsum(hs) * (1.0 / D)
        hc = [x - mean for x in hs]
        rs = jax.lax.rsqrt(_colsum([x * x for x in hc]) * (1.0 / D) + EPS)
        return [x * rs for x in hc]

    def phase_f(tp, _):
        h0 = tile_f(2 * tp)
        h1 = tile_f(2 * tp + 1)
        hh = H // 8
        for r in range(0, hh, 2):
            ops = [_a_ops(h0[r + k], h1[r + k], h0[hh + r + k], h1[hh + r + k]) for k in range(2)]
            for j in range(7):
                aop[j, tp, 8 * r:8 * r + 16, :] = jnp.concatenate([ops[0][j], ops[1][j]], axis=0).astype(bf16)

    jax.lax.fori_loop(0, NT // 2, phase_f, None)

    cp_b1.wait()
    cp_b2.wait()
    b1f = b1v[...].astype(f32)
    b2f = b2v[...].astype(f32)
    tbl[0:40, :] = jnp.concatenate([b1f, jnp.zeros((4, 128), f32)], axis=0)
    tbl[40:56, :] = b2f
    n1 = FC // 2

    def mlp1(i, _):
        pltpu.make_async_copy(w1_h.at[:, 0:FC], w1v.at[i], sem.at[w1sem + i]).wait()
        w = w1v.at[i]

        def blk(r, c):
            return jnp.concatenate([w[(2 * k + r) * 128:(2 * k + r + 1) * 128, c * n1:(c + 1) * n1]
                                    for k in range(NT // 2)], axis=0)

        bs = _b_ops(blk(0, 0), blk(0, 1), blk(1, 0), blk(1, 1))
        m = [_dot(jnp.concatenate([aop[j, k] for k in range(NT // 2)], axis=1), bs[j]) for j in range(7)]
        cs = _c_ops(m)
        bias = [jnp.concatenate([tbl[pl.ds(i * (FC // 128) + c * (n1 // 128) + k, 1), :] for k in range(n1 // 128)],
                                axis=1) for c in range(2)]
        g = [_gelu2(cs[k] + bias[k % 2]) for k in range(4)]
        ops = _a_ops(*g)
        for j in range(7):
            for k in range(n1 // 128):
                gop[j, i * (n1 // 128) + k] = ops[j][:, k * 128:(k + 1) * 128].astype(bf16)

    jax.lax.fori_loop(0, NF, mlp1, None)

    n2 = SC // 2

    def out_copy(i):
        return pltpu.make_async_copy(obuf.at[i], out_h.at[:, pl.ds(pl.multiple_of(i * SC, SC), SC)], osem.at[i])

    def mlp2(i, _):
        pltpu.make_async_copy(w2_h.at[:, 0:SC], w2v.at[i], sem.at[w2sem + i]).wait()
        w = w2v.at[i]

        def blk(r, c):
            return jnp.concatenate([w[k * FC + r * n1:k * FC + (r + 1) * n1, c * n2:(c + 1) * n2]
                                    for k in range(NF)], axis=0)

        bs = _b_ops(blk(0, 0), blk(0, 1), blk(1, 0), blk(1, 1))
        m = [_dot(jnp.concatenate([gop[j, k] for k in range(F // 256)], axis=1), bs[j]) for j in range(7)]
        cs = _c_ops(m)
        for k in range(4):
            rh, ch = divmod(k, 2)
            gb = tbl[5 * D + rh * H:5 * D + (rh + 1) * H, :]
            for tt in range(n2 // 128):
                tl = ch * (n2 // 128) + tt
                t = i * (SC // 128) + tl
                y = cs[k][:, tt * 128:(tt + 1) * 128] * 0.5 + tbl[pl.ds(40 + t, 1), :]
                obuf[i, rh * H:(rh + 1) * H, tl * 128:(tl + 1) * 128] = (
                    x1[t, rh * H:(rh + 1) * H, :] + gb * y).astype(bf16)
        out_copy(i).start()

    jax.lax.fori_loop(0, NS, mlp2, None)
    for i in range(NS):
        out_copy(i).wait()


@jax.jit
def pallas_adaLN_cond__spectral_gfnet__mixer_token_mlp__prompt_kernel(
    A_x: jax.Array,
    A_w_r: jax.Array,
    A_w_i: jax.Array,
    B_x: jax.Array,
    B_w1: jax.Array,
    B_b1: jax.Array,
    B_w2: jax.Array,
    B_b2: jax.Array,
    c: jax.Array,
    w_mod: jax.Array,
):
    del B_x
    any_spec = pl.BlockSpec(memory_space=pl.ANY)
    scratch = [
        pltpu.VMEM((D, S), bf16),
        pltpu.VMEM((289, S), bf16),
        pltpu.VMEM((289, S), bf16),
        pltpu.VMEM((2, NT, 152, 128), u32),
        pltpu.VMEM((NF, S, FC), bf16),
        pltpu.VMEM((NS, F, SC), bf16),
        pltpu.VMEM((F // 128, 128), bf16),
        pltpu.VMEM((S // 128, 128), bf16),
        pltpu.VMEM((1, D), bf16),
        pltpu.VMEM((D, 6 * D), bf16),
        pltpu.VMEM((10, 128, 128), bf16),
        pltpu.VMEM((NT, 2, 128, 128), bf16),
        pltpu.VMEM((6 * D, 128), f32),
        pltpu.VMEM((NT, 5, 64, 128), u32),
        pltpu.VMEM((NT, NR, 128), f32),
        pltpu.VMEM((NT, NR, 128), bf16),
        pltpu.VMEM((NT, D, 128), f32),
        pltpu.VMEM((7, NT // 2, H, 128), bf16),
        pltpu.VMEM((7, F // 256, H, 128), bf16),
        pltpu.VMEM((NS, D, SC), bf16),
        pltpu.SemaphoreType.DMA((32,)),
        pltpu.SemaphoreType.DMA((NS,)),
    ]
    outT = pl.pallas_call(
        functools.partial(_kernel, stop=None),
        out_shape=jax.ShapeDtypeStruct((D, S), bf16),
        in_specs=[any_spec] * 11,
        out_specs=any_spec,
        scratch_shapes=scratch,
        compiler_params=pltpu.CompilerParams(vmem_limit_bytes=120 * 1024 * 1024),
        name="adaln_gfnet_mixer",
    )(A_x[0].T, A_w_r.T, A_w_i.T, B_w1, B_b1.reshape(F // 128, 128), B_w2,
      B_b2.reshape(S // 128, 128), c, w_mod, _DMAT, _SMAT)
    return outT.T[None]
```

```python
import contextlib
import functools

import jax
import jax.numpy as jnp
import numpy as np
import ml_dtypes
import jax.experimental.pallas as pl
import jax.experimental.pallas.tpu as pltpu

S, D, F = 2048, 576, 4608
NT = S // 128
NQ = 37
NR = NQ * 16
H = D // 4
f32, bf16, u32 = jnp.float32, jnp.bfloat16, jnp.uint32
EPS = 1e-5

_TH = 2 * np.pi / 9
C1, C2, C4 = float(np.cos(_TH)), float(np.cos(2 * _TH)), float(np.cos(4 * _TH))
S1, S3, S4 = float(np.sin(_TH)), float(np.sin(3 * _TH)), float(np.sin(4 * _TH))


def _row_groups():
    gs = []
    for g in range(1, 5):
        for c in (g, g + 9, 9 - g, 18 - g):
            for mh in range(2):
                gs.append((g, c, mh))
    for c in (0, 9):
        for mh in range(2):
            gs.append((0, c, mh))
    gs.append((0, 288, 0))
    return gs


_GROUPS = _row_groups()


def _d_mats():
    d2 = np.arange(64)
    fwd = np.zeros((5, 128, 128))
    inv = np.zeros((5, 128, 128))
    sc = {1: S1, 2: S1, 4: S1, 3: S3}
    kcol = 16 * (d2 // 8) + 2 * (d2 % 8)
    for g in range(5):
        loc = [x for x in _GROUPS if x[0] == g]
        for ql, (_, c0, mh) in enumerate(loc):
            kxs = [288] if c0 == 288 else [c0 + 18 * (8 * mh + i) for i in range(8)]
            for i, kx in enumerate(kxs):
                ph = 2 * np.pi * ((kx * d2) % D) / D
                c, s = np.cos(ph), np.sin(ph)
                if kx % 288 == 0:
                    s = np.zeros_like(s)
                sg = 1.0 if kx % 9 == g else -1.0
                rr, ri = 16 * ql + i, 16 * ql + 8 + i
                fwd[g, rr, kcol] = c
                fwd[g, ri, kcol] = -s
                w = (1.0 if kx % 288 == 0 else 2.0) / (S * D)
                kr, ki = 16 * ql + 2 * i, 16 * ql + 2 * i + 1
                inv[g, d2, kr] = w * c
                inv[g, d2, ki] = -w * s
                if g:
                    fwd[g, rr, kcol + 1] = -sg * s * sc[g]
                    fwd[g, ri, kcol + 1] = -sg * c * sc[g]
                    inv[g, 64 + d2, kr] = sg * w * s * sc[g]
                    inv[g, 64 + d2, ki] = sg * w * c * sc[g]
    return np.concatenate([fwd, inv], 0).astype(ml_dtypes.bfloat16)


def _s_mats():
    m = np.zeros((NT, 2, 128, 128))
    lane = np.arange(128)
    for b in range(NT):
        a = (lane - b) % 16
        k = 128 * a + (lane - a) % 128
        ph = 2 * np.pi * ((lane[:, None] * k[None, :]) % S) / S
        m[b, 0] = np.cos(ph)
        m[b, 1] = -np.sin(ph)
    return m.astype(ml_dtypes.bfloat16)


_DMAT = _d_mats()
_SMAT = _s_mats()


def _dot(a, b):
    return jnp.dot(a, b, preferred_element_type=f32)


def _dot_t(a, b):
    return jax.lax.dot_general(a, b, (((1,), (1,)), ((), ())), preferred_element_type=f32)


def _pack(a, b):
    return pltpu.pack_elementwise([a, b], packed_dtype=bf16)


def _unpack(x, i):
    return pltpu.unpack_elementwise(x, index=i, packed_dtype=bf16, unpacked_dtype=f32)


def _radix9_fwd(a):
    p = [None] + [a[n] + a[9 - n] for n in range(1, 5)]
    m = [None] + [a[n] - a[9 - n] for n in range(1, 5)]
    t = p[1] + p[2] + p[4]
    u = a[0] + p[3]
    b = a[0] - 0.5 * p[3]
    e1 = p[1] - p[4]
    e2 = p[2] - p[4]
    r1 = C1 * e1 + C2 * e2
    r2 = C2 * e1 + C4 * e2
    f1 = m[1] + m[2]
    f2 = m[2] + m[4]
    f3 = m[1] - m[4]
    q1 = f1 + (S4 / S1) * f2
    q2 = f3 + (S4 / S1) * f1
    n3 = (S3 / S1) * m[3]
    return u + t, [(b + r1, q1 + n3), (b + r2, q2 - n3), (u - 0.5 * t, m[1] - m[2] + m[4]),
                   (b - (r1 + r2), (q2 - q1) + n3)]


def _radix9_inv(v0, v):
    (r1_, i1), (r2_, i2), (r3_, i3), (r4_, i4) = v
    t = r1_ + r2_ + r4_
    u = v0 + r3_
    b = v0 - 0.5 * r3_
    e1 = r1_ - r4_
    e2 = r2_ - r4_
    r1 = C1 * e1 + C2 * e2
    r2 = C2 * e1 + C4 * e2
    a1, a2, a3, a4 = b + r1, b + r2, u - 0.5 * t, b - (r1 + r2)
    f1 = i1 + i2
    f2 = i2 + i4
    f3 = i1 - i4
    q1 = f1 + (S4 / S1) * f2
    q2 = f3 + (S4 / S1) * f1
    b1, b2, b4 = q1 + i3, q2 - i3, (q2 - q1) + i3
    b3 = (S3 / S1) * (i1 - i2 + i4)
    return [u + t, a1 - b1, a2 - b2, a3 - b3, a4 - b4, a4 + b4, a3 + b3, a2 + b2, a1 + b1]


def _bfly4(a, b, c, d, sgn, c_rot=False):
    if c_rot:
        if sgn < 0:
            t0 = (a[0] + c[1], a[1] - c[0])
            t1 = (a[0] - c[1], a[1] + c[0])
        else:
            t0 = (a[0] - c[1], a[1] + c[0])
            t1 = (a[0] + c[1], a[1] - c[0])
    else:
        t0 = (a[0] + c[0], a[1] + c[1])
        t1 = (a[0] - c[0], a[1] - c[1])
    t2 = (b[0] + d[0], b[1] + d[1])
    t3 = (b[0] - d[0], b[1] - d[1])
    x0 = (t0[0] + t2[0], t0[1] + t2[1])
    x2 = (t0[0] - t2[0], t0[1] - t2[1])
    xm = (t1[0] + t3[1], t1[1] - t3[0])
    xp = (t1[0] - t3[1], t1[1] + t3[0])
    return [x0, xm, x2, xp] if sgn < 0 else [x0, xp, x2, xm]


def _tw16(z, e, sgn):
    c = float(np.cos(2 * np.pi * e / 16))
    s = float(sgn * np.sin(2 * np.pi * e / 16))
    x, y = z
    if e % 2 == 0:
        if (c > 0) == (s > 0):
            return ((x - y) * c, (x + y) * c)
        return ((x + y) * c, (y - x) * c)
    return (x * c - y * s, x * s + y * c)


def _radix16(x, sgn):
    u = [_bfly4(x[n2], x[4 + n2], x[8 + n2], x[12 + n2], sgn) for n2 in range(4)]
    out = [None] * 16
    for k1 in range(4):
        v = []
        for n2 in range(4):
            e = k1 * n2
            v.append(u[n2][k1] if e % 4 == 0 else _tw16(u[n2][k1], e, sgn))
        y = _bfly4(v[0], v[1], v[2], v[3], sgn, c_rot=(k1 == 2))
        for k2 in range(4):
            out[k1 + 4 * k2] = y[k2]
    return out


def _sa(a11, a12, a21, a22):
    return [a11 + a22, a21 + a22, a11, a22, a11 + a12, a21 - a11, a12 - a22]


def _sb(b11, b12, b21, b22):
    return [b11 + b22, b11, b12 - b22, b21 - b11, b22, b11 + b12, b21 + b22]


def _sc(m):
    m1, m2, m3, m4, m5, m6, m7 = m
    return [m4 + m7 - m5 + m1, m5 + m3, m2 + m4, m1 - m2 + m3 + m6]


def _sa2(blk):
    lvl = [_sa(blk[ri][ci], blk[ri][2 + ci], blk[2 + ri][ci], blk[2 + ri][2 + ci])
           for ri in range(2) for ci in range(2)]
    return [x for o in range(7) for x in _sa(*[l[o] for l in lvl])]


def _sc2(m):
    p = [_sc(m[7 * o:7 * o + 7]) for o in range(7)]
    out = [[None] * 4 for _ in range(4)]
    for ii in range(4):
        for oi, v in enumerate(_sc([p[o][ii] for o in range(7)])):
            out[2 * (oi // 2) + ii // 2][2 * (oi % 2) + ii % 2] = v
    return out


_SB_TERMS = (((1, 0, 0), (1, 1, 1)), ((1, 0, 0),), ((1, 0, 1), (-1, 1, 1)), ((1, 1, 0), (-1, 0, 0)),
             ((1, 1, 1),), ((1, 0, 0), (1, 0, 1)), ((1, 1, 0), (1, 1, 1)))
_ORDER = (1, 3, 6, 4, 0, 2, 5)


def _strassen2(lhs, raw):
    m = [None] * 49
    for o in _ORDER:
        blocks = {}
        halves = []
        for h in range(2):
            quad = []
            for ri in range(2):
                for ci in range(2):
                    acc = None
                    for sg, ro, co in _SB_TERMS[o]:
                        key = (2 * ro + ri, 2 * co + ci)
                        if key not in blocks:
                            blocks[key] = raw(o, *key)
                        v = _unpack(blocks[key], h)
                        acc = v if acc is None else (acc + v if sg > 0 else acc - v)
                    quad.append(acc)
            halves.append(_sb(*quad))
        for j in _ORDER:
            rhs = pltpu.bitcast(_pack(halves[0][j], halves[1][j]), bf16)
            m[7 * o + j] = _dot(lhs(7 * o + j), rhs)
    return m


def _gelu2(u):
    k0 = 0.7978845608028654
    z = u * (k0 + (k0 * 0.044715) * (u * u))
    return u * jnp.tanh(z) + u


def _tree(vs):
    vs = list(vs)
    while len(vs) > 1:
        vs = [vs[i] + vs[i + 1] if i + 1 < len(vs) else vs[i] for i in range(0, len(vs), 2)]
    return vs[0]


def _colsum(vs, lanes=4):
    accs = []
    for k in range(lanes):
        acc = None
        for v in vs[k::lanes]:
            acc = v if acc is None else acc + v
        accs.append(acc)
    return jnp.sum(_tree(accs), axis=0, keepdims=True)


def _interleave(*lists):
    items = []
    for ci, lst in enumerate(lists):
        for k, it in enumerate(lst):
            items.append(((k + 0.5) / len(lst), ci, k, it))
    items.sort(key=lambda x: x[:3])
    for x in items:
        x[3]()


FC = 512
NF = F // FC
SC = 512
NS = S // SC
XC = 4
DS1 = 8
DS2 = 8


def _kernel(zsm, xT_h, wr_h, wi_h, w1_h, b1_h, w2_h, b2_h, c_h, wm_h, dm_h, sm_h, out_h,
            xT, wraw_r, wraw_i, wp, w1v, w2v, b1v, b2v, cv, wm, dm, sm, tbl, ybuf, xbuf, cbuf, sab,
            mnb, stat, zbuf, x1, aop, gop, obuf, sem, w1sem, w2sem, osem, *, scopes, u1):
    n = [0]

    def scope(name):
        return jax.named_scope(name) if scopes else contextlib.nullcontext()

    def cp(src, dst):
        d = pltpu.make_async_copy(src, dst, sem.at[n[0]])
        n[0] += 1
        return d

    cp_c = cp(c_h, cv)
    cp_wm0 = cp(wm_h.at[:, 512:1152], wm.at[:, 512:1152])
    cp_dm = cp(dm_h, dm)
    xw = S // XC
    cp_x = [cp(xT_h.at[:, i * xw:(i + 1) * xw], xT.at[:, i * xw:(i + 1) * xw]) for i in range(XC)]
    cp_wms = cp(wm_h.at[:, 0:512], wm.at[:, 0:512])
    cp_sm = cp(sm_h, sm)
    cp_wr = cp(wr_h, wraw_r)
    cp_wi = cp(wi_h, wraw_i)
    cp_wm1 = cp(wm_h.at[:, 1152:6 * D], wm.at[:, 1152:6 * D])
    cp_b1 = cp(b1_h, b1v)
    cp_b2 = cp(b2_h, b2v)
    xsem = 3

    def strip(src, dst, sems, j):
        cols = pl.ds(pl.multiple_of(j * 128, 128), 128)
        return pltpu.make_async_copy(src.at[:, cols], dst.bitcast(bf16).at[j], sems.at[j])

    cp_w1 = [strip(w1_h, w1v, w1sem, j) for j in range(F // 128)]
    cp_w2 = [strip(w2_h, w2v, w2sem, j) for j in range(NT)]

    for d in [cp_c, cp_wm0, cp_x[0], cp_dm] + cp_x[1:] + [cp_wms, cp_sm, cp_wr, cp_wi, cp_wm1, cp_b1, cp_b2]:
        d.start()

    cp_c.wait()
    cc = cv[...].astype(f32)
    sc = jnp.broadcast_to(cc * jax.nn.sigmoid(cc), (16, D)).astype(bf16)

    def mod_items(lo, hi):
        box = []

        def first():
            box.append(_dot(sc, wm[:, lo:hi]))

        def tile(j):
            r0 = lo + j * 128
            row = box[0][0:1, j * 128:(j + 1) * 128]
            col = r0 + jax.lax.broadcasted_iota(jnp.int32, (1, 128), 1)
            is_scale = ((col >= D) & (col < 2 * D)) | ((col >= 4 * D) & (col < 5 * D))
            row = row * jnp.where(col >= 5 * D, 0.5, 1.0) + jnp.where(is_scale, 1.0, 0.0)
            tbl[r0:r0 + 128, :] = jnp.broadcast_to(row, (128, 128)).T

        return [first] + [functools.partial(tile, j) for j in range((hi - lo) // 128)]

    with scope("wait_wm0"):
        cp_wm0.wait()
    with scope("mod0"):
        for it in mod_items(512, 1152):
            it()

    ones = jnp.ones((16, D), bf16)
    rsq = lambda v: jax.lax.rsqrt(v + EPS)

    def finish(k, fn):
        for t in range(NT):
            stat[k, t] = jnp.broadcast_to(fn(jnp.sum(stat[k, t], axis=0, keepdims=True) * (1.0 / D)), (8, 128))

    def b_mean(t):
        ln = pl.ds(pl.multiple_of(t * 128, 128), 128)
        xs = [xT[8 * r:8 * r + 8, ln].astype(f32) for r in range(D // 8)]
        mnb[t] = jnp.broadcast_to(_colsum(xs, 3) * (1.0 / D), (8, 128))

    def radix9_store(t, load):
        for j in range(8):
            y0, ys = _radix9_fwd([load(8 * n9 + j) for n9 in range(9)])
            ybuf[t, 4, 8 * j:8 * j + 8, :] = _pack(y0, jnp.zeros_like(y0))
            for g in range(4):
                ybuf[t, g, 8 * j:8 * j + 8, :] = _pack(*ys[g])

    def b_vpu(t):
        ln = pl.ds(pl.multiple_of(t * 128, 128), 128)
        mean = mnb[t]
        accs = [None] * 3

        def load(r):
            xc = xT[8 * r:8 * r + 8, ln].astype(f32) - mean
            k = (r // 8) % 3
            accs[k] = xc * xc if accs[k] is None else accs[k] + xc * xc
            return xc * tbl[D + 8 * r:D + 8 * r + 8, :]

        radix9_store(t, load)
        stat[0, t] = _tree(accs)

    def b_loop(t, _):
        @pl.when(((t + 1) % (NT // XC) == 0) & (t + 1 < NT))
        def _():
            pltpu.make_async_copy(xT_h.at[:, 0:xw], xT.at[:, 0:xw], sem.at[xsem + (t + 1) // (NT // XC)]).wait()

        b_vpu(t)
        b_mean(jnp.minimum(t + 1, NT - 1))

    with scope("wait_x"):
        cp_x[0].wait()
    with scope("B"):
        b_mean(0)
        jax.lax.fori_loop(0, NT, b_loop, None)
        finish(0, rsq)
    for d in cp_w1:
        d.start()

    def d_fwd(g, t):
        rows = 128 if g < 4 else NR - 512
        return _dot(dm[(g + 1) % 5, 0:rows, :], pltpu.bitcast(ybuf[t, g], bf16))

    def b_mxu(g, t):
        r = d_fwd(g, t)
        xbuf[t, 128 * g:128 * g + r.shape[0], :] = r

    def phase_c(q):
        r0 = q * 16
        y = _radix16([(xbuf[t, r0:r0 + 8, :] * stat[0, t], xbuf[t, r0 + 8:r0 + 16, :] * stat[0, t])
                      for t in range(NT)], -1)
        for b in range(NT):
            cbuf[b, r0:r0 + 16, :] = jnp.concatenate(y[b], axis=0).astype(bf16)

    P = functools.partial
    qs = lambda g: range(8 * g, min(8 * g + 8, NQ))

    def region(fn):
        jax.lax.fori_loop(0, one, lambda i, _: fn(), None)

    one = zsm[0]
    cp_dm.wait()
    with scope("C"):
        region(lambda: _interleave([P(b_mxu, 0, t) for t in range(NT)]))
        for g in range(1, 5):
            region(lambda: _interleave([P(b_mxu, g, t) for t in range(NT)], [P(phase_c, q) for q in qs(g - 1)]))
        region(lambda: _interleave([P(phase_c, q) for q in qs(4)]))

    def sa_items():
        def last():
            for g in range(5):
                r = d_fwd(g, NT)
                sab[128 * g:128 * g + r.shape[0], :] = r * float(S)
        return mod_items(0, 512) + [lambda: radix9_store(NT, lambda r: tbl[8 * r:8 * r + 8, :]), last]

    lane = jax.lax.broadcasted_iota(jnp.int32, (8, 128), 1)
    masks = [(lane & (1 << b)) != 0 for b in range(4)]

    def shuffle(vals):
        vals = [pltpu.roll(v, a, 1) if a else v for a, v in enumerate(vals)]
        vals = [vals[(-b) % 16] for b in range(16)]
        for b in range(4):
            vals = [jnp.where(masks[b], vals[(i - (1 << b)) % 16], vals[i]) for i in range(16)]
        return vals

    def w_rows(p, raw, r):
        if r < 18:
            vals = shuffle([pltpu.bitcast(raw[16 * r:16 * r + 16, a * 128:(a + 1) * 128], u32) for a in range(16)])
        else:
            last = jnp.broadcast_to(raw[288:289, :].astype(f32), (8, S))
            vals = shuffle([pltpu.bitcast(last[:, a * 128:(a + 1) * 128], u32) for a in range(16)])
        for b in range(16):
            wp[p, b, 8 * r:8 * r + 8, :] = vals[b]

    def phase_d1(b):
        pp = _dot(cbuf[b], jnp.concatenate([sm[b, 0], sm[b, 1]], axis=1))
        for q in range(NQ):
            re, im = pp[16 * q:16 * q + 8], pp[16 * q + 8:16 * q + 16]
            xbuf[b, 16 * q:16 * q + 8, :] = re[:, :128] - im[:, 128:]
            xbuf[b, 16 * q + 8:16 * q + 16, :] = re[:, 128:] + im[:, :128]

    def w_group(p, b, grp):
        _, c0, mh = grp
        if c0 == 288:
            return pltpu.bitcast(wp[p, b, 144:152, :], f32)
        return _unpack(wp[p, b, pl.ds(c0 // 2 + 72 * mh, 8, stride=9), :], c0 % 2)

    def phase_d2(b):
        zs = []
        for q in range(NQ):
            xr, xi = xbuf[b, 16 * q:16 * q + 8, :], xbuf[b, 16 * q + 8:16 * q + 16, :]
            if b == 0:
                xr = xr + jnp.where(lane == 0, sab[16 * q:16 * q + 8, :], 0.0)
                xi = xi + jnp.where(lane == 0, sab[16 * q + 8:16 * q + 16, :], 0.0)
            wr, wi = w_group(0, b, _GROUPS[q]), w_group(1, b, _GROUPS[q])
            zs += [xr * wr - xi * wi, xr * wi + xi * wr]
        z = jnp.concatenate(zs, axis=0).astype(bf16)
        qq = _dot_t(z, jnp.concatenate([sm[b, 0], sm[b, 1]], axis=0))
        for q in range(NQ):
            re, im = qq[16 * q:16 * q + 8], qq[16 * q + 8:16 * q + 16]
            zbuf[b, 16 * q:16 * q + 8, :] = re[:, :128] + im[:, 128:]
            zbuf[b, 16 * q + 8:16 * q + 16, :] = im[:, :128] - re[:, 128:]

    with scope("wait_sm"):
        cp_sm.wait()
    with scope("D1a"):
        region(lambda: _interleave([P(phase_d1, b) for b in range(DS1)]))
    with scope("wait_w"):
        cp_wms.wait()
        cp_wr.wait()
        cp_wi.wait()
    with scope("D1b"):
        region(lambda: _interleave([P(phase_d1, b) for b in range(DS1, NT)],
                                   [P(w_rows, p, raw, r) for p, raw in enumerate((wraw_r, wraw_i)) for r in range(19)],
                                   sa_items()))
    with scope("D2a"):
        region(lambda: _interleave([P(phase_d2, b) for b in range(DS2)]))
    with scope("wait_wm1"):
        cp_wm1.wait()
        for d in cp_w2:
            d.start()
    with scope("D2b"):
        region(lambda: _interleave([P(phase_d2, b) for b in range(DS2, NT)], mod_items(1152, 6 * D)))

    def phase_e(q):
        r0 = q * 16
        y = _radix16([(zbuf[b, r0:r0 + 8, :], zbuf[b, r0 + 8:r0 + 16, :]) for b in range(NT)], 1)
        for t in range(NT):
            ybuf[t, q // 8, (q % 8) * 8:(q % 8) * 8 + 8, :] = _pack(*y[t])

    def f_mxu(g, t):
        if g < 4:
            xbuf[t, 128 * g:128 * (g + 1), :] = _dot(dm[6 + g], pltpu.bitcast(ybuf[t, g], bf16))
        else:
            xbuf[t, 512:576, :] = _dot(dm[5, 0:64, 0:80], pltpu.bitcast(ybuf[t, 4, 0:40, :], bf16))

    def center_sb():
        sb = [tbl[3 * D + 8 * r:3 * D + 8 * r + 8, :] for r in range(D // 8)]
        sbm = _colsum(sb) * (1.0 / D)
        for r in range(D // 8):
            sab[8 * r:8 * r + 8, :] = sb[r] - sbm

    with scope("E"):
        region(lambda: _interleave([P(phase_e, q) for q in qs(4)]))
        for g in range(4):
            region(lambda: _interleave([P(f_mxu, (g - 1) % 5, t) for t in range(NT)], [P(phase_e, q) for q in qs(g)]))
        region(lambda: _interleave([P(f_mxu, 3, t) for t in range(NT)], [center_sb]))

    def f_p1(t, _):
        ln = pl.ds(pl.multiple_of(t * 128, 128), 128)
        accs = [None] * 3
        for j in range(8):
            v = [(xbuf[t, 128 * g + 8 * j:128 * g + 8 * j + 8, :],
                  xbuf[t, 128 * g + 64 + 8 * j:128 * g + 72 + 8 * j, :]) for g in range(4)]
            ys = _radix9_inv(xbuf[t, 512 + 8 * j:520 + 8 * j, :], v)
            for n9 in range(9):
                r = 8 * n9 + j
                xv = xT[8 * r:8 * r + 8, ln].astype(f32) + ys[n9] * tbl[2 * D + 8 * r:2 * D + 8 * r + 8, :]
                x1[t, 8 * r:8 * r + 8, :] = xv
                accs[n9 % 3] = xv if accs[n9 % 3] is None else accs[n9 % 3] + xv
        stat[0, t] = _tree(accs)

    def f_p2(t, _):
        mean = stat[0, t]
        a2 = [None] * 2
        az = [None] * 2
        for r in range(D // 8):
            xc = x1[t, 8 * r:8 * r + 8, :] - mean
            z = xc * tbl[4 * D + 8 * r:4 * D + 8 * r + 8, :]
            xbuf[t, 8 * r:8 * r + 8, :] = z
            k = r % 2
            a2[k] = xc * xc if a2[k] is None else a2[k] + xc * xc
            az[k] = z if az[k] is None else az[k] + z
        stat[1, t] = _tree(a2)
        stat[2, t] = _tree(az)

    def f_p3(t, _):
        rs = stat[1, t]
        mz = stat[2, t]
        a2 = [None] * 2
        for r in range(D // 8):
            dv = (xbuf[t, 8 * r:8 * r + 8, :] - mz) * rs + sab[8 * r:8 * r + 8, :]
            zbuf[t, pl.ds(16 * (r // 2) + r % 2, 8, stride=2), :] = dv
            k = r % 2
            a2[k] = dv * dv if a2[k] is None else a2[k] + dv * dv
        stat[3, t] = _tree(a2)

    def f_p4(k, _):
        rs = [stat[3, 4 * k + c] for c in range(4)]
        for r0 in range(0, H, 16):
            ops = [_sa2([[zbuf[4 * k + c, r * H + r0 + 8 * h:r * H + r0 + 8 * h + 8, :] * rs[c] for c in range(4)]
                         for r in range(4)]) for h in range(2)]
            for j in range(49):
                aop[j, k, r0 // 2:r0 // 2 + 8, :] = _pack(ops[0][j], ops[1][j])

    with scope("F1"):
        jax.lax.fori_loop(0, NT, f_p1, None)
        finish(0, lambda v: v)
    with scope("F2"):
        jax.lax.fori_loop(0, NT, f_p2, None)
        finish(1, rsq)
        finish(2, lambda v: v)
    with scope("F3"):
        jax.lax.fori_loop(0, NT, f_p3, None)
        finish(3, rsq)
    with scope("F4"):
        jax.lax.fori_loop(0, NT // 4, f_p4, None)

    cp_b1.wait()
    cp_b2.wait()
    tbl[0:40, :] = jnp.concatenate([b1v[...].astype(f32), jnp.zeros((4, 128), f32)], axis=0)
    tbl[40:56, :] = b2v[...].astype(f32) * 2.0

    def bias(r):
        return jnp.broadcast_to(tbl[pl.ds(r, 1), :], (8, 128))

    def mlp1(i, _):
        for c in range(4):
            strip(w1_h, w1v, w1sem, 4 * i + c).wait()
        m = _strassen2(
            lambda j: jnp.concatenate([pltpu.bitcast(aop[j, k], bf16) for k in range(4)], axis=1),
            lambda o, r, c: jnp.concatenate(
                [w1v[4 * i + c + zsm[1 + o], 64 * (4 * k + r):64 * (4 * k + r + 1), :] for k in range(4)], axis=0))
        bs = [bias(4 * i + c) for c in range(4)]
        for r0 in range(0, H, 16):
            ops = []
            for h in range(2):
                u = _sc2([x[r0 + 8 * h:r0 + 8 * h + 8] for x in m])
                ops.append(_sa2([[_gelu2(u[r][c] + bs[c]) for c in range(4)] for r in range(4)]))
            for j in range(49):
                gop[j, i, r0 // 2:r0 // 2 + 8, :] = _pack(ops[0][j], ops[1][j])

    with scope("mlp1"):
        jax.lax.fori_loop(0, NF, mlp1, None, unroll=u1)

    def out_copy(t):
        cols = pl.ds(pl.multiple_of(t * 128, 128), 128)
        return pltpu.make_async_copy(obuf.bitcast(bf16).at[t], out_h.at[:, cols], osem.at[t])

    def mlp2(i, _):
        for c in range(4):
            strip(w2_h, w2v, w2sem, 4 * i + c).wait()
        m = _strassen2(
            lambda j: jnp.concatenate([pltpu.bitcast(gop[j, k], bf16) for k in range(NF)], axis=1),
            lambda o, r, c: jnp.concatenate(
                [w2v[4 * i + c + zsm[1 + o], 64 * (4 * k + r):64 * (4 * k + r + 1), :] for k in range(NF)], axis=0))
        bs = [bias(40 + 4 * i + c) for c in range(4)]
        for r0 in range(0, H, 16):
            y = [_sc2([x[r0 + 8 * h:r0 + 8 * h + 8] for x in m]) for h in range(2)]
            for r in range(4):
                row = r * H + r0
                gb = [tbl[pl.ds(5 * D + row + h, 8, stride=2), :] for h in range(2)]
                for c in range(4):
                    o = [x1[4 * i + c, pl.ds(row + h, 8, stride=2), :] + gb[h] * (y[h][r][c] + bs[c])
                         for h in range(2)]
                    obuf[4 * i + c, row // 2:row // 2 + 8, :] = _pack(o[0], o[1])
        for c in range(4):
            out_copy(4 * i + c).start()

    with scope("mlp2"):
        jax.lax.fori_loop(0, NS, mlp2, None)
    for t in range(NT):
        out_copy(t).wait()


@jax.jit
def pallas_adaLN_cond__spectral_gfnet__mixer_token_mlp__prompt_kernel(
    A_x: jax.Array,
    A_w_r: jax.Array,
    A_w_i: jax.Array,
    B_x: jax.Array,
    B_w1: jax.Array,
    B_b1: jax.Array,
    B_w2: jax.Array,
    B_b2: jax.Array,
    c: jax.Array,
    w_mod: jax.Array,
):
    del B_x
    any_spec = pl.BlockSpec(memory_space=pl.ANY)
    scratch = [
        pltpu.VMEM((D, S), bf16),
        pltpu.VMEM((289, S), bf16),
        pltpu.VMEM((289, S), bf16),
        pltpu.VMEM((2, NT, 152, 128), u32),
        pltpu.VMEM((F // 128, S // 2, 128), u32),
        pltpu.VMEM((NT, F // 2, 128), u32),
        pltpu.VMEM((F // 128, 128), bf16),
        pltpu.VMEM((S // 128, 128), bf16),
        pltpu.VMEM((1, D), bf16),
        pltpu.VMEM((D, 6 * D), bf16),
        pltpu.VMEM((10, 128, 128), bf16),
        pltpu.VMEM((NT, 2, 128, 128), bf16),
        pltpu.VMEM((6 * D, 128), f32),
        pltpu.VMEM((NT + 1, 5, 64, 128), u32),
        pltpu.VMEM((NT, NR, 128), f32),
        pltpu.VMEM((NT, NR, 128), bf16),
        pltpu.VMEM((NR, 128), f32),
        pltpu.VMEM((NT, 8, 128), f32),
        pltpu.VMEM((4, NT, 8, 128), f32),
        pltpu.VMEM((NT, NR, 128), f32),
        pltpu.VMEM((NT, D, 128), f32),
        pltpu.VMEM((49, 4, H // 2, 128), u32),
        pltpu.VMEM((49, NF, H // 2, 128), u32),
        pltpu.VMEM((NT, D // 2, 128), u32),
        pltpu.SemaphoreType.DMA((16,)),
        pltpu.SemaphoreType.DMA((F // 128,)),
        pltpu.SemaphoreType.DMA((NT,)),
        pltpu.SemaphoreType.DMA((NT,)),
    ]
    outT = pl.pallas_call(
        functools.partial(_kernel, scopes=False, u1=1),
        out_shape=jax.ShapeDtypeStruct((D, S), bf16),
        in_specs=[pl.BlockSpec(memory_space=pltpu.SMEM)] + [any_spec] * 11,
        out_specs=any_spec,
        scratch_shapes=scratch,
        compiler_params=pltpu.CompilerParams(vmem_limit_bytes=120 * 1024 * 1024),
        name="adaln_gfnet_mixer",
    )(np.array([1, 0, 0, 0, 0, 0, 0, 0], np.int32), A_x[0].T, A_w_r.T, A_w_i.T, B_w1, B_b1.reshape(F // 128, 128), B_w2,
      B_b2.reshape(S // 128, 128), c, w_mod, _DMAT, _SMAT)
    return outT.T[None]
```

```python
import contextlib
import functools

import jax
import jax.numpy as jnp
import numpy as np
import ml_dtypes
import jax.experimental.pallas as pl
import jax.experimental.pallas.tpu as pltpu

S, D, F = 2048, 576, 4608
NT = S // 128
NP = 19
NR = NP * 16
H = D // 4
f32, bf16, u32 = jnp.float32, jnp.bfloat16, jnp.uint32
EPS = 1e-5

_TH = 2 * np.pi / 9
C1, C2, C4 = float(np.cos(_TH)), float(np.cos(2 * _TH)), float(np.cos(4 * _TH))
S1, S3, S4 = float(np.sin(_TH)), float(np.sin(3 * _TH)), float(np.sin(4 * _TH))


_SETS = [[g, g + 9, 9 - g, 18 - g] for g in range(1, 5)] + [[0, 9, 288]]
_FLAT = [c for grp in _SETS for c in grp]


def _d_mats():
    d2 = np.arange(64)
    fwd = np.zeros((5, 128, 128))
    inv = np.zeros((5, 128, 128))
    col = 16 * (d2 // 8) + 2 * (d2 % 8)
    for g, grp in enumerate(_SETS):
        res = (g + 1) % 5
        scale = (0.0, S1, S1, S3, S1)[res]
        for cc, c0 in enumerate(grp):
            for m in range(1 if c0 == 288 else 16):
                kx = c0 + 18 * m
                ph = 2 * np.pi * ((kx * d2) % D) / D
                c, s = np.cos(ph), np.sin(ph)
                if kx % 288 == 0:
                    s = np.zeros_like(s)
                sg = (1.0 if kx % 9 == res else -1.0) * scale
                row = 32 * cc + 16 * (m % 2) + m // 2
                fwd[g, row, col] = c
                fwd[g, row + 8, col] = -s
                fwd[g, row, col + 1] = -sg * s
                fwd[g, row + 8, col + 1] = -sg * c
                w = (1.0 if kx % 288 == 0 else 2.0) / (S * D)
                k = 32 * cc + 2 * (2 * (m % 8) + m // 8)
                inv[g, d2, k] = w * c
                inv[g, d2, k + 1] = -w * s
                inv[g, 64 + d2, k] = sg * w * s
                inv[g, 64 + d2, k + 1] = sg * w * c
    return fwd.astype(ml_dtypes.bfloat16), inv.astype(ml_dtypes.bfloat16)


def _s_mats():
    m = np.zeros((NT, 3, 128, 128))
    lane = np.arange(128)
    for b in range(NT):
        a = (lane - b) % 16
        k = 128 * a + (lane - a) % 128
        ph = 2 * np.pi * ((lane[:, None] * k[None, :]) % S) / S
        re, im = np.cos(ph), -np.sin(ph)
        m[b] = re, im - re, re + im
    return m.astype(ml_dtypes.bfloat16)


_DFWD, _DINV = _d_mats()
_SMAT = _s_mats()


def _dot(a, b):
    return jnp.dot(a, b, preferred_element_type=f32)


def _dot_t(a, b):
    return jax.lax.dot_general(a, b, (((1,), (1,)), ((), ())), preferred_element_type=f32)


def _pack(a, b):
    return pltpu.pack_elementwise([a, b], packed_dtype=bf16)


def _unpack(x, i):
    return pltpu.unpack_elementwise(x, index=i, packed_dtype=bf16, unpacked_dtype=f32)


def _radix9_fwd(a):
    p = [None] + [a[n] + a[9 - n] for n in range(1, 5)]
    m = [None] + [a[n] - a[9 - n] for n in range(1, 5)]
    t = p[1] + p[2] + p[4]
    u = a[0] + p[3]
    b = a[0] - 0.5 * p[3]
    e1 = p[1] - p[4]
    e2 = p[2] - p[4]
    r1 = C1 * e1 + C2 * e2
    r2 = C2 * e1 + C4 * e2
    f1 = m[1] + m[2]
    f2 = m[2] + m[4]
    f3 = m[1] - m[4]
    q1 = f1 + (S4 / S1) * f2
    q2 = f3 + (S4 / S1) * f1
    n3 = (S3 / S1) * m[3]
    return u + t, [(b + r1, q1 + n3), (b + r2, q2 - n3), (u - 0.5 * t, m[1] - m[2] + m[4]),
                   (b - (r1 + r2), (q2 - q1) + n3)]


def _radix9_inv(v0, v):
    (r1_, i1), (r2_, i2), (r3_, i3), (r4_, i4) = v
    t = r1_ + r2_ + r4_
    u = v0 + r3_
    b = v0 - 0.5 * r3_
    e1 = r1_ - r4_
    e2 = r2_ - r4_
    r1 = C1 * e1 + C2 * e2
    r2 = C2 * e1 + C4 * e2
    a1, a2, a3, a4 = b + r1, b + r2, u - 0.5 * t, b - (r1 + r2)
    f1 = i1 + i2
    f2 = i2 + i4
    f3 = i1 - i4
    q1 = f1 + (S4 / S1) * f2
    q2 = f3 + (S4 / S1) * f1
    b1, b2, b4 = q1 + i3, q2 - i3, (q2 - q1) + i3
    b3 = (S3 / S1) * (i1 - i2 + i4)
    return [u + t, a1 - b1, a2 - b2, a3 - b3, a4 - b4, a4 + b4, a3 + b3, a2 + b2, a1 + b1]


def _bfly4(a, b, c, d, sgn, c_rot=False):
    if c_rot:
        if sgn < 0:
            t0 = (a[0] + c[1], a[1] - c[0])
            t1 = (a[0] - c[1], a[1] + c[0])
        else:
            t0 = (a[0] - c[1], a[1] + c[0])
            t1 = (a[0] + c[1], a[1] - c[0])
    else:
        t0 = (a[0] + c[0], a[1] + c[1])
        t1 = (a[0] - c[0], a[1] - c[1])
    t2 = (b[0] + d[0], b[1] + d[1])
    t3 = (b[0] - d[0], b[1] - d[1])
    x0 = (t0[0] + t2[0], t0[1] + t2[1])
    x2 = (t0[0] - t2[0], t0[1] - t2[1])
    xm = (t1[0] + t3[1], t1[1] - t3[0])
    xp = (t1[0] - t3[1], t1[1] + t3[0])
    return [x0, xm, x2, xp] if sgn < 0 else [x0, xp, x2, xm]


def _tw16(z, e, sgn):
    c = float(np.cos(2 * np.pi * e / 16))
    s = float(sgn * np.sin(2 * np.pi * e / 16))
    x, y = z
    if e % 2 == 0:
        if (c > 0) == (s > 0):
            return ((x - y) * c, (x + y) * c)
        return ((x + y) * c, (y - x) * c)
    return (x * c - y * s, x * s + y * c)


def _radix16(x, sgn):
    u = [_bfly4(x[n2], x[4 + n2], x[8 + n2], x[12 + n2], sgn) for n2 in range(4)]
    out = [None] * 16
    for k1 in range(4):
        v = []
        for n2 in range(4):
            e = k1 * n2
            v.append(u[n2][k1] if e % 4 == 0 else _tw16(u[n2][k1], e, sgn))
        y = _bfly4(v[0], v[1], v[2], v[3], sgn, c_rot=(k1 == 2))
        for k2 in range(4):
            out[k1 + 4 * k2] = y[k2]
    return out


def _sa(a11, a12, a21, a22):
    return [a11 + a22, a21 + a22, a11, a22, a11 + a12, a21 - a11, a12 - a22]


def _sb(b11, b12, b21, b22):
    return [b11 + b22, b11, b12 - b22, b21 - b11, b22, b11 + b12, b21 + b22]


def _sc(m):
    m1, m2, m3, m4, m5, m6, m7 = m
    return [m4 + m7 - m5 + m1, m5 + m3, m2 + m4, m1 - m2 + m3 + m6]


def _sa2(blk):
    lvl = [_sa(blk[ri][ci], blk[ri][2 + ci], blk[2 + ri][ci], blk[2 + ri][2 + ci])
           for ri in range(2) for ci in range(2)]
    return [x for o in range(7) for x in _sa(*[l[o] for l in lvl])]


def _sc2(m):
    p = [_sc(m[7 * o:7 * o + 7]) for o in range(7)]
    out = [[None] * 4 for _ in range(4)]
    for ii in range(4):
        for oi, v in enumerate(_sc([p[o][ii] for o in range(7)])):
            out[2 * (oi // 2) + ii // 2][2 * (oi % 2) + ii % 2] = v
    return out


_SB_TERMS = (((1, 0, 0), (1, 1, 1)), ((1, 0, 0),), ((1, 0, 1), (-1, 1, 1)), ((1, 1, 0), (-1, 0, 0)),
             ((1, 1, 1),), ((1, 0, 0), (1, 0, 1)), ((1, 1, 0), (1, 1, 1)))
_ORDER = (1, 3, 6, 4, 0, 2, 5)


def _strassen2(lhs, raw, hook=None):
    m = [None] * 49
    done = 0
    for o in _ORDER:
        blocks = {}
        halves = []
        for h in range(2):
            quad = []
            for ri in range(2):
                for ci in range(2):
                    acc = None
                    for sg, ro, co in _SB_TERMS[o]:
                        key = (2 * ro + ri, 2 * co + ci)
                        if key not in blocks:
                            blocks[key] = raw(o, *key)
                        v = _unpack(blocks[key], h)
                        acc = v if acc is None else (acc + v if sg > 0 else acc - v)
                    quad.append(acc)
            halves.append(_sb(*quad))
        for j in _ORDER:
            if hook is not None:
                hook(done)
            done += 1
            rhs = pltpu.bitcast(_pack(halves[0][j], halves[1][j]), bf16)
            m[7 * o + j] = _dot(lhs(7 * o + j), rhs)
    return m


def _gelu2(u):
    k0 = 0.7978845608028654
    z = u * (k0 + (k0 * 0.044715) * (u * u))
    return u * jnp.tanh(z) + u


def _tree(vs):
    vs = list(vs)
    while len(vs) > 1:
        vs = [vs[i] + vs[i + 1] if i + 1 < len(vs) else vs[i] for i in range(0, len(vs), 2)]
    return vs[0]


def _colsum(vs, lanes=4):
    accs = []
    for k in range(lanes):
        acc = None
        for v in vs[k::lanes]:
            acc = v if acc is None else acc + v
        accs.append(acc)
    return jnp.sum(_tree(accs), axis=0, keepdims=True)


def _interleave(*lists):
    items = []
    for ci, lst in enumerate(lists):
        for k, it in enumerate(lst):
            items.append(((k + 0.5) / len(lst), ci, k, it))
    items.sort(key=lambda x: x[:3])
    for x in items:
        x[3]()


FC = 512
NF = F // FC
SC = 512
NS = S // SC
XC = 8
WSPLIT = (0, 96, 192, 289)


def _kernel(z_h, xT_h, wr_h, wi_h, w1_h, b1_h, w2_h, b2_h, c_h, wm_h, df_h, di_h, sm_h, out_h,
            xT, wraw_r, wraw_i, wp, w1v, w2v, b1v, b2v, cv, wm, df, di, sm, tbl, ybuf, xbuf, cbuf, sab,
            mnb, stat, zbuf, x1, aop, gop, obuf, zsm, sem, w1sem, w2sem, osem, *, scopes, opt):
    n = [0]

    def scope(name):
        return jax.named_scope(name) if scopes else contextlib.nullcontext()

    def cp(src, dst):
        d = pltpu.make_async_copy(src, dst, sem.at[n[0]])
        n[0] += 1
        return d

    xw = S // XC
    cp_c = cp(c_h, cv)
    cp_wm0 = cp(wm_h.at[:, 512:1152], wm.at[:, 512:1152])
    cp_x = [cp(xT_h.at[:, i * xw:(i + 1) * xw], xT.at[:, i * xw:(i + 1) * xw]) for i in range(XC)]
    cp_z = cp(z_h, zsm)
    cp_df = cp(df_h, df)
    cp_sm = cp(sm_h, sm)
    cp_w = [[cp(src.at[lo:hi], dst.at[lo:hi]) for src, dst in ((wr_h, wraw_r), (wi_h, wraw_i))]
            for lo, hi in zip(WSPLIT[:-1], WSPLIT[1:])]
    cp_wms = cp(wm_h.at[:, 0:512], wm.at[:, 0:512])
    cp_di = cp(di_h, di)
    cp_wm1 = cp(wm_h.at[:, 1152:2944], wm.at[:, 1152:2944])
    cp_wm2 = cp(wm_h.at[:, 2944:6 * D], wm.at[:, 2944:6 * D])
    cp_b1 = cp(b1_h, b1v)
    cp_b2 = cp(b2_h, b2v)

    def strip(src, dst, sems, j):
        cols = pl.ds(pl.multiple_of(j * 128, 128), 128)
        return pltpu.make_async_copy(src.at[:, cols], dst.bitcast(bf16).at[j], sems.at[j // 4])

    cp_w1 = [strip(w1_h, w1v, w1sem, j) for j in range(F // 128)]
    cp_w2 = [strip(w2_h, w2v, w2sem, j) for j in range(NT)]

    for d in [cp_c, cp_wm0, *cp_x, cp_z, cp_df, cp_sm, *sum(cp_w, []), cp_wms, cp_di, cp_wm1, cp_b1, cp_b2]:
        d.start()

    cp_c.wait()
    cc = cv[...].astype(f32)
    sc = jnp.broadcast_to(cc * jax.nn.sigmoid(cc), (16, D)).astype(bf16)

    def mod_items(lo, hi):
        box = []

        def first():
            box.append(_dot(sc, wm[:, lo:hi]))

        def tile(j):
            r0 = lo + j * 128
            row = box[0][0:1, j * 128:(j + 1) * 128]
            col = r0 + jax.lax.broadcasted_iota(jnp.int32, (1, 128), 1)
            is_scale = ((col >= D) & (col < 2 * D)) | ((col >= 4 * D) & (col < 5 * D))
            row = row * jnp.where(col >= 5 * D, 0.5, 1.0) + jnp.where(is_scale, 1.0, 0.0)
            tbl[r0:r0 + 128, :] = jnp.broadcast_to(row, (128, 128)).T

        return [first] + [functools.partial(tile, j) for j in range((hi - lo) // 128)]

    with scope("wait_wm0"):
        cp_wm0.wait()
    with scope("mod0"):
        for it in mod_items(512, 1152):
            it()

    ones = jnp.ones((16, D), bf16)
    rsq = lambda v: jax.lax.rsqrt(v + EPS)

    def finish(k, fn):
        for t in range(NT):
            stat[k, t] = jnp.broadcast_to(fn(jnp.sum(stat[k, t], axis=0, keepdims=True) * (1.0 / D)), (8, 128))

    def b_mean(t):
        ln = pl.ds(pl.multiple_of(t * 128, 128), 128)
        xs = [xT[8 * r:8 * r + 8, ln].astype(f32) for r in range(D // 8)]
        mnb[t] = jnp.broadcast_to(_colsum(xs, 3) * (1.0 / D), (8, 128))

    def radix9_store(t, load):
        for j in range(8):
            y0, ys = _radix9_fwd([load(8 * n9 + j) for n9 in range(9)])
            ybuf[t, 4, 8 * j:8 * j + 8, :] = _pack(y0, jnp.zeros_like(y0))
            for g in range(4):
                ybuf[t, g, 8 * j:8 * j + 8, :] = _pack(*ys[g])

    def b_vpu(t):
        ln = pl.ds(pl.multiple_of(t * 128, 128), 128)
        mean = mnb[t]
        accs = [None] * 3

        def load(r):
            xc = xT[8 * r:8 * r + 8, ln].astype(f32) - mean
            k = (r // 8) % 3
            accs[k] = xc * xc if accs[k] is None else accs[k] + xc * xc
            return xc * tbl[D + 8 * r:D + 8 * r + 8, :]

        radix9_store(t, load)
        stat[0, t] = _tree(accs)

    def b_pair(tp, _):
        b_vpu(2 * tp)
        b_vpu(2 * tp + 1)

    for i in range(XC):
        with scope("wait_x"):
            cp_x[i].wait()
        with scope("B"):
            for t in range(i * (NT // XC), (i + 1) * (NT // XC)):
                b_mean(t)
            b_pair(i, None)
    finish(0, rsq)
    for d in cp_w1:
        d.start()

    def d_fwd(g, t):
        rows = 128 if g < 4 else 80
        return _dot(df[g, 0:rows, :], pltpu.bitcast(ybuf[t, g], bf16))

    def phase_c():
        for g, grp in enumerate(_SETS):
            xs = [d_fwd(g, t) for t in range(NT)]
            for cc, c0 in enumerate(grp):
                y = []
                for r0 in (32 * cc,) if c0 == 288 else (32 * cc, 32 * cc + 16):
                    y.append(_radix16([(xs[t][r0:r0 + 8] * stat[0, t], xs[t][r0 + 8:r0 + 16] * stat[0, t])
                                       for t in range(NT)], -1))
                rows = slice(8 * (4 * g + cc), 8 * (4 * g + cc) + 8)
                for b in range(NT):
                    (er, ei), (odr, odi) = y[0][b], y[-1][b]
                    cbuf[b, 0, rows, :] = _pack(er + ei, odr + odi)
                    cbuf[b, 1, rows, :] = _pack(er, odr)
                    cbuf[b, 2, rows, :] = _pack(ei, odi)

    def b_mxu(g, t):
        r = d_fwd(g, t)
        xbuf[t + zsm[1], 128 * g:128 * g + r.shape[0], :] = r

    def c_pair(g, cc):
        base = 128 * g + 32 * cc
        y = [_radix16([(xbuf[t, r0:r0 + 8, :] * stat[0, t], xbuf[t, r0 + 8:r0 + 16, :] * stat[0, t])
                       for t in range(NT)], -1)
             for r0 in ((base,) if _SETS[g][cc] == 288 else (base, base + 16))]
        rows = slice(8 * (4 * g + cc), 8 * (4 * g + cc) + 8)
        for b in range(NT):
            (er, ei), (odr, odi) = y[0][b], y[-1][b]
            cbuf[b, 0, rows, :] = _pack(er + ei, odr + odi)
            cbuf[b, 1, rows, :] = _pack(er, odr)
            cbuf[b, 2, rows, :] = _pack(ei, odi)

    def phase_c2():
        order = (4, 0, 1, 2, 3)
        _interleave([P(b_mxu, order[0], t) for t in range(NT)])
        for prev, g in zip(order[:-1], order[1:]):
            _interleave([P(b_mxu, g, t) for t in range(NT)], [P(c_pair, prev, cc) for cc in range(len(_SETS[prev]))])
        _interleave([P(c_pair, order[-1], cc) for cc in range(4)])

    P = functools.partial
    qs = lambda g: range(8 * g, min(8 * g + 8, 2 * NP - 1))

    def region(fn):
        jax.lax.fori_loop(0, one, lambda i, _: fn(), None)

    cp_z.wait()
    one = zsm[0]
    cp_df.wait()
    with scope("C"):
        region(phase_c2 if opt.get('c2', 0) else phase_c)

    def sa_items():
        def last():
            for g, grp in enumerate(_SETS):
                r = d_fwd(g, NT) * float(S)
                for cc, c0 in enumerate(grp):
                    for par in range(2):
                        r0 = 32 * cc + (0 if c0 == 288 else 16 * par)
                        for ri in range(2):
                            sab[pl.ds(ri * NR + 16 * (4 * g + cc) + par, 8, stride=2), :] = r[r0 + 8 * ri:r0 + 8 * ri + 8]
        return mod_items(0, 512) + [lambda: radix9_store(NT, lambda r: tbl[8 * r:8 * r + 8, :]), last]

    lane = jax.lax.broadcasted_iota(jnp.int32, (8, 128), 1)
    masks = [(lane & (1 << b)) != 0 for b in range(4)]

    def shuffle(vals):
        vals = [pltpu.roll(v, a, 1) if a else v for a, v in enumerate(vals)]
        vals = [vals[(-b) % 16] for b in range(16)]
        for b in range(4):
            vals = [jnp.where(masks[b], vals[(i - (1 << b)) % 16], vals[i]) for i in range(16)]
        return vals

    def w_rows(p, raw, r):
        if r < 18:
            vals = shuffle([pltpu.bitcast(raw[16 * r:16 * r + 16, a * 128:(a + 1) * 128], u32) for a in range(16)])
        else:
            last = jnp.broadcast_to(raw[288:289, :].astype(f32), (8, S))
            vals = shuffle([pltpu.bitcast(last[:, a * 128:(a + 1) * 128], u32) for a in range(16)])
        for b in range(16):
            wp[p, b, 8 * r:8 * r + 8, :] = vals[b]

    def phase_d1(b):
        k = [_dot(pltpu.bitcast(cbuf[b, p], bf16), sm[b, p]) for p in range(3)]
        xbuf[b, 0:NR, :] = k[0] - k[2]
        xbuf[b, NR:2 * NR, :] = k[0] + k[1]

    def w_group(p, b, c0, mh):
        if c0 == 288:
            return pltpu.bitcast(wp[p, b, 144:152, :], f32)
        return _unpack(wp[p, b, pl.ds(c0 // 2 + 72 * mh, 8, stride=9), :], c0 % 2)

    def phase_d2(b):
        zs = [[], [], []]
        for p, c0 in enumerate(_FLAT):
            z = []
            for mh in range(1 if c0 == 288 else 2):
                r0 = 16 * p + 8 * mh
                xr, xi = xbuf[b, r0:r0 + 8, :], xbuf[b, NR + r0:NR + r0 + 8, :]
                if b == 0:
                    xr = xr + jnp.where(lane == 0, sab[r0:r0 + 8, :], 0.0)
                    xi = xi + jnp.where(lane == 0, sab[NR + r0:NR + r0 + 8, :], 0.0)
                wr, wi = w_group(0, b, c0, mh), w_group(1, b, c0, mh)
                zr, zi = xr * wr - xi * wi, xr * wi + xi * wr
                z.append((zr + zi, zr, zi))
            for k in range(3):
                zs[k].append(_pack(z[0][k], z[-1][k]))
        k = [_dot_t(pltpu.bitcast(jnp.concatenate(zs[p], axis=0), bf16), sm[b, (0, 2, 1)[p]]) for p in range(3)]
        zbuf[b, 0:NR, :] = k[0] + k[2]
        zbuf[b, NR:2 * NR, :] = k[0] - k[1]

    def w_items(i):
        rows = range(WSPLIT[i] // 16, -(-WSPLIT[i + 1] // 16))
        return [P(w_rows, p, raw, r) for r in rows for p, raw in enumerate((wraw_r, wraw_i))]

    ds1 = opt.get("ds1", (0, 8, 13, 16))
    cp_sm.wait()
    for i in range(len(ds1) - 1):
        with scope("wait_w"):
            for d in cp_w[i]:
                d.wait()
        with scope("D1"):
            region(lambda: _interleave([P(phase_d1, b) for b in range(ds1[i], ds1[i + 1])], w_items(i)))
    with scope("wait_wms"):
        cp_wms.wait()
    with scope("D2"):
        def phase_d():
            _interleave([P(phase_d2, b) for b in range(NT - 1, 0, -1)], sa_items())
            phase_d2(0)
        region(phase_d)
    with scope("wait_wm1"):
        cp_di.wait()
        cp_wm1.wait()
    for d in [cp_wm2] + cp_w2:
        d.start()

    def phase_e(q):
        r0 = 8 * q
        y = _radix16([(zbuf[b, r0:r0 + 8, :], zbuf[b, NR + r0:NR + r0 + 8, :]) for b in range(NT)], 1)
        for t in range(NT):
            ybuf[t + zsm[1], q // 8, (q % 8) * 8:(q % 8) * 8 + 8, :] = _pack(*y[t])

    def f_mxu(g, t):
        if g < 4:
            xbuf[t, 128 * g:128 * (g + 1), :] = _dot(di[g], pltpu.bitcast(ybuf[t, g], bf16))
        else:
            xbuf[t, 512:576, :] = _dot(di[4, 0:64, 0:80], pltpu.bitcast(ybuf[t, 4, 0:40, :], bf16))

    def phase_ef():
        _interleave([P(phase_e, q) for q in qs(4)], mod_items(1152, 2944))
        for g in range(4):
            _interleave([P(f_mxu, (g - 1) % 5, t) for t in range(NT)], [P(phase_e, q) for q in qs(g)])
        _interleave([P(f_mxu, 3, t) for t in range(NT)], [center_sb])

    def center_sb():
        sb = [tbl[3 * D + 8 * r:3 * D + 8 * r + 8, :] for r in range(D // 8)]
        sbm = _colsum(sb) * (1.0 / D)
        for r in range(D // 8):
            sab[8 * r:8 * r + 8, :] = sb[r] - sbm

    with scope("E"):
        region(phase_ef)

    def f_p1(t, _):
        ln = pl.ds(pl.multiple_of(t * 128, 128), 128)
        accs = [None] * 3
        for j in range(8):
            v = [(xbuf[t, 128 * g + 8 * j:128 * g + 8 * j + 8, :],
                  xbuf[t, 128 * g + 64 + 8 * j:128 * g + 72 + 8 * j, :]) for g in range(4)]
            ys = _radix9_inv(xbuf[t, 512 + 8 * j:520 + 8 * j, :], v)
            for n9 in range(9):
                r = 8 * n9 + j
                xv = xT[8 * r:8 * r + 8, ln].astype(f32) + ys[n9] * tbl[2 * D + 8 * r:2 * D + 8 * r + 8, :]
                x1[t, 8 * r:8 * r + 8, :] = xv
                accs[n9 % 3] = xv if accs[n9 % 3] is None else accs[n9 % 3] + xv
        stat[0, t] = _tree(accs)

    def f_p2(t, _):
        mean = stat[0, t]
        a2 = [None] * 2
        az = [None] * 2
        for r in range(D // 8):
            xc = x1[t, 8 * r:8 * r + 8, :] - mean
            z = xc * tbl[4 * D + 8 * r:4 * D + 8 * r + 8, :]
            xbuf[t, 8 * r:8 * r + 8, :] = z
            k = r % 2
            a2[k] = xc * xc if a2[k] is None else a2[k] + xc * xc
            az[k] = z if az[k] is None else az[k] + z
        stat[1, t] = _tree(a2)
        stat[2, t] = _tree(az)

    def f_p3(t, _):
        rs = stat[1, t]
        mz = stat[2, t]
        a2 = [None] * 2
        for r in range(D // 8):
            dv = (xbuf[t, 8 * r:8 * r + 8, :] - mz) * rs + sab[8 * r:8 * r + 8, :]
            zbuf[t, pl.ds(16 * (r // 2) + r % 2, 8, stride=2), :] = dv
            k = r % 2
            a2[k] = dv * dv if a2[k] is None else a2[k] + dv * dv
        stat[3, t] = _tree(a2)

    with scope("F1"):
        jax.lax.fori_loop(0, NT, f_p1, None, unroll=2)
        finish(0, lambda v: v)
    with scope("F2"):
        jax.lax.fori_loop(0, NT, f_p2, None, unroll=2)
        finish(1, rsq)
        finish(2, lambda v: v)
    with scope("F3"):
        jax.lax.fori_loop(0, NT, f_p3, None, unroll=2)
        finish(3, rsq)

    cp_b1.wait()
    cp_b2.wait()
    tbl[0:40, :] = jnp.concatenate([b1v[...].astype(f32), jnp.zeros((4, 128), f32)], axis=0)
    tbl[40:56, :] = b2v[...].astype(f32) * 2.0

    def bias(r):
        return jnp.broadcast_to(tbl[pl.ds(r, 1), :], (8, 128))

    def left_rows(block, dst, slot, r0):
        ops = [_sa2([[block(r, c, r0 + 8 * h) for c in range(4)] for r in range(4)]) for h in range(2)]
        out = [_pack(ops[0][j], ops[1][j]) for j in range(49)]
        for j in range(49):
            dst[j, slot, r0 // 2:r0 // 2 + 8, :] = out[j]
        return out

    def f_p4(k, _):
        rs = [stat[3, 4 * k + c] for c in range(4)]
        for r0 in range(0, H, 16):
            left_rows(lambda r, c, row: zbuf[4 * k + c, r * H + row:r * H + row + 8, :] * rs[c], aop, k, r0)

    with scope("F4"):
        jax.lax.fori_loop(0, NT // 4, f_p4, None)

    def wait_w(src, dst, sems, i):
        for c in range(4):
            strip(src, dst, sems, 4 * i + c).wait()

    def hidden_rows(i, r0):
        return left_rows(lambda r, c, row: _gelu2(xbuf[4 * r + c, row:row + 8, :] + bias(4 * i + c)), gop, i, r0)

    def mlp1_chunk(i):
        prev = jnp.where(i == 0, NF - 1, i - 1)
        first, step = opt.get("h0", 1), opt.get("h1", 2)

        def hook(n):
            if n >= first and (n - first) % step == 0 and (n - first) // step < H // 16:
                r0 = 16 * ((n - first) // step)
                out = hidden_rows(prev, r0)
                tok = out[opt.get("tk", (0,))[0]]
                for j in opt.get("tk", (0,))[1:]:
                    tok = tok | out[j]
                aop[49 + zsm[1], 0, 0:8, :] = tok

        m = _strassen2(
            lambda j: jnp.concatenate([pltpu.bitcast(aop[j, k], bf16) for k in range(4)], axis=1),
            lambda o, r, c: jnp.concatenate(
                [w1v[4 * i + c + zsm[1 + o], 64 * (4 * k + r):64 * (4 * k + r + 1), :] for k in range(4)], axis=0),
            hook)
        u = _sc2(m)
        for r in range(4):
            for c in range(4):
                xbuf[4 * r + c, 0:H, :] = u[r][c]

    u1 = opt.get("u1", 1)

    def mlp1_step(n, _):
        for k in range(u1):
            wait_w(w1_h, w1v, w1sem, u1 * n + k)
        for k in range(u1):
            mlp1_chunk(u1 * n + k)

    with scope("mlp1"):
        jax.lax.fori_loop(0, NF // u1, mlp1_step, None)

    def out_copy(t):
        cols = pl.ds(pl.multiple_of(t * 128, 128), 128)
        return pltpu.make_async_copy(obuf.bitcast(bf16).at[t], out_h.at[:, cols], osem.at[t // 4])

    def mlp2(i, lhs):
        m = _strassen2(lhs, lambda o, r, c: jnp.concatenate(
            [w2v[4 * i + c + zsm[1 + o], 64 * (4 * k + r):64 * (4 * k + r + 1), :] for k in range(NF)], axis=0))
        y = _sc2(m)
        for c in range(4):
            bc = bias(40 + 4 * i + c)
            for r in (2, 3, 0, 1):
                for r0 in range(0, H, 16):
                    row = r * H + r0
                    o = [x1[4 * i + c, pl.ds(row + h, 8, stride=2), :]
                         + tbl[pl.ds(5 * D + row + h, 8, stride=2), :] * (y[r][c][r0 + 8 * h:r0 + 8 * h + 8] + bc)
                         for h in range(2)]
                    obuf[4 * i + c, row // 2:row // 2 + 8, :] = _pack(o[0], o[1])
            if opt.get("early", 1):
                out_copy(4 * i + c).start()
        if not opt.get("early", 1):
            for c in range(4):
                out_copy(4 * i + c).start()

    def mlp2_first():
        wait_w(w2_h, w2v, w2sem, 0)
        cp_wm2.wait()
        for it in mod_items(2944, 6 * D):
            it()
        for r0 in range(0, H, 16):
            hidden_rows(NF - 1, r0)
        mlp2(0, lambda j: jnp.concatenate([pltpu.bitcast(gop[j, k], bf16) for k in range(NF)], axis=1))

    def mlp2_step(i, _):
        wait_w(w2_h, w2v, w2sem, i)
        mlp2(i, lambda j: jnp.concatenate([pltpu.bitcast(gop[j, k], bf16) for k in range(NF)], axis=1))

    def mlp2_pre():
        cp_wm2.wait()
        _interleave(mod_items(2944, 6 * D), [P(hidden_rows, NF - 1, r0) for r0 in range(0, H, 16)])

    peel = opt.get("peel", 1)
    with scope("mlp2_0"):
        region(mlp2_first if peel else mlp2_pre)
    def mlp2_rest():
        for i in range(1, NS):
            wait_w(w2_h, w2v, w2sem, i)
        for i in range(1, NS):
            mlp2(i, lambda j: jnp.concatenate([pltpu.bitcast(gop[j, k], bf16) for k in range(NF)], axis=1))

    with scope("mlp2"):
        if opt.get("u2", 0):
            region(mlp2_rest)
        else:
            jax.lax.fori_loop(peel, NS, mlp2_step, None)
    for t in range(NT):
        out_copy(t).wait()


@jax.jit
def pallas_adaLN_cond__spectral_gfnet__mixer_token_mlp__prompt_kernel(
    A_x: jax.Array,
    A_w_r: jax.Array,
    A_w_i: jax.Array,
    B_x: jax.Array,
    B_w1: jax.Array,
    B_b1: jax.Array,
    B_w2: jax.Array,
    B_b2: jax.Array,
    c: jax.Array,
    w_mod: jax.Array,
):
    del B_x
    any_spec = pl.BlockSpec(memory_space=pl.ANY)
    scratch = [
        pltpu.VMEM((D, S), bf16),
        pltpu.VMEM((289, S), bf16),
        pltpu.VMEM((289, S), bf16),
        pltpu.VMEM((2, NT, 152, 128), u32),
        pltpu.VMEM((F // 128, S // 2, 128), u32),
        pltpu.VMEM((NT, F // 2, 128), u32),
        pltpu.VMEM((F // 128, 128), bf16),
        pltpu.VMEM((S // 128, 128), bf16),
        pltpu.VMEM((1, D), bf16),
        pltpu.VMEM((D, 6 * D), bf16),
        pltpu.VMEM((5, 128, 128), bf16),
        pltpu.VMEM((5, 128, 128), bf16),
        pltpu.VMEM((NT, 3, 128, 128), bf16),
        pltpu.VMEM((6 * D, 128), f32),
        pltpu.VMEM((NT + 1, 5, 64, 128), u32),
        pltpu.VMEM((NT, 2 * NR, 128), f32),
        pltpu.VMEM((NT, 3, NR // 2, 128), u32),
        pltpu.VMEM((2 * NR, 128), f32),
        pltpu.VMEM((NT, 8, 128), f32),
        pltpu.VMEM((4, NT, 8, 128), f32),
        pltpu.VMEM((NT, 2 * NR, 128), f32),
        pltpu.VMEM((NT, D, 128), f32),
        pltpu.VMEM((50, 4, H // 2, 128), u32),
        pltpu.VMEM((49, NF, H // 2, 128), u32),
        pltpu.VMEM((NT, D // 2, 128), u32),
        pltpu.SMEM((8,), jnp.int32),
        pltpu.SemaphoreType.DMA((25,)),
        pltpu.SemaphoreType.DMA((NF,)),
        pltpu.SemaphoreType.DMA((NS,)),
        pltpu.SemaphoreType.DMA((NS,)),
    ]
    outT = pl.pallas_call(
        functools.partial(_kernel, scopes=False, opt={}),
        out_shape=jax.ShapeDtypeStruct((D, S), bf16),
        in_specs=[any_spec] * 13,
        out_specs=any_spec,
        scratch_shapes=scratch,
        compiler_params=pltpu.CompilerParams(vmem_limit_bytes=120 * 1024 * 1024),
        name="adaln_gfnet_mixer",
    )(np.array([1, 0, 0, 0, 0, 0, 0, 0], np.int32), A_x[0].T, A_w_r.T, A_w_i.T, B_w1, B_b1.reshape(F // 128, 128), B_w2,
      B_b2.reshape(S // 128, 128), c, w_mod, _DFWD, _DINV, _SMAT)
    return outT.T[None]
```

```python
import contextlib
import functools

import jax
import jax.numpy as jnp
import numpy as np
import ml_dtypes
import jax.experimental.pallas as pl
import jax.experimental.pallas.tpu as pltpu

S, D, F = 2048, 576, 4608
NT = S // 128
NP = 19
NR = NP * 16
H = D // 4
f32, bf16, u32 = jnp.float32, jnp.bfloat16, jnp.uint32
EPS = 1e-5

_TH = 2 * np.pi / 9
C1, C2, C4 = float(np.cos(_TH)), float(np.cos(2 * _TH)), float(np.cos(4 * _TH))
S1, S3, S4 = float(np.sin(_TH)), float(np.sin(3 * _TH)), float(np.sin(4 * _TH))


_SETS = [[g, g + 9, 9 - g, 18 - g] for g in range(1, 5)] + [[0, 9, 288]]
_FLAT = [c for grp in _SETS for c in grp]


def _row_pairs(m):
    bits = m.astype(ml_dtypes.bfloat16).view(np.uint16).astype(np.uint32)
    return bits[..., 0::2, :] | (bits[..., 1::2, :] << 16)


def _d_mats():
    d2 = np.arange(64)
    fwd = np.zeros((5, 128, 128))
    inv = np.zeros((5, 128, 128))
    col = 16 * (d2 // 8) + 2 * (d2 % 8)
    for g, grp in enumerate(_SETS):
        res = (g + 1) % 5
        scale = (0.0, S1, S1, S3, S1)[res]
        for cc, c0 in enumerate(grp):
            for m in range(1 if c0 == 288 else 16):
                kx = c0 + 18 * m
                ph = 2 * np.pi * ((kx * d2) % D) / D
                c, s = np.cos(ph), np.sin(ph)
                if kx % 288 == 0:
                    s = np.zeros_like(s)
                sg = (1.0 if kx % 9 == res else -1.0) * scale
                row = 32 * cc + 16 * (m % 2) + m // 2
                fwd[g, row, col] = c
                fwd[g, row + 8, col] = -s
                fwd[g, row, col + 1] = -sg * s
                fwd[g, row + 8, col + 1] = -sg * c
                w = (1.0 if kx % 288 == 0 else 2.0) / (S * D)
                k = 32 * cc + 2 * (2 * (m % 8) + m // 8)
                inv[g, d2, k] = w * c
                inv[g, d2, k + 1] = -w * s
                inv[g, 64 + d2, k] = sg * w * s
                inv[g, 64 + d2, k + 1] = sg * w * c
    return _row_pairs(fwd), _row_pairs(inv)


def _s_mats():
    m = np.zeros((NT, 2, 128, 128))
    lane = np.arange(128)
    for b in range(NT):
        a = (lane - b) % 16
        k = 128 * a + (lane - a) % 128
        ph = 2 * np.pi * ((lane[:, None] * k[None, :]) % S) / S
        m[b] = np.cos(ph), -np.sin(ph)
    return _row_pairs(m)


_DFWD, _DINV = _d_mats()
_SMAT = _s_mats()


def _as_bf16(x):
    return pltpu.bitcast(x, bf16)


def _dot(a, b):
    return jnp.dot(a, b, preferred_element_type=f32)


def _dot_t(a, b):
    return jax.lax.dot_general(a, b, (((1,), (1,)), ((), ())), preferred_element_type=f32)


def _pack(a, b):
    return pltpu.pack_elementwise([a, b], packed_dtype=bf16)


def _unpack(x, i):
    return pltpu.unpack_elementwise(x, index=i, packed_dtype=bf16, unpacked_dtype=f32)


def _radix9_fwd(a):
    p = [None] + [a[n] + a[9 - n] for n in range(1, 5)]
    m = [None] + [a[n] - a[9 - n] for n in range(1, 5)]
    t = p[1] + p[2] + p[4]
    u = a[0] + p[3]
    b = a[0] - 0.5 * p[3]
    e1 = p[1] - p[4]
    e2 = p[2] - p[4]
    r1 = C1 * e1 + C2 * e2
    r2 = C2 * e1 + C4 * e2
    f1 = m[1] + m[2]
    f2 = m[2] + m[4]
    f3 = m[1] - m[4]
    q1 = f1 + (S4 / S1) * f2
    q2 = f3 + (S4 / S1) * f1
    n3 = (S3 / S1) * m[3]
    return u + t, [(b + r1, q1 + n3), (b + r2, q2 - n3), (u - 0.5 * t, m[1] - m[2] + m[4]),
                   (b - (r1 + r2), (q2 - q1) + n3)]


def _radix9_inv(v0, v):
    (r1_, i1), (r2_, i2), (r3_, i3), (r4_, i4) = v
    t = r1_ + r2_ + r4_
    u = v0 + r3_
    b = v0 - 0.5 * r3_
    e1 = r1_ - r4_
    e2 = r2_ - r4_
    r1 = C1 * e1 + C2 * e2
    r2 = C2 * e1 + C4 * e2
    a1, a2, a3, a4 = b + r1, b + r2, u - 0.5 * t, b - (r1 + r2)
    f1 = i1 + i2
    f2 = i2 + i4
    f3 = i1 - i4
    q1 = f1 + (S4 / S1) * f2
    q2 = f3 + (S4 / S1) * f1
    b1, b2, b4 = q1 + i3, q2 - i3, (q2 - q1) + i3
    b3 = (S3 / S1) * (i1 - i2 + i4)
    return [u + t, a1 - b1, a2 - b2, a3 - b3, a4 - b4, a4 + b4, a3 + b3, a2 + b2, a1 + b1]


def _bfly4(a, b, c, d, sgn, c_rot=False):
    if c_rot:
        if sgn < 0:
            t0 = (a[0] + c[1], a[1] - c[0])
            t1 = (a[0] - c[1], a[1] + c[0])
        else:
            t0 = (a[0] - c[1], a[1] + c[0])
            t1 = (a[0] + c[1], a[1] - c[0])
    else:
        t0 = (a[0] + c[0], a[1] + c[1])
        t1 = (a[0] - c[0], a[1] - c[1])
    t2 = (b[0] + d[0], b[1] + d[1])
    t3 = (b[0] - d[0], b[1] - d[1])
    x0 = (t0[0] + t2[0], t0[1] + t2[1])
    x2 = (t0[0] - t2[0], t0[1] - t2[1])
    xm = (t1[0] + t3[1], t1[1] - t3[0])
    xp = (t1[0] - t3[1], t1[1] + t3[0])
    return [x0, xm, x2, xp] if sgn < 0 else [x0, xp, x2, xm]


def _tw16(z, e, sgn):
    c = float(np.cos(2 * np.pi * e / 16))
    s = float(sgn * np.sin(2 * np.pi * e / 16))
    x, y = z
    if e % 2 == 0:
        if (c > 0) == (s > 0):
            return ((x - y) * c, (x + y) * c)
        return ((x + y) * c, (y - x) * c)
    return (x * c - y * s, x * s + y * c)


def _radix16(x, sgn):
    u = [_bfly4(x[n2], x[4 + n2], x[8 + n2], x[12 + n2], sgn) for n2 in range(4)]
    out = [None] * 16
    for k1 in range(4):
        v = []
        for n2 in range(4):
            e = k1 * n2
            v.append(u[n2][k1] if e % 4 == 0 else _tw16(u[n2][k1], e, sgn))
        y = _bfly4(v[0], v[1], v[2], v[3], sgn, c_rot=(k1 == 2))
        for k2 in range(4):
            out[k1 + 4 * k2] = y[k2]
    return out


def _sa(a11, a12, a21, a22):
    return [a11 + a22, a21 + a22, a11, a22, a11 + a12, a21 - a11, a12 - a22]


def _sb(b11, b12, b21, b22):
    return [b11 + b22, b11, b12 - b22, b21 - b11, b22, b11 + b12, b21 + b22]


def _sc(m):
    m1, m2, m3, m4, m5, m6, m7 = m
    return [m4 + m7 - m5 + m1, m5 + m3, m2 + m4, m1 - m2 + m3 + m6]


def _sa2(blk):
    lvl = [_sa(blk[ri][ci], blk[ri][2 + ci], blk[2 + ri][ci], blk[2 + ri][2 + ci])
           for ri in range(2) for ci in range(2)]
    return [x for o in range(7) for x in _sa(*[l[o] for l in lvl])]


def _sc2(m):
    p = [_sc(m[7 * o:7 * o + 7]) for o in range(7)]
    out = [[None] * 4 for _ in range(4)]
    for ii in range(4):
        for oi, v in enumerate(_sc([p[o][ii] for o in range(7)])):
            out[2 * (oi // 2) + ii // 2][2 * (oi % 2) + ii % 2] = v
    return out


_SB_TERMS = (((1, 0, 0), (1, 1, 1)), ((1, 0, 0),), ((1, 0, 1), (-1, 1, 1)), ((1, 1, 0), (-1, 0, 0)),
             ((1, 1, 1),), ((1, 0, 0), (1, 0, 1)), ((1, 1, 0), (1, 1, 1)))
_ORDER = (1, 3, 6, 4, 0, 2, 5)


def _strassen2(lhs, raw, hook=None):
    m = [None] * 49
    done = 0
    for o in _ORDER:
        blocks = {}
        halves = []
        for h in range(2):
            quad = []
            for ri in range(2):
                for ci in range(2):
                    acc = None
                    for sg, ro, co in _SB_TERMS[o]:
                        key = (2 * ro + ri, 2 * co + ci)
                        if key not in blocks:
                            blocks[key] = raw(o, *key)
                        v = _unpack(blocks[key], h)
                        acc = v if acc is None else (acc + v if sg > 0 else acc - v)
                    quad.append(acc)
            halves.append(_sb(*quad))
        for j in _ORDER:
            if hook is not None:
                hook(done)
            done += 1
            rhs = pltpu.bitcast(_pack(halves[0][j], halves[1][j]), bf16)
            m[7 * o + j] = _dot(lhs(7 * o + j), rhs)
    return m


def _gelu2(u):
    k0 = 0.7978845608028654
    z = u * (k0 + (k0 * 0.044715) * (u * u))
    return u * jnp.tanh(z) + u


def _tree(vs):
    vs = list(vs)
    while len(vs) > 1:
        vs = [vs[i] + vs[i + 1] if i + 1 < len(vs) else vs[i] for i in range(0, len(vs), 2)]
    return vs[0]


def _colsum(vs, lanes=4):
    accs = []
    for k in range(lanes):
        acc = None
        for v in vs[k::lanes]:
            acc = v if acc is None else acc + v
        accs.append(acc)
    return jnp.sum(_tree(accs), axis=0, keepdims=True)


def _interleave(*lists):
    items = []
    for ci, lst in enumerate(lists):
        for k, it in enumerate(lst):
            items.append(((k + 0.5) / len(lst), ci, k, it))
    items.sort(key=lambda x: x[:3])
    for x in items:
        x[3]()


FC = 512
NF = F // FC
SC = 512
NS = S // SC
XC = 8
WSPLIT = (0, 96, 192, 289)


def _kernel(z_h, xT_h, wr_h, wi_h, w1_h, b1_h, w2_h, b2_h, c_h, wm_h, df_h, di_h, sm_h, out_h,
            xw, xT, wraw_r, wraw_i, wp, w1v, w2v, b1v, b2v, cv, wm, df, di, sm, sm3, tbl, ybuf, xbuf, cbuf, sab,
            mnb, stat, zbuf, x1, aop, gop, obuf, zsm, sem, w1sem, w2sem, osem, *, scopes, opt):
    n = [0]

    def scope(name):
        return jax.named_scope(name) if scopes else contextlib.nullcontext()

    def cp(src, dst):
        d = pltpu.make_async_copy(src, dst, sem.at[n[0]])
        n[0] += 1
        return d

    cp_c = cp(c_h, cv)
    cp_wm0 = cp(wm_h.at[:, 512:1152], wm.at[:, 512:1152])
    xsem = n[0]
    cp_x = [cp(xT_h.at[:, i * 256:(i + 1) * 256], xw.at[i]) for i in range(NT // 2)]
    cp_z = cp(z_h, zsm)
    cp_df = cp(df_h, df)
    cp_sm = cp(sm_h, sm)
    cp_w = [[cp(src.at[lo:hi], dst.at[lo:hi]) for src, dst in ((wr_h, wraw_r), (wi_h, wraw_i))]
            for lo, hi in zip(WSPLIT[:-1], WSPLIT[1:])]
    cp_wms = cp(wm_h.at[:, 0:512], wm.at[:, 0:512])
    cp_di = cp(di_h, di)
    cp_wm1 = cp(wm_h.at[:, 1152:2944], wm.at[:, 1152:2944])
    cp_wm2 = cp(wm_h.at[:, 2944:6 * D], wm.at[:, 2944:6 * D])
    cp_b1 = cp(b1_h, b1v)
    cp_b2 = cp(b2_h, b2v)

    def strip(src, dst, sems, j):
        cols = pl.ds(pl.multiple_of(j * 128, 128), 128)
        return pltpu.make_async_copy(src.at[:, cols], dst.bitcast(bf16).at[j], sems.at[j // 4])

    cp_w1 = [strip(w1_h, w1v, w1sem, j) for j in range(F // 128)]
    cp_w2 = [strip(w2_h, w2v, w2sem, j) for j in range(NT)]

    for d in [cp_c, cp_wm0, *cp_x, cp_z, cp_df, cp_sm, *sum(cp_w, []), cp_wms, cp_di, cp_wm1, cp_b1, cp_b2]:
        d.start()

    cp_c.wait()
    cc = cv[...].astype(f32)
    sc = jnp.broadcast_to(cc * jax.nn.sigmoid(cc), (16, D)).astype(bf16)

    def mod_items(lo, hi):
        box = []

        def first():
            box.append(_dot(sc, wm[:, lo:hi]))

        def tile(j):
            r0 = lo + j * 128
            row = box[0][0:1, j * 128:(j + 1) * 128]
            col = r0 + jax.lax.broadcasted_iota(jnp.int32, (1, 128), 1)
            is_scale = ((col >= D) & (col < 2 * D)) | ((col >= 4 * D) & (col < 5 * D))
            row = row * jnp.where(col >= 5 * D, 0.5, 1.0) + jnp.where(is_scale, 1.0, 0.0)
            tbl[r0:r0 + 128, :] = jnp.broadcast_to(row, (128, 128)).T

        return [first] + [functools.partial(tile, j) for j in range((hi - lo) // 128)]

    with scope("wait_wm0"):
        cp_wm0.wait()
    with scope("mod0"):
        for it in mod_items(512, 1152):
            it()

    ones = jnp.ones((16, D), bf16)
    rsq = lambda v: jax.lax.rsqrt(v + EPS)

    def finish(k, fn):
        for t in range(NT):
            stat[k, t] = jnp.broadcast_to(fn(jnp.sum(stat[k, t], axis=0, keepdims=True) * (1.0 / D)), (8, 128))

    def x_rows(t, r):
        v = pltpu.bitcast(xT[t, 8 * (r // 2):8 * (r // 2) + 8, :], bf16).astype(f32)
        return v[8 * (r % 2):8 * (r % 2) + 8]

    def b_mean(tp, k):
        t = 2 * tp + k
        xs = []
        for r in range(D // 16):
            v = xw[tp, 16 * r:16 * r + 16, 128 * k:128 * k + 128]
            xT[t, 8 * r:8 * r + 8, :] = pltpu.bitcast(v, u32)
            v = v.astype(f32)
            xs += [v[0:8], v[8:16]]
        mnb[t] = jnp.broadcast_to(_colsum(xs, 3) * (1.0 / D), (8, 128))

    def radix9_store(t, load):
        for j in range(8):
            y0, ys = _radix9_fwd([load(8 * n9 + j) for n9 in range(9)])
            ybuf[t, 4, 8 * j:8 * j + 8, :] = _pack(y0, jnp.zeros_like(y0))
            for g in range(4):
                ybuf[t, g, 8 * j:8 * j + 8, :] = _pack(*ys[g])

    def b_vpu(t):
        mean = mnb[t]
        accs = [None] * 3

        def load(r):
            xc = x_rows(t, r) - mean
            k = (r // 8) % 3
            accs[k] = xc * xc if accs[k] is None else accs[k] + xc * xc
            return xc * tbl[D + 8 * r:D + 8 * r + 8, :]

        radix9_store(t, load)
        stat[0, t] = _tree(accs)

    def b_pair(tp, _):
        pltpu.make_async_copy(xT_h.at[:, 0:256], xw.at[tp], sem.at[xsem + tp]).wait()
        b_mean(tp, 0)
        b_mean(tp, 1)
        b_vpu(2 * tp)
        b_vpu(2 * tp + 1)

    with scope("B"):
        jax.lax.fori_loop(0, NT // 2, b_pair, None)
    finish(0, rsq)
    for d in cp_w1:
        d.start()

    def d_fwd(g, t):
        rows = 128 if g < 4 else 80
        return _dot(_as_bf16(df[g, 0:rows // 2, :]), _as_bf16(ybuf[t, g]))

    def phase_c():
        for g, grp in enumerate(_SETS):
            for cc, c0 in enumerate(grp):
                nr = 16 if c0 == 288 else 32
                z = zsm[1 + cc] if opt.get("cz", 1) else 0
                xs = [_dot(_as_bf16(df[g, 16 * cc:16 * cc + nr // 2, :]), _as_bf16(ybuf[t + z, g])) for t in range(NT)]
                y = [_radix16([(xs[t][r0:r0 + 8] * stat[0, t], xs[t][r0 + 8:r0 + 16] * stat[0, t])
                               for t in range(NT)], -1) for r0 in range(0, nr, 16)]
                rows = slice(8 * (4 * g + cc), 8 * (4 * g + cc) + 8)
                for b in range(NT):
                    (er, ei), (odr, odi) = y[0][b], y[-1][b]
                    cbuf[b, 0, rows, :] = _pack(er + ei, odr + odi)
                    cbuf[b, 1, rows, :] = _pack(er, odr)
                    cbuf[b, 2, rows, :] = _pack(ei, odi)

    P = functools.partial
    qs = lambda g: range(8 * g, min(8 * g + 8, 2 * NP - 1))

    def region(fn):
        jax.lax.fori_loop(0, one, lambda i, _: fn(), None)

    cp_z.wait()
    one = jnp.minimum(zsm[0], 1)
    cp_df.wait()
    with scope("C"):
        region(phase_c)

    def sa_items():
        def last():
            for g, grp in enumerate(_SETS):
                r = d_fwd(g, NT) * float(S)
                for cc, c0 in enumerate(grp):
                    for par in range(2):
                        r0 = 32 * cc + (0 if c0 == 288 else 16 * par)
                        for ri in range(2):
                            sab[pl.ds(ri * NR + 16 * (4 * g + cc) + par, 8, stride=2), :] = r[r0 + 8 * ri:r0 + 8 * ri + 8]
        return mod_items(0, 512) + [lambda: radix9_store(NT, lambda r: tbl[8 * r:8 * r + 8, :]), last]

    lane = jax.lax.broadcasted_iota(jnp.int32, (8, 128), 1)
    masks = [(lane & (1 << b)) != 0 for b in range(4)]

    def shuffle(vals):
        vals = [pltpu.roll(v, a, 1) if a else v for a, v in enumerate(vals)]
        vals = [vals[(-b) % 16] for b in range(16)]
        for b in range(4):
            vals = [jnp.where(masks[b], vals[(i - (1 << b)) % 16], vals[i]) for i in range(16)]
        return vals

    def w_rows(p, raw, r):
        if r < 18:
            vals = shuffle([pltpu.bitcast(raw[16 * r:16 * r + 16, a * 128:(a + 1) * 128], u32) for a in range(16)])
        else:
            last = jnp.broadcast_to(raw[288:289, :].astype(f32), (8, S))
            vals = shuffle([pltpu.bitcast(last[:, a * 128:(a + 1) * 128], u32) for a in range(16)])
        for b in range(16):
            wp[p, b, 8 * r:8 * r + 8, :] = vals[b]

    def phase_d1(b):
        fr, fi = sm[b, 0], sm[b, 1]
        dif = _pack(*[_unpack(fi, h) - _unpack(fr, h) for h in range(2)])
        tot = _pack(*[_unpack(fr, h) + _unpack(fi, h) for h in range(2)])
        sm3[b, 0] = dif
        sm3[b, 1] = tot
        k = [_dot(_as_bf16(cbuf[b, p]), _as_bf16(m)) for p, m in enumerate((fr, dif, tot))]
        xbuf[b, 0:NR, :] = k[0] - k[2]
        xbuf[b, NR:2 * NR, :] = k[0] + k[1]

    def w_group(p, b, c0, mh):
        if c0 == 288:
            return pltpu.bitcast(wp[p, b, 144:152, :], f32)
        return _unpack(wp[p, b, pl.ds(c0 // 2 + 72 * mh, 8, stride=9), :], c0 % 2)

    def phase_d2(b):
        zs = [[], [], []]
        for p, c0 in enumerate(_FLAT):
            z = []
            for mh in range(1 if c0 == 288 else 2):
                r0 = 16 * p + 8 * mh
                xr, xi = xbuf[b, r0:r0 + 8, :], xbuf[b, NR + r0:NR + r0 + 8, :]
                if b == 0:
                    xr = xr + jnp.where(lane == 0, sab[r0:r0 + 8, :], 0.0)
                    xi = xi + jnp.where(lane == 0, sab[NR + r0:NR + r0 + 8, :], 0.0)
                wr, wi = w_group(0, b, c0, mh), w_group(1, b, c0, mh)
                zr, zi = xr * wr - xi * wi, xr * wi + xi * wr
                z.append((zr + zi, zr, zi))
            for k in range(3):
                zs[k].append(_pack(z[0][k], z[-1][k]))
        k = [_dot_t(_as_bf16(jnp.concatenate(z, axis=0)), _as_bf16(m))
             for z, m in zip(zs, (sm[b, 0], sm3[b, 1], sm3[b, 0]))]
        zbuf[b, 0:NR, :] = k[0] + k[2]
        zbuf[b, NR:2 * NR, :] = k[0] - k[1]

    def w_items(i):
        rows = range(WSPLIT[i] // 16, -(-WSPLIT[i + 1] // 16))
        return [P(w_rows, p, raw, r) for r in rows for p, raw in enumerate((wraw_r, wraw_i))]

    ds1 = opt.get("ds1", (0, 8, 13, 16))
    cp_sm.wait()
    for i in range(len(ds1) - 1):
        with scope("wait_w"):
            for d in cp_w[i]:
                d.wait()
        with scope("D1"):
            region(lambda: _interleave([P(phase_d1, b) for b in range(ds1[i], ds1[i + 1])], w_items(i)))
    with scope("wait_wms"):
        cp_wms.wait()
    with scope("D2"):
        def phase_d():
            _interleave([P(phase_d2, b) for b in range(NT - 1, 0, -1)], sa_items())
            phase_d2(0)
        region(phase_d)
    with scope("wait_wm1"):
        cp_di.wait()
        cp_wm1.wait()
    for d in [cp_wm2] + cp_w2:
        d.start()

    def phase_e(q):
        r0 = 8 * q
        y = _radix16([(zbuf[b, r0:r0 + 8, :], zbuf[b, NR + r0:NR + r0 + 8, :]) for b in range(NT)], 1)
        for t in range(NT):
            ybuf[t + zsm[1], q // 8, (q % 8) * 8:(q % 8) * 8 + 8, :] = _pack(*y[t])

    def f_mxu(g, t):
        if g < 4:
            xbuf[t, 128 * g:128 * (g + 1), :] = _dot(_as_bf16(di[g]), _as_bf16(ybuf[t, g]))
        else:
            xbuf[t, 512:576, :] = _dot(_as_bf16(di[4, 0:32, :])[:, 0:80], _as_bf16(ybuf[t, 4, 0:40, :]))

    def phase_ef():
        _interleave([P(phase_e, q) for q in qs(4)], mod_items(1152, 2944))
        for g in range(4):
            _interleave([P(f_mxu, (g - 1) % 5, t) for t in range(NT)], [P(phase_e, q) for q in qs(g)])
        _interleave([P(f_mxu, 3, t) for t in range(NT)], [center_sb])

    def center_sb():
        sb = [tbl[3 * D + 8 * r:3 * D + 8 * r + 8, :] for r in range(D // 8)]
        sbm = _colsum(sb) * (1.0 / D)
        for r in range(D // 8):
            sab[8 * r:8 * r + 8, :] = sb[r] - sbm

    with scope("E"):
        region(phase_ef)

    def f_p1(t, _):
        accs = [None] * 3
        for j in range(8):
            v = [(xbuf[t, 128 * g + 8 * j:128 * g + 8 * j + 8, :],
                  xbuf[t, 128 * g + 64 + 8 * j:128 * g + 72 + 8 * j, :]) for g in range(4)]
            ys = _radix9_inv(xbuf[t, 512 + 8 * j:520 + 8 * j, :], v)
            for n9 in range(9):
                r = 8 * n9 + j
                xv = x_rows(t, r) + ys[n9] * tbl[2 * D + 8 * r:2 * D + 8 * r + 8, :]
                x1[t, 8 * r:8 * r + 8, :] = xv
                accs[n9 % 3] = xv if accs[n9 % 3] is None else accs[n9 % 3] + xv
        stat[0, t] = _tree(accs)

    def f_p2(t, _):
        mean = stat[0, t]
        a2 = [None] * 2
        az = [None] * 2
        for r in range(D // 8):
            xc = x1[t, 8 * r:8 * r + 8, :] - mean
            z = xc * tbl[4 * D + 8 * r:4 * D + 8 * r + 8, :]
            xbuf[t, 8 * r:8 * r + 8, :] = z
            k = r % 2
            a2[k] = xc * xc if a2[k] is None else a2[k] + xc * xc
            az[k] = z if az[k] is None else az[k] + z
        stat[1, t] = _tree(a2)
        stat[2, t] = _tree(az)

    def f_p3(t, _):
        rs = stat[1, t]
        mz = stat[2, t]
        a2 = [None] * 2
        for r in range(D // 8):
            dv = (xbuf[t, 8 * r:8 * r + 8, :] - mz) * rs + sab[8 * r:8 * r + 8, :]
            zbuf[t, pl.ds(16 * (r // 2) + r % 2, 8, stride=2), :] = dv
            k = r % 2
            a2[k] = dv * dv if a2[k] is None else a2[k] + dv * dv
        stat[3, t] = _tree(a2)

    with scope("F1"):
        jax.lax.fori_loop(0, NT, f_p1, None, unroll=2)
        finish(0, lambda v: v)
    with scope("F2"):
        jax.lax.fori_loop(0, NT, f_p2, None, unroll=2)
        finish(1, rsq)
        finish(2, lambda v: v)
    with scope("F3"):
        jax.lax.fori_loop(0, NT, f_p3, None, unroll=2)
        finish(3, rsq)

    cp_b1.wait()
    cp_b2.wait()
    tbl[0:40, :] = jnp.concatenate([b1v[...].astype(f32), jnp.zeros((4, 128), f32)], axis=0)
    tbl[40:56, :] = b2v[...].astype(f32) * 2.0

    def bias(r):
        return jnp.broadcast_to(tbl[pl.ds(r, 1), :], (8, 128))

    def left_rows(block, dst, slot, r0):
        ops = [_sa2([[block(r, c, r0 + 8 * h) for c in range(4)] for r in range(4)]) for h in range(2)]
        out = [_pack(ops[0][j], ops[1][j]) for j in range(49)]
        for j in range(49):
            dst[j, slot, r0 // 2:r0 // 2 + 8, :] = out[j]
        return out

    def f_p4(k, _):
        rs = [stat[3, 4 * k + c] for c in range(4)]
        for r0 in range(0, H, 16):
            left_rows(lambda r, c, row: zbuf[4 * k + c, r * H + row:r * H + row + 8, :] * rs[c], aop, k, r0)

    with scope("F4"):
        jax.lax.fori_loop(0, NT // 4, f_p4, None)

    def wait_w(src, dst, sems, i):
        for c in range(4):
            strip(src, dst, sems, 4 * i + c).wait()

    def hidden_rows(i, r0):
        return left_rows(lambda r, c, row: _gelu2(xbuf[4 * r + c, row:row + 8, :] + bias(4 * i + c)), gop, i, r0)

    def mlp1_chunk(i):
        prev = jnp.where(i == 0, NF - 1, i - 1)
        first, step = opt.get("h0", 1), opt.get("h1", 2)

        def hook(n):
            if n >= first and (n - first) % step == 0 and (n - first) // step < H // 16:
                r0 = 16 * ((n - first) // step)
                out = hidden_rows(prev, r0)
                tok = out[opt.get("tk", (0,))[0]]
                for j in opt.get("tk", (0,))[1:]:
                    tok = tok | out[j]
                aop[49 + zsm[1], 0, 0:8, :] = tok

        m = _strassen2(
            lambda j: jnp.concatenate([pltpu.bitcast(aop[j, k], bf16) for k in range(4)], axis=1),
            lambda o, r, c: jnp.concatenate(
                [w1v[4 * i + c + zsm[1 + o], 64 * (4 * k + r):64 * (4 * k + r + 1), :] for k in range(4)], axis=0),
            hook)
        u = _sc2(m)
        for r in range(4):
            for c in range(4):
                xbuf[4 * r + c, 0:H, :] = u[r][c]

    u1 = opt.get("u1", 1)

    def mlp1_step(n, _):
        for k in range(u1):
            wait_w(w1_h, w1v, w1sem, u1 * n + k)
        for k in range(u1):
            mlp1_chunk(u1 * n + k)

    with scope("mlp1"):
        jax.lax.fori_loop(0, NF // u1, mlp1_step, None)

    def out_copy(t):
        cols = pl.ds(pl.multiple_of(t * 128, 128), 128)
        return pltpu.make_async_copy(obuf.bitcast(bf16).at[t], out_h.at[:, cols], osem.at[t // 4])

    def mlp2(i, lhs):
        m = _strassen2(lhs, lambda o, r, c: jnp.concatenate(
            [w2v[4 * i + c + zsm[1 + o], 64 * (4 * k + r):64 * (4 * k + r + 1), :] for k in range(NF)], axis=0))
        y = _sc2(m)
        for c in range(4):
            bc = bias(40 + 4 * i + c)
            for r in (2, 3, 0, 1):
                for r0 in range(0, H, 16):
                    row = r * H + r0
                    o = [x1[4 * i + c, pl.ds(row + h, 8, stride=2), :]
                         + tbl[pl.ds(5 * D + row + h, 8, stride=2), :] * (y[r][c][r0 + 8 * h:r0 + 8 * h + 8] + bc)
                         for h in range(2)]
                    obuf[4 * i + c, row // 2:row // 2 + 8, :] = _pack(o[0], o[1])
            if opt.get("early", 1):
                out_copy(4 * i + c).start()
        if not opt.get("early", 1):
            for c in range(4):
                out_copy(4 * i + c).start()

    def mlp2_first():
        wait_w(w2_h, w2v, w2sem, 0)
        cp_wm2.wait()
        for it in mod_items(2944, 6 * D):
            it()
        for r0 in range(0, H, 16):
            hidden_rows(NF - 1, r0)
        mlp2(0, lambda j: jnp.concatenate([pltpu.bitcast(gop[j, k], bf16) for k in range(NF)], axis=1))

    def mlp2_step(i, _):
        wait_w(w2_h, w2v, w2sem, i)
        mlp2(i, lambda j: jnp.concatenate([pltpu.bitcast(gop[j, k], bf16) for k in range(NF)], axis=1))

    def mlp2_pre():
        cp_wm2.wait()
        _interleave(mod_items(2944, 6 * D), [P(hidden_rows, NF - 1, r0) for r0 in range(0, H, 16)])

    peel = opt.get("peel", 1)
    with scope("mlp2_0"):
        region(mlp2_first if peel else mlp2_pre)
    def mlp2_rest():
        for i in range(1, NS):
            wait_w(w2_h, w2v, w2sem, i)
        for i in range(1, NS):
            mlp2(i, lambda j: jnp.concatenate([pltpu.bitcast(gop[j, k], bf16) for k in range(NF)], axis=1))

    with scope("mlp2"):
        if opt.get("u2", 0):
            region(mlp2_rest)
        else:
            jax.lax.fori_loop(peel, NS, mlp2_step, None)
    for t in range(NT):
        out_copy(t).wait()


@jax.jit
def pallas_adaLN_cond__spectral_gfnet__mixer_token_mlp__prompt_kernel(
    A_x: jax.Array,
    A_w_r: jax.Array,
    A_w_i: jax.Array,
    B_x: jax.Array,
    B_w1: jax.Array,
    B_b1: jax.Array,
    B_w2: jax.Array,
    B_b2: jax.Array,
    c: jax.Array,
    w_mod: jax.Array,
):
    del B_x
    any_spec = pl.BlockSpec(memory_space=pl.ANY)
    scratch = [
        pltpu.VMEM((NT // 2, D, 256), bf16),
        pltpu.VMEM((NT, D // 2, 128), u32),
        pltpu.VMEM((289, S), bf16),
        pltpu.VMEM((289, S), bf16),
        pltpu.VMEM((2, NT, 152, 128), u32),
        pltpu.VMEM((F // 128, S // 2, 128), u32),
        pltpu.VMEM((NT, F // 2, 128), u32),
        pltpu.VMEM((F // 128, 128), bf16),
        pltpu.VMEM((S // 128, 128), bf16),
        pltpu.VMEM((1, D), bf16),
        pltpu.VMEM((D, 6 * D), bf16),
        pltpu.VMEM((5, 64, 128), u32),
        pltpu.VMEM((5, 64, 128), u32),
        pltpu.VMEM((NT, 2, 64, 128), u32),
        pltpu.VMEM((NT, 2, 64, 128), u32),
        pltpu.VMEM((6 * D, 128), f32),
        pltpu.VMEM((NT + 1, 5, 64, 128), u32),
        pltpu.VMEM((NT, 2 * NR, 128), f32),
        pltpu.VMEM((NT, 3, NR // 2, 128), u32),
        pltpu.VMEM((2 * NR, 128), f32),
        pltpu.VMEM((NT, 8, 128), f32),
        pltpu.VMEM((4, NT, 8, 128), f32),
        pltpu.VMEM((NT, 2 * NR, 128), f32),
        pltpu.VMEM((NT, D, 128), f32),
        pltpu.VMEM((50, 4, H // 2, 128), u32),
        pltpu.VMEM((49, NF, H // 2, 128), u32),
        pltpu.VMEM((NT, D // 2, 128), u32),
        pltpu.SMEM((8,), jnp.int32),
        pltpu.SemaphoreType.DMA((25,)),
        pltpu.SemaphoreType.DMA((NF,)),
        pltpu.SemaphoreType.DMA((NS,)),
        pltpu.SemaphoreType.DMA((NS,)),
    ]
    outT = pl.pallas_call(
        functools.partial(_kernel, scopes=False, opt={}),
        out_shape=jax.ShapeDtypeStruct((D, S), bf16),
        in_specs=[any_spec] * 13,
        out_specs=any_spec,
        scratch_shapes=scratch,
        compiler_params=pltpu.CompilerParams(vmem_limit_bytes=120 * 1024 * 1024),
        name="adaln_gfnet_mixer",
    )(np.array([1, 0, 0, 0, 0, 0, 0, 0], np.int32), A_x[0].T, A_w_r.T, A_w_i.T, B_w1, B_b1.reshape(F // 128, 128), B_w2,
      B_b2.reshape(S // 128, 128), c, w_mod, _DFWD, _DINV, _SMAT)
    return outT.T[None]
```

```python
import contextlib
import functools

import jax
import jax.numpy as jnp
import numpy as np
import ml_dtypes
import jax.experimental.pallas as pl
import jax.experimental.pallas.tpu as pltpu

S, D, F = 2048, 576, 4608
NT = S // 128
NP = 19
NR = NP * 16
H = D // 4
f32, bf16, u32 = jnp.float32, jnp.bfloat16, jnp.uint32
EPS = 1e-5

_TH = 2 * np.pi / 9
C1, C2, C4 = float(np.cos(_TH)), float(np.cos(2 * _TH)), float(np.cos(4 * _TH))
S1, S3, S4 = float(np.sin(_TH)), float(np.sin(3 * _TH)), float(np.sin(4 * _TH))


_SETS = [[g, g + 9, 9 - g, 18 - g] for g in range(1, 5)] + [[0, 9, 288]]
_FLAT = [c for grp in _SETS for c in grp]


def _row_pairs(m):
    bits = m.astype(ml_dtypes.bfloat16).view(np.uint16).astype(np.uint32)
    return bits[..., 0::2, :] | (bits[..., 1::2, :] << 16)


def _d_mats():
    d2 = np.arange(64)
    fwd = np.zeros((5, 128, 128))
    inv = np.zeros((5, 128, 128))
    col = 16 * (d2 // 8) + 2 * (d2 % 8)
    for g, grp in enumerate(_SETS):
        res = (g + 1) % 5
        scale = (0.0, S1, S1, S3, S1)[res]
        for cc, c0 in enumerate(grp):
            for m in range(1 if c0 == 288 else 16):
                kx = c0 + 18 * m
                ph = 2 * np.pi * ((kx * d2) % D) / D
                c, s = np.cos(ph), np.sin(ph)
                if kx % 288 == 0:
                    s = np.zeros_like(s)
                sg = (1.0 if kx % 9 == res else -1.0) * scale
                row = 32 * cc + 16 * (m % 2) + m // 2
                fwd[g, row, col] = c
                fwd[g, row + 8, col] = -s
                fwd[g, row, col + 1] = -sg * s
                fwd[g, row + 8, col + 1] = -sg * c
                w = (1.0 if kx % 288 == 0 else 2.0) / (S * D)
                k = 32 * cc + 2 * (2 * (m % 8) + m // 8)
                inv[g, d2, k] = w * c
                inv[g, d2, k + 1] = -w * s
                inv[g, 64 + d2, k] = sg * w * s
                inv[g, 64 + d2, k + 1] = sg * w * c
    return _row_pairs(fwd), _row_pairs(inv)


def _s_mats():
    m = np.zeros((NT, 2, 128, 128))
    lane = np.arange(128)
    for b in range(NT):
        a = (lane - b) % 16
        k = 128 * a + (lane - a) % 128
        ph = 2 * np.pi * ((lane[:, None] * k[None, :]) % S) / S
        m[b] = np.cos(ph), -np.sin(ph)
    return _row_pairs(m)


_DFWD, _DINV = _d_mats()
_SMAT = _s_mats()


def _as_bf16(x):
    return pltpu.bitcast(x, bf16)


def _dot(a, b):
    return jnp.dot(a, b, preferred_element_type=f32)


def _dot_t(a, b):
    return jax.lax.dot_general(a, b, (((1,), (1,)), ((), ())), preferred_element_type=f32)


def _pack(a, b):
    return pltpu.pack_elementwise([a, b], packed_dtype=bf16)


def _unpack(x, i):
    return pltpu.unpack_elementwise(x, index=i, packed_dtype=bf16, unpacked_dtype=f32)


def _radix9_fwd(a):
    p = [None] + [a[n] + a[9 - n] for n in range(1, 5)]
    m = [None] + [a[n] - a[9 - n] for n in range(1, 5)]
    t = p[1] + p[2] + p[4]
    u = a[0] + p[3]
    b = a[0] - 0.5 * p[3]
    e1 = p[1] - p[4]
    e2 = p[2] - p[4]
    r1 = C1 * e1 + C2 * e2
    r2 = C2 * e1 + C4 * e2
    f1 = m[1] + m[2]
    f2 = m[2] + m[4]
    f3 = m[1] - m[4]
    q1 = f1 + (S4 / S1) * f2
    q2 = f3 + (S4 / S1) * f1
    n3 = (S3 / S1) * m[3]
    return u + t, [(b + r1, q1 + n3), (b + r2, q2 - n3), (u - 0.5 * t, m[1] - m[2] + m[4]),
                   (b - (r1 + r2), (q2 - q1) + n3)]


def _radix9_inv(v0, v):
    (r1_, i1), (r2_, i2), (r3_, i3), (r4_, i4) = v
    t = r1_ + r2_ + r4_
    u = v0 + r3_
    b = v0 - 0.5 * r3_
    e1 = r1_ - r4_
    e2 = r2_ - r4_
    r1 = C1 * e1 + C2 * e2
    r2 = C2 * e1 + C4 * e2
    a1, a2, a3, a4 = b + r1, b + r2, u - 0.5 * t, b - (r1 + r2)
    f1 = i1 + i2
    f2 = i2 + i4
    f3 = i1 - i4
    q1 = f1 + (S4 / S1) * f2
    q2 = f3 + (S4 / S1) * f1
    b1, b2, b4 = q1 + i3, q2 - i3, (q2 - q1) + i3
    b3 = (S3 / S1) * (i1 - i2 + i4)
    return [u + t, a1 - b1, a2 - b2, a3 - b3, a4 - b4, a4 + b4, a3 + b3, a2 + b2, a1 + b1]


def _bfly4(a, b, c, d, sgn, c_rot=False):
    if c_rot:
        if sgn < 0:
            t0 = (a[0] + c[1], a[1] - c[0])
            t1 = (a[0] - c[1], a[1] + c[0])
        else:
            t0 = (a[0] - c[1], a[1] + c[0])
            t1 = (a[0] + c[1], a[1] - c[0])
    else:
        t0 = (a[0] + c[0], a[1] + c[1])
        t1 = (a[0] - c[0], a[1] - c[1])
    t2 = (b[0] + d[0], b[1] + d[1])
    t3 = (b[0] - d[0], b[1] - d[1])
    x0 = (t0[0] + t2[0], t0[1] + t2[1])
    x2 = (t0[0] - t2[0], t0[1] - t2[1])
    xm = (t1[0] + t3[1], t1[1] - t3[0])
    xp = (t1[0] - t3[1], t1[1] + t3[0])
    return [x0, xm, x2, xp] if sgn < 0 else [x0, xp, x2, xm]


def _tw16(z, e, sgn):
    c = float(np.cos(2 * np.pi * e / 16))
    s = float(sgn * np.sin(2 * np.pi * e / 16))
    x, y = z
    if e % 2 == 0:
        if (c > 0) == (s > 0):
            return ((x - y) * c, (x + y) * c)
        return ((x + y) * c, (y - x) * c)
    return (x * c - y * s, x * s + y * c)


def _radix16(x, sgn):
    u = [_bfly4(x[n2], x[4 + n2], x[8 + n2], x[12 + n2], sgn) for n2 in range(4)]
    out = [None] * 16
    for k1 in range(4):
        v = []
        for n2 in range(4):
            e = k1 * n2
            v.append(u[n2][k1] if e % 4 == 0 else _tw16(u[n2][k1], e, sgn))
        y = _bfly4(v[0], v[1], v[2], v[3], sgn, c_rot=(k1 == 2))
        for k2 in range(4):
            out[k1 + 4 * k2] = y[k2]
    return out


def _sa(a11, a12, a21, a22):
    return [a11 + a22, a21 + a22, a11, a22, a11 + a12, a21 - a11, a12 - a22]


def _sb(b11, b12, b21, b22):
    return [b11 + b22, b11, b12 - b22, b21 - b11, b22, b11 + b12, b21 + b22]


def _sc(m):
    m1, m2, m3, m4, m5, m6, m7 = m
    return [m4 + m7 - m5 + m1, m5 + m3, m2 + m4, m1 - m2 + m3 + m6]


def _sa2(blk):
    lvl = [_sa(blk[ri][ci], blk[ri][2 + ci], blk[2 + ri][ci], blk[2 + ri][2 + ci])
           for ri in range(2) for ci in range(2)]
    return [x for o in range(7) for x in _sa(*[l[o] for l in lvl])]


def _sc2(m):
    p = [_sc(m[7 * o:7 * o + 7]) for o in range(7)]
    out = [[None] * 4 for _ in range(4)]
    for ii in range(4):
        for oi, v in enumerate(_sc([p[o][ii] for o in range(7)])):
            out[2 * (oi // 2) + ii // 2][2 * (oi % 2) + ii % 2] = v
    return out


_SB_TERMS = (((1, 0, 0), (1, 1, 1)), ((1, 0, 0),), ((1, 0, 1), (-1, 1, 1)), ((1, 1, 0), (-1, 0, 0)),
             ((1, 1, 1),), ((1, 0, 0), (1, 0, 1)), ((1, 1, 0), (1, 1, 1)))
_ORDER = (1, 3, 6, 4, 0, 2, 5)


def _strassen2(lhs, raw, hook=None, outer=_ORDER, inner=_ORDER):
    m = [None] * 49
    done = 0
    for o in outer:
        blocks = {}
        halves = []
        for h in range(2):
            quad = []
            for ri in range(2):
                for ci in range(2):
                    acc = None
                    for sg, ro, co in _SB_TERMS[o]:
                        key = (2 * ro + ri, 2 * co + ci)
                        if key not in blocks:
                            blocks[key] = raw(o, *key)
                        v = _unpack(blocks[key], h)
                        acc = v if acc is None else (acc + v if sg > 0 else acc - v)
                    quad.append(acc)
            halves.append(_sb(*quad))
        for j in inner:
            if hook is not None:
                hook(done)
            done += 1
            rhs = pltpu.bitcast(_pack(halves[0][j], halves[1][j]), bf16)
            m[7 * o + j] = _dot(lhs(7 * o + j), rhs)
    return m


def _gelu2(u):
    k0 = 0.7978845608028654
    z = u * (k0 + (k0 * 0.044715) * (u * u))
    return u * jnp.tanh(z) + u


def _tree(vs):
    vs = list(vs)
    while len(vs) > 1:
        vs = [vs[i] + vs[i + 1] if i + 1 < len(vs) else vs[i] for i in range(0, len(vs), 2)]
    return vs[0]


def _colsum(vs, lanes=4):
    accs = []
    for k in range(lanes):
        acc = None
        for v in vs[k::lanes]:
            acc = v if acc is None else acc + v
        accs.append(acc)
    return jnp.sum(_tree(accs), axis=0, keepdims=True)


def _interleave(*lists):
    items = []
    for ci, lst in enumerate(lists):
        for k, it in enumerate(lst):
            items.append(((k + 0.5) / len(lst), ci, k, it))
    items.sort(key=lambda x: x[:3])
    for x in items:
        x[3]()


FC = 512
NF = F // FC
SC = 512
NS = S // SC
XC = 8
WSPLIT = (0, 96, 192, 289)


def _kernel(z_h, xT_h, wr_h, wi_h, w1_h, b1_h, w2_h, b2_h, c_h, wm_h, df_h, di_h, sm_h, out_h,
            xw, xT, wraw_r, wraw_i, wp, w1v, w2v, b1v, b2v, cv, wm, df, di, sm, sm3, tbl, ybuf, xbuf, cbuf, sab,
            mnb, stat, zbuf, x1, aop, gop, obuf, zsm, sem, w1sem, w2sem, osem, *, scopes, opt):
    n = [0]

    def scope(name):
        return jax.named_scope(name) if scopes else contextlib.nullcontext()

    def cp(src, dst):
        d = pltpu.make_async_copy(src, dst, sem.at[n[0]])
        n[0] += 1
        return d

    cp_c = cp(c_h, cv)
    cp_wm0 = cp(wm_h.at[:, 512:1152], wm.at[:, 512:1152])
    xsem = n[0]
    cp_x = [cp(xT_h.at[:, i * 256:(i + 1) * 256], xw.at[i]) for i in range(NT // 2)]
    cp_z = cp(z_h, zsm)
    cp_df = cp(df_h, df)
    cp_sm = cp(sm_h, sm)
    cp_w = [[cp(src.at[lo:hi], dst.at[lo:hi]) for src, dst in ((wr_h, wraw_r), (wi_h, wraw_i))]
            for lo, hi in zip(WSPLIT[:-1], WSPLIT[1:])]
    cp_wms = cp(wm_h.at[:, 0:512], wm.at[:, 0:512])
    cp_di = cp(di_h, di)
    cp_wm1 = cp(wm_h.at[:, 1152:2944], wm.at[:, 1152:2944])
    cp_wm2 = cp(wm_h.at[:, 2944:6 * D], wm.at[:, 2944:6 * D])
    cp_b1 = cp(b1_h, b1v)
    cp_b2 = cp(b2_h, b2v)

    def strip(src, dst, sems, j):
        cols = pl.ds(pl.multiple_of(j * 128, 128), 128)
        return pltpu.make_async_copy(src.at[:, cols], dst.bitcast(bf16).at[j], sems.at[j // 4])

    cp_w1 = [strip(w1_h, w1v, w1sem, j) for j in range(F // 128)]
    cp_w2 = [strip(w2_h, w2v, w2sem, j) for j in range(NT)]

    for d in [cp_c, cp_wm0, *cp_x, cp_z, cp_df, cp_sm, *sum(cp_w, []), cp_wms, cp_di, cp_wm1, cp_b1, cp_b2]:
        d.start()

    cp_c.wait()
    cc = cv[...].astype(f32)
    sc = jnp.broadcast_to(cc * jax.nn.sigmoid(cc), (16, D)).astype(bf16)

    def mod_items(lo, hi):
        box = []

        def first():
            box.append(_dot(sc, wm[:, lo:hi]))

        def tile(j):
            r0 = lo + j * 128
            row = box[0][0:1, j * 128:(j + 1) * 128]
            col = r0 + jax.lax.broadcasted_iota(jnp.int32, (1, 128), 1)
            is_scale = ((col >= D) & (col < 2 * D)) | ((col >= 4 * D) & (col < 5 * D))
            row = row * jnp.where(col >= 5 * D, 0.5, 1.0) + jnp.where(is_scale, 1.0, 0.0)
            tbl[r0:r0 + 128, :] = jnp.broadcast_to(row, (128, 128)).T

        return [first] + [functools.partial(tile, j) for j in range((hi - lo) // 128)]

    with scope("wait_wm0"):
        cp_wm0.wait()
    with scope("mod0"):
        for it in mod_items(512, 1152):
            it()

    ones = jnp.ones((16, D), bf16)
    rsq = lambda v: jax.lax.rsqrt(v + EPS)

    def finish(k, fn):
        for t in range(NT):
            stat[k, t] = jnp.broadcast_to(fn(jnp.sum(stat[k, t], axis=0, keepdims=True) * (1.0 / D)), (8, 128))

    def x_rows(t, r):
        v = pltpu.bitcast(xT[t, 8 * (r // 2):8 * (r // 2) + 8, :], bf16).astype(f32)
        return v[8 * (r % 2):8 * (r % 2) + 8]

    def b_mean(tp, k):
        t = 2 * tp + k
        xs = []
        for r in range(D // 16):
            v = xw[tp, 16 * r:16 * r + 16, 128 * k:128 * k + 128]
            xT[t, 8 * r:8 * r + 8, :] = pltpu.bitcast(v, u32)
            v = v.astype(f32)
            xs += [v[0:8], v[8:16]]
        mnb[t] = jnp.broadcast_to(_colsum(xs, 3) * (1.0 / D), (8, 128))

    def radix9_store(t, load):
        for j in range(8):
            y0, ys = _radix9_fwd([load(8 * n9 + j) for n9 in range(9)])
            ybuf[t, 4, 8 * j:8 * j + 8, :] = _pack(y0, jnp.zeros_like(y0))
            for g in range(4):
                ybuf[t, g, 8 * j:8 * j + 8, :] = _pack(*ys[g])

    def b_vpu(t):
        mean = mnb[t]
        accs = [None] * 3

        def load(r):
            xc = x_rows(t, r) - mean
            k = (r // 8) % 3
            accs[k] = xc * xc if accs[k] is None else accs[k] + xc * xc
            return xc * tbl[D + 8 * r:D + 8 * r + 8, :]

        radix9_store(t, load)
        stat[0, t] = _tree(accs)

    def b_pair(tp, _):
        pltpu.make_async_copy(xT_h.at[:, 0:256], xw.at[tp], sem.at[xsem + tp]).wait()
        b_mean(tp, 0)
        b_mean(tp, 1)
        b_vpu(2 * tp)
        b_vpu(2 * tp + 1)

    with scope("B"):
        jax.lax.fori_loop(0, NT // 2, b_pair, None)
    finish(0, rsq)
    for d in cp_w1:
        d.start()

    def d_fwd(g, t):
        rows = 128 if g < 4 else 80
        return _dot(_as_bf16(df[g, 0:rows // 2, :]), _as_bf16(ybuf[t, g]))

    def phase_c():
        for g, grp in enumerate(_SETS):
            for cc, c0 in enumerate(grp):
                nr = 16 if c0 == 288 else 32
                z = zero[cc]
                xs = [_dot(_as_bf16(df[g, 16 * cc:16 * cc + nr // 2, :]), _as_bf16(ybuf[t + z, g])) for t in range(NT)]
                y = [_radix16([(xs[t][r0:r0 + 8] * stat[0, t], xs[t][r0 + 8:r0 + 16] * stat[0, t])
                               for t in range(NT)], -1) for r0 in range(0, nr, 16)]
                rows = slice(8 * (4 * g + cc), 8 * (4 * g + cc) + 8)
                for b in range(NT):
                    (er, ei), (odr, odi) = y[0][b], y[-1][b]
                    cbuf[b, 0, rows, :] = _pack(er + ei, odr + odi)
                    cbuf[b, 1, rows, :] = _pack(er, odr)
                    cbuf[b, 2, rows, :] = _pack(ei, odi)

    P = functools.partial
    qs = lambda g: range(8 * g, min(8 * g + 8, 2 * NP - 1))

    def region(fn):
        jax.lax.fori_loop(0, one, lambda i, _: fn(), None)

    cp_z.wait()
    one = jnp.minimum(zsm[0], 1)
    zero = [zsm[1 + k] for k in range(7)]
    cp_df.wait()
    with scope("C"):
        region(phase_c)

    def sa_items():
        def last():
            for g, grp in enumerate(_SETS):
                r = d_fwd(g, NT) * float(S)
                for cc, c0 in enumerate(grp):
                    for par in range(2):
                        r0 = 32 * cc + (0 if c0 == 288 else 16 * par)
                        for ri in range(2):
                            sab[pl.ds(ri * NR + 16 * (4 * g + cc) + par, 8, stride=2), :] = r[r0 + 8 * ri:r0 + 8 * ri + 8]
        return mod_items(0, 512) + [lambda: radix9_store(NT, lambda r: tbl[8 * r:8 * r + 8, :]), last]

    lane = jax.lax.broadcasted_iota(jnp.int32, (8, 128), 1)
    masks = [(lane & (1 << b)) != 0 for b in range(4)]

    def shuffle(vals):
        vals = [pltpu.roll(v, a, 1) if a else v for a, v in enumerate(vals)]
        vals = [vals[(-b) % 16] for b in range(16)]
        for b in range(4):
            vals = [jnp.where(masks[b], vals[(i - (1 << b)) % 16], vals[i]) for i in range(16)]
        return vals

    def w_rows(p, raw, r):
        if r < 18:
            vals = shuffle([pltpu.bitcast(raw[16 * r:16 * r + 16, a * 128:(a + 1) * 128], u32) for a in range(16)])
        else:
            last = jnp.broadcast_to(raw[288:289, :].astype(f32), (8, S))
            vals = shuffle([pltpu.bitcast(last[:, a * 128:(a + 1) * 128], u32) for a in range(16)])
        for b in range(16):
            wp[p, b, 8 * r:8 * r + 8, :] = vals[b]

    def phase_d1(b):
        fr, fi = sm[b, 0], sm[b, 1]
        dif = _pack(*[_unpack(fi, h) - _unpack(fr, h) for h in range(2)])
        tot = _pack(*[_unpack(fr, h) + _unpack(fi, h) for h in range(2)])
        sm3[b, 0] = dif
        sm3[b, 1] = tot
        k = [_dot(_as_bf16(cbuf[b, p]), _as_bf16(m)) for p, m in enumerate((fr, dif, tot))]
        xbuf[b, 0:NR, :] = k[0] - k[2]
        xbuf[b, NR:2 * NR, :] = k[0] + k[1]

    def w_group(p, b, c0, mh):
        if c0 == 288:
            return pltpu.bitcast(wp[p, b, 144:152, :], f32)
        return _unpack(wp[p, b, pl.ds(c0 // 2 + 72 * mh, 8, stride=9), :], c0 % 2)

    def phase_d2(b):
        zs = [[], [], []]
        for p, c0 in enumerate(_FLAT):
            z = []
            for mh in range(1 if c0 == 288 else 2):
                r0 = 16 * p + 8 * mh
                xr, xi = xbuf[b, r0:r0 + 8, :], xbuf[b, NR + r0:NR + r0 + 8, :]
                if b == 0:
                    xr = xr + jnp.where(lane == 0, sab[r0:r0 + 8, :], 0.0)
                    xi = xi + jnp.where(lane == 0, sab[NR + r0:NR + r0 + 8, :], 0.0)
                wr, wi = w_group(0, b, c0, mh), w_group(1, b, c0, mh)
                zr, zi = xr * wr - xi * wi, xr * wi + xi * wr
                z.append((zr + zi, zr, zi))
            for k in range(3):
                zs[k].append(_pack(z[0][k], z[-1][k]))
        k = [_dot_t(_as_bf16(jnp.concatenate(z, axis=0)), _as_bf16(m))
             for z, m in zip(zs, (sm[b, 0], sm3[b, 1], sm3[b, 0]))]
        zbuf[b, 0:NR, :] = k[0] + k[2]
        zbuf[b, NR:2 * NR, :] = k[0] - k[1]

    def w_items(i):
        rows = range(WSPLIT[i] // 16, -(-WSPLIT[i + 1] // 16))
        return [P(w_rows, p, raw, r) for r in rows for p, raw in enumerate((wraw_r, wraw_i))]

    ds1 = opt.get("ds1", (0, 8, 13, 16))
    cp_sm.wait()
    for i in range(len(ds1) - 1):
        with scope("wait_w"):
            for d in cp_w[i]:
                d.wait()
        with scope("D1"):
            region(lambda: _interleave([P(phase_d1, b) for b in range(ds1[i], ds1[i + 1])], w_items(i)))
    with scope("wait_wms"):
        cp_wms.wait()
    with scope("D2"):
        def phase_d():
            _interleave([P(phase_d2, b) for b in range(NT - 1, 0, -1)], sa_items())
            phase_d2(0)
        region(phase_d)
    with scope("wait_wm1"):
        cp_di.wait()
        cp_wm1.wait()
    for d in [cp_wm2] + cp_w2:
        d.start()

    def phase_e(q):
        r0 = 8 * q
        y = _radix16([(zbuf[b, r0:r0 + 8, :], zbuf[b, NR + r0:NR + r0 + 8, :]) for b in range(NT)], 1)
        for t in range(NT):
            ybuf[t + zero[0], q // 8, (q % 8) * 8:(q % 8) * 8 + 8, :] = _pack(*y[t])

    def f_mxu(g, t):
        if g < 4:
            xbuf[t, 128 * g:128 * (g + 1), :] = _dot(_as_bf16(di[g]), _as_bf16(ybuf[t, g]))
        else:
            xbuf[t, 512:576, :] = _dot(_as_bf16(di[4, 0:32, :])[:, 0:80], _as_bf16(ybuf[t, 4, 0:40, :]))

    def phase_ef():
        _interleave([P(phase_e, q) for q in qs(4)], mod_items(1152, 2944))
        for g in range(4):
            _interleave([P(f_mxu, (g - 1) % 5, t) for t in range(NT)], [P(phase_e, q) for q in qs(g)])
        _interleave([P(f_mxu, 3, t) for t in range(NT)], [center_sb])

    def center_sb():
        sb = [tbl[3 * D + 8 * r:3 * D + 8 * r + 8, :] for r in range(D // 8)]
        sbm = _colsum(sb) * (1.0 / D)
        for r in range(D // 8):
            sab[8 * r:8 * r + 8, :] = sb[r] - sbm

    with scope("E"):
        region(phase_ef)

    def f_p1(t, _):
        accs = [None] * 3
        for j in range(8):
            v = [(xbuf[t, 128 * g + 8 * j:128 * g + 8 * j + 8, :],
                  xbuf[t, 128 * g + 64 + 8 * j:128 * g + 72 + 8 * j, :]) for g in range(4)]
            ys = _radix9_inv(xbuf[t, 512 + 8 * j:520 + 8 * j, :], v)
            for n9 in range(9):
                r = 8 * n9 + j
                xv = x_rows(t, r) + ys[n9] * tbl[2 * D + 8 * r:2 * D + 8 * r + 8, :]
                x1[t, 8 * r:8 * r + 8, :] = xv
                accs[n9 % 3] = xv if accs[n9 % 3] is None else accs[n9 % 3] + xv
        stat[0, t] = _tree(accs)

    def f_p2(t, _):
        mean = stat[0, t]
        a2 = [None] * 2
        az = [None] * 2
        for r in range(D // 8):
            xc = x1[t, 8 * r:8 * r + 8, :] - mean
            z = xc * tbl[4 * D + 8 * r:4 * D + 8 * r + 8, :]
            xbuf[t, 8 * r:8 * r + 8, :] = z
            k = r % 2
            a2[k] = xc * xc if a2[k] is None else a2[k] + xc * xc
            az[k] = z if az[k] is None else az[k] + z
        stat[1, t] = _tree(a2)
        stat[2, t] = _tree(az)

    def f_p3(t, _):
        rs = stat[1, t]
        mz = stat[2, t]
        a2 = [None] * 2
        for r in range(D // 8):
            dv = (xbuf[t, 8 * r:8 * r + 8, :] - mz) * rs + sab[8 * r:8 * r + 8, :]
            zbuf[t, pl.ds(16 * (r // 2) + r % 2, 8, stride=2), :] = dv
            k = r % 2
            a2[k] = dv * dv if a2[k] is None else a2[k] + dv * dv
        stat[3, t] = _tree(a2)

    with scope("F1"):
        jax.lax.fori_loop(0, NT, f_p1, None, unroll=2)
        finish(0, lambda v: v)
    with scope("F2"):
        jax.lax.fori_loop(0, NT, f_p2, None, unroll=2)
        finish(1, rsq)
        finish(2, lambda v: v)
    with scope("F3"):
        jax.lax.fori_loop(0, NT, f_p3, None, unroll=2)
        finish(3, rsq)

    cp_b1.wait()
    cp_b2.wait()
    tbl[0:40, :] = jnp.concatenate([b1v[...].astype(f32), jnp.zeros((4, 128), f32)], axis=0)
    tbl[40:56, :] = b2v[...].astype(f32) * 2.0

    def bias(r):
        return jnp.broadcast_to(tbl[pl.ds(r, 1), :], (8, 128))

    def left_rows(block, dst, slot, r0):
        ops = [_sa2([[block(r, c, r0 + 8 * h) for c in range(4)] for r in range(4)]) for h in range(2)]
        out = [_pack(ops[0][j], ops[1][j]) for j in range(49)]
        for j in range(49):
            dst[j, slot, r0 // 2:r0 // 2 + 8, :] = out[j]
        return out

    def f_p4(k, _):
        rs = [stat[3, 4 * k + c] for c in range(4)]
        for r0 in range(0, H, 16):
            left_rows(lambda r, c, row: zbuf[4 * k + c, r * H + row:r * H + row + 8, :] * rs[c], aop, k, r0)

    with scope("F4"):
        jax.lax.fori_loop(0, NT // 4, f_p4, None)

    def wait_w(src, dst, sems, i):
        view = dst.at[pl.ds(4 * i, 4)]
        pltpu.make_async_copy(view, view, sems.at[i]).wait()

    def hidden_rows(i, r0):
        return left_rows(lambda r, c, row: _gelu2(xbuf[4 * r + c, row:row + 8, :] + bias(4 * i + c)), gop, i, r0)

    def mlp1_chunk(i):
        prev = jnp.where(i == 0, NF - 1, i - 1)
        first, step = opt.get("h0", 1), opt.get("h1", 2)

        def hook(n):
            if n >= first and (n - first) % step == 0 and (n - first) // step < H // 16:
                r0 = 16 * ((n - first) // step)
                out = hidden_rows(prev, r0)
                tok = out[opt.get("tk", (0,))[0]]
                for j in opt.get("tk", (0,))[1:]:
                    tok = tok | out[j]
                aop[49 + zero[0], 0, 0:8, :] = tok

        m = _strassen2(
            lambda j: jnp.concatenate([pltpu.bitcast(aop[j, k], bf16) for k in range(4)], axis=1),
            lambda o, r, c: jnp.concatenate(
                [w1v[4 * i + c + zero[opt.get('zz1', range(7))[o]], 64 * (4 * k + r):64 * (4 * k + r + 1), :] for k in range(4)], axis=0),
            hook, opt.get("oo1", (1, 5, 2, 4, 0, 3, 6)), opt.get("io1", _ORDER))
        u = _sc2(m)
        for r in range(4):
            for c in range(4):
                xbuf[4 * r + c, 0:H, :] = u[r][c]

    u1 = opt.get("u1", 1)

    def mlp1_step(n, _):
        for k in range(u1):
            wait_w(w1_h, w1v, w1sem, u1 * n + k)
        for k in range(u1):
            mlp1_chunk(u1 * n + k)

    with scope("mlp1"):
        jax.lax.fori_loop(0, NF // u1, mlp1_step, None)

    def mlp2(i, lhs):
        m = _strassen2(lhs, lambda o, r, c: jnp.concatenate(
            [w2v[4 * i + c + zero[opt.get('zz2', range(7))[o]], 64 * (4 * k + r):64 * (4 * k + r + 1), :] for k in range(NF)], axis=0),
            None, opt.get("oo2", _ORDER), opt.get("io2", _ORDER))
        y = _sc2(m)
        for ro, co in ((1, 0), (0, 0), (0, 1), (1, 1)):
            for c in (2 * co, 2 * co + 1):
                t = 4 * i + c
                bc = bias(40 + t)
                for r in (2 * ro, 2 * ro + 1):
                    for r0 in range(0, H, 16):
                        row = r * H + r0
                        o = [x1[t, pl.ds(row + h, 8, stride=2), :]
                             + tbl[pl.ds(5 * D + row + h, 8, stride=2), :]
                             * (y[r][c][r0 + 8 * h:r0 + 8 * h + 8] + bc) for h in range(2)]
                        obuf[t, row // 2:row // 2 + 8, :] = _pack(o[0], o[1])
                rows = pl.ds(2 * H * ro, 2 * H)
                cols = pl.ds(pl.multiple_of(t * 128, 128), 128)
                pltpu.make_async_copy(obuf.bitcast(bf16).at[t, rows], out_h.at[rows, cols], osem.at[i]).start()

    def mlp2_first():
        wait_w(w2_h, w2v, w2sem, 0)
        cp_wm2.wait()
        for it in mod_items(2944, 6 * D):
            it()
        for r0 in range(0, H, 16):
            hidden_rows(NF - 1, r0)
        mlp2(0, lambda j: jnp.concatenate([pltpu.bitcast(gop[j, k], bf16) for k in range(NF)], axis=1))

    def mlp2_step(i, _):
        wait_w(w2_h, w2v, w2sem, i)
        mlp2(i, lambda j: jnp.concatenate([pltpu.bitcast(gop[j, k], bf16) for k in range(NF)], axis=1))

    def mlp2_pre():
        cp_wm2.wait()
        _interleave(mod_items(2944, 6 * D), [P(hidden_rows, NF - 1, r0) for r0 in range(0, H, 16)])

    peel = opt.get("peel", 1)
    with scope("mlp2_0"):
        region(mlp2_first if peel else mlp2_pre)
    def mlp2_rest():
        for i in range(1, NS):
            wait_w(w2_h, w2v, w2sem, i)
        for i in range(1, NS):
            mlp2(i, lambda j: jnp.concatenate([pltpu.bitcast(gop[j, k], bf16) for k in range(NF)], axis=1))

    with scope("mlp2"):
        if opt.get("u2", 0):
            region(mlp2_rest)
        else:
            jax.lax.fori_loop(peel, NS, mlp2_step, None)
    for i in range(NS):
        view = obuf.at[pl.ds(4 * i, 4)]
        pltpu.make_async_copy(view, view, osem.at[i]).wait()


@jax.jit
def pallas_adaLN_cond__spectral_gfnet__mixer_token_mlp__prompt_kernel(
    A_x: jax.Array,
    A_w_r: jax.Array,
    A_w_i: jax.Array,
    B_x: jax.Array,
    B_w1: jax.Array,
    B_b1: jax.Array,
    B_w2: jax.Array,
    B_b2: jax.Array,
    c: jax.Array,
    w_mod: jax.Array,
):
    del B_x
    any_spec = pl.BlockSpec(memory_space=pl.ANY)
    scratch = [
        pltpu.VMEM((NT // 2, D, 256), bf16),
        pltpu.VMEM((NT, D // 2, 128), u32),
        pltpu.VMEM((289, S), bf16),
        pltpu.VMEM((289, S), bf16),
        pltpu.VMEM((2, NT, 152, 128), u32),
        pltpu.VMEM((F // 128, S // 2, 128), u32),
        pltpu.VMEM((NT, F // 2, 128), u32),
        pltpu.VMEM((F // 128, 128), bf16),
        pltpu.VMEM((S // 128, 128), bf16),
        pltpu.VMEM((1, D), bf16),
        pltpu.VMEM((D, 6 * D), bf16),
        pltpu.VMEM((5, 64, 128), u32),
        pltpu.VMEM((5, 64, 128), u32),
        pltpu.VMEM((NT, 2, 64, 128), u32),
        pltpu.VMEM((NT, 2, 64, 128), u32),
        pltpu.VMEM((6 * D, 128), f32),
        pltpu.VMEM((NT + 1, 5, 64, 128), u32),
        pltpu.VMEM((NT, 2 * NR, 128), f32),
        pltpu.VMEM((NT, 3, NR // 2, 128), u32),
        pltpu.VMEM((2 * NR, 128), f32),
        pltpu.VMEM((NT, 8, 128), f32),
        pltpu.VMEM((4, NT, 8, 128), f32),
        pltpu.VMEM((NT, 2 * NR, 128), f32),
        pltpu.VMEM((NT, D, 128), f32),
        pltpu.VMEM((50, 4, H // 2, 128), u32),
        pltpu.VMEM((49, NF, H // 2, 128), u32),
        pltpu.VMEM((NT, D // 2, 128), u32),
        pltpu.SMEM((8,), jnp.int32),
        pltpu.SemaphoreType.DMA((25,)),
        pltpu.SemaphoreType.DMA((NF,)),
        pltpu.SemaphoreType.DMA((NS,)),
        pltpu.SemaphoreType.DMA((NS,)),
    ]
    outT = pl.pallas_call(
        functools.partial(_kernel, scopes=False, opt={}),
        out_shape=jax.ShapeDtypeStruct((D, S), bf16),
        in_specs=[any_spec] * 13,
        out_specs=any_spec,
        scratch_shapes=scratch,
        compiler_params=pltpu.CompilerParams(vmem_limit_bytes=120 * 1024 * 1024),
        name="adaln_gfnet_mixer",
    )(np.array([1, 0, 0, 0, 0, 0, 0, 0], np.int32), A_x[0].T, A_w_r.T, A_w_i.T, B_w1, B_b1.reshape(F // 128, 128), B_w2,
      B_b2.reshape(S // 128, 128), c, w_mod, _DFWD, _DINV, _SMAT)
    return outT.T[None]
```

```python
import contextlib
import functools

import jax
import jax.numpy as jnp
import numpy as np
import jax.experimental.pallas as pl
import jax.experimental.pallas.tpu as pltpu

S, D, F = 2048, 576, 4608
NT = S // 128
NP = 19
NR = NP * 16
H = D // 4
f32, bf16, u32 = jnp.float32, jnp.bfloat16, jnp.uint32
EPS = 1e-5

_TH = 2 * np.pi / 9
C1, C2, C4 = float(np.cos(_TH)), float(np.cos(2 * _TH)), float(np.cos(4 * _TH))
S1, S3, S4 = float(np.sin(_TH)), float(np.sin(3 * _TH)), float(np.sin(4 * _TH))


_SETS = [[g, g + 9, 9 - g, 18 - g] for g in range(1, 5)] + [[0, 9, 288]]
_FLAT = [c for grp in _SETS for c in grp]


def _row_pairs(m):
    bits = m.astype(bf16).view(np.uint16).astype(np.uint32)
    return bits[..., 0::2, :] | (bits[..., 1::2, :] << 16)


def _d_mats():
    d2 = np.arange(64)
    fwd = np.zeros((5, 128, 128))
    inv = np.zeros((5, 128, 128))
    col = 16 * (d2 // 8) + d2 % 8
    for g, grp in enumerate(_SETS):
        res = (g + 1) % 5
        scale = (0.0, S1, S1, S3, S1)[res]
        for cc, c0 in enumerate(grp):
            for m in range(1 if c0 == 288 else 16):
                kx = c0 + 18 * m
                ph = 2 * np.pi * ((kx * d2) % D) / D
                c, s = np.cos(ph), np.sin(ph)
                if kx % 288 == 0:
                    s = np.zeros_like(s)
                sg = (1.0 if kx % 9 == res else -1.0) * scale
                row = 32 * cc + 16 * (m // 8) + m % 8
                fwd[g, row, col] = c
                fwd[g, row + 8, col] = -s
                fwd[g, row, col + 8] = -sg * s
                fwd[g, row + 8, col + 8] = -sg * c
                w = (1.0 if kx % 288 == 0 else 2.0) / (S * D)
                inv[g, d2, row] = w * c
                inv[g, d2, row + 8] = -w * s
                inv[g, 64 + d2, row] = sg * w * s
                inv[g, 64 + d2, row + 8] = sg * w * c
    return _row_pairs(fwd), _row_pairs(inv)


def _s_mats():
    m = np.zeros((NT, 2, 128, 128))
    lane = np.arange(128)
    for b in range(NT):
        a = (lane - b) % 16
        k = 128 * a + (lane - a) % 128
        ph = 2 * np.pi * ((lane[:, None] * k[None, :]) % S) / S
        m[b] = np.cos(ph), -np.sin(ph)
    return m.astype(bf16)


_DFWD, _DINV = _d_mats()
_SMAT = _s_mats()


def _as_bf16(x):
    return pltpu.bitcast(x, bf16)


def _dot(a, b):
    return jnp.dot(a, b, preferred_element_type=f32)


def _dot_t(a, b):
    return jax.lax.dot_general(a, b, (((1,), (1,)), ((), ())), preferred_element_type=f32)


def _rows16(a, b):
    return jnp.concatenate([a, b], axis=0).astype(bf16)


def _half(x, i):
    return pltpu.bitcast(x & jnp.uint32(0xFFFF0000) if i else x << 16, f32)


def _radix9_fwd(a):
    p = [None] + [a[n] + a[9 - n] for n in range(1, 5)]
    m = [None] + [a[n] - a[9 - n] for n in range(1, 5)]
    t = p[1] + p[2] + p[4]
    u = a[0] + p[3]
    b = a[0] - 0.5 * p[3]
    e1 = p[1] - p[4]
    e2 = p[2] - p[4]
    r1 = C1 * e1 + C2 * e2
    r2 = C2 * e1 + C4 * e2
    f1 = m[1] + m[2]
    f2 = m[2] + m[4]
    f3 = m[1] - m[4]
    q1 = f1 + (S4 / S1) * f2
    q2 = f3 + (S4 / S1) * f1
    n3 = (S3 / S1) * m[3]
    return u + t, [(b + r1, q1 + n3), (b + r2, q2 - n3), (u - 0.5 * t, m[1] - m[2] + m[4]),
                   (b - (r1 + r2), (q2 - q1) + n3)]


def _radix9_inv(v0, v):
    (r1_, i1), (r2_, i2), (r3_, i3), (r4_, i4) = v
    t = r1_ + r2_ + r4_
    u = v0 + r3_
    b = v0 - 0.5 * r3_
    e1 = r1_ - r4_
    e2 = r2_ - r4_
    r1 = C1 * e1 + C2 * e2
    r2 = C2 * e1 + C4 * e2
    a1, a2, a3, a4 = b + r1, b + r2, u - 0.5 * t, b - (r1 + r2)
    f1 = i1 + i2
    f2 = i2 + i4
    f3 = i1 - i4
    q1 = f1 + (S4 / S1) * f2
    q2 = f3 + (S4 / S1) * f1
    b1, b2, b4 = q1 + i3, q2 - i3, (q2 - q1) + i3
    b3 = (S3 / S1) * (i1 - i2 + i4)
    return [u + t, a1 - b1, a2 - b2, a3 - b3, a4 - b4, a4 + b4, a3 + b3, a2 + b2, a1 + b1]


def _bfly4(a, b, c, d, sgn, c_rot=False):
    if c_rot:
        if sgn < 0:
            t0 = (a[0] + c[1], a[1] - c[0])
            t1 = (a[0] - c[1], a[1] + c[0])
        else:
            t0 = (a[0] - c[1], a[1] + c[0])
            t1 = (a[0] + c[1], a[1] - c[0])
    else:
        t0 = (a[0] + c[0], a[1] + c[1])
        t1 = (a[0] - c[0], a[1] - c[1])
    t2 = (b[0] + d[0], b[1] + d[1])
    t3 = (b[0] - d[0], b[1] - d[1])
    x0 = (t0[0] + t2[0], t0[1] + t2[1])
    x2 = (t0[0] - t2[0], t0[1] - t2[1])
    xm = (t1[0] + t3[1], t1[1] - t3[0])
    xp = (t1[0] - t3[1], t1[1] + t3[0])
    return [x0, xm, x2, xp] if sgn < 0 else [x0, xp, x2, xm]


def _tw16(z, e, sgn):
    c = float(np.cos(2 * np.pi * e / 16))
    s = float(sgn * np.sin(2 * np.pi * e / 16))
    x, y = z
    if e % 2 == 0:
        if (c > 0) == (s > 0):
            return ((x - y) * c, (x + y) * c)
        return ((x + y) * c, (y - x) * c)
    return (x * c - y * s, x * s + y * c)


def _radix16(x, sgn):
    u = [_bfly4(x[n2], x[4 + n2], x[8 + n2], x[12 + n2], sgn) for n2 in range(4)]
    out = [None] * 16
    for k1 in range(4):
        v = []
        for n2 in range(4):
            e = k1 * n2
            v.append(u[n2][k1] if e % 4 == 0 else _tw16(u[n2][k1], e, sgn))
        y = _bfly4(v[0], v[1], v[2], v[3], sgn, c_rot=(k1 == 2))
        for k2 in range(4):
            out[k1 + 4 * k2] = y[k2]
    return out


def _sa(a11, a12, a21, a22):
    return [a11 + a22, a21 + a22, a11, a22, a11 + a12, a21 - a11, a12 - a22]


def _sb(b11, b12, b21, b22):
    return [b11 + b22, b11, b12 - b22, b21 - b11, b22, b11 + b12, b21 + b22]


def _sc(m):
    m1, m2, m3, m4, m5, m6, m7 = m
    return [m4 + m7 - m5 + m1, m5 + m3, m2 + m4, m1 - m2 + m3 + m6]


def _sa2(blk):
    lvl = [_sa(blk[ri][ci], blk[ri][2 + ci], blk[2 + ri][ci], blk[2 + ri][2 + ci])
           for ri in range(2) for ci in range(2)]
    return [x for o in range(7) for x in _sa(*[l[o] for l in lvl])]


def _sc2(m):
    p = [_sc(m[7 * o:7 * o + 7]) for o in range(7)]
    out = [[None] * 4 for _ in range(4)]
    for ii in range(4):
        for oi, v in enumerate(_sc([p[o][ii] for o in range(7)])):
            out[2 * (oi // 2) + ii // 2][2 * (oi % 2) + ii % 2] = v
    return out


_SB_TERMS = (((1, 0, 0), (1, 1, 1)), ((1, 0, 0),), ((1, 0, 1), (-1, 1, 1)), ((1, 1, 0), (-1, 0, 0)),
             ((1, 1, 1),), ((1, 0, 0), (1, 0, 1)), ((1, 1, 0), (1, 1, 1)))
_ORDER = (1, 3, 6, 4, 0, 2, 5)


def _strassen2(lhs, raw, hook=None, outer=_ORDER, inner=_ORDER):
    m = [None] * 49
    done = 0
    for o in outer:
        quad = []
        for ri in range(2):
            for ci in range(2):
                acc = None
                for sg, ro, co in _SB_TERMS[o]:
                    v = raw(o, 2 * ro + ri, 2 * co + ci)
                    acc = v if acc is None else (acc + v if sg > 0 else acc - v)
                quad.append(acc)
        ops = _sb(*quad)
        for j in inner:
            if hook is not None:
                hook(done)
            done += 1
            rhs = ops[j].astype(bf16)
            m[7 * o + j] = _dot(lhs(7 * o + j), rhs)
    return m


def _gelu2(u):
    k0 = 0.7978845608028654
    z = u * (k0 + (k0 * 0.044715) * (u * u))
    return u * jnp.tanh(z) + u


def _tree(vs):
    vs = list(vs)
    while len(vs) > 1:
        vs = [vs[i] + vs[i + 1] if i + 1 < len(vs) else vs[i] for i in range(0, len(vs), 2)]
    return vs[0]


def _colsum(vs, lanes=4):
    accs = []
    for k in range(lanes):
        acc = None
        for v in vs[k::lanes]:
            acc = v if acc is None else acc + v
        accs.append(acc)
    return jnp.sum(_tree(accs), axis=0, keepdims=True)


def _interleave(*lists):
    items = []
    for ci, lst in enumerate(lists):
        for k, it in enumerate(lst):
            items.append(((k + 0.5) / len(lst), ci, k, it))
    items.sort(key=lambda x: x[:3])
    for x in items:
        x[3]()


FC = 512
NF = F // FC
SC = 512
NS = S // SC
XC = 8
WSPLIT = (0, 96, 192, 289)


def _kernel(z_h, xT_h, wr_h, wi_h, w1_h, b1_h, w2_h, b2_h, c_h, wm_h, df_h, di_h, sm_h, out_h,
            xw, xT, wraw_r, wraw_i, wp, w1v, w2v, b1v, b2v, cv, wm, df, di, sm, sm3, tbl, ybuf, xbuf, cbuf, sab,
            mnb, stat, zbuf, x1, aop, gop, obuf, zsm, sem, w1sem, w2sem, osem, *, scopes, opt):
    n = [0]

    def scope(name):
        return jax.named_scope(name) if scopes else contextlib.nullcontext()

    def cp(src, dst):
        d = pltpu.make_async_copy(src, dst, sem.at[n[0]])
        n[0] += 1
        return d

    cp_c = cp(c_h, cv)
    cp_wm0 = cp(wm_h.at[:, 512:1152], wm.at[:, 512:1152])
    xsem = n[0]
    cp_x = [cp(xT_h.at[:, i * 256:(i + 1) * 256], xw.at[i]) for i in range(NT // 2)]
    cp_z = cp(z_h, zsm)
    cp_df = cp(df_h, df)
    cp_sm = cp(sm_h, sm)
    cp_w = [[cp(src.at[lo:hi], dst.at[lo:hi]) for src, dst in ((wr_h, wraw_r), (wi_h, wraw_i))]
            for lo, hi in zip(WSPLIT[:-1], WSPLIT[1:])]
    cp_wms = cp(wm_h.at[:, 0:512], wm.at[:, 0:512])
    cp_di = cp(di_h, di)
    cp_wm1 = cp(wm_h.at[:, 1152:6 * D], wm.at[:, 1152:6 * D])
    cp_b1 = cp(b1_h, b1v)
    cp_b2 = cp(b2_h, b2v)

    def strip(src, dst, sems, j):
        cols = pl.ds(pl.multiple_of(j * 128, 128), 128)
        return pltpu.make_async_copy(src.at[:, cols], dst.at[j], sems.at[j // 4])

    cp_w1 = [strip(w1_h, w1v, w1sem, j) for j in range(F // 128)]
    cp_w2 = [strip(w2_h, w2v, w2sem, j) for j in range(NT)]

    for d in [cp_c, cp_wm0, *cp_x, cp_z, cp_df, cp_sm, *sum(cp_w, []), cp_wms, cp_di, cp_wm1, cp_b1, cp_b2]:
        d.start()

    cp_c.wait()
    cc = cv[...].astype(f32)
    sc = jnp.broadcast_to(cc * jax.nn.sigmoid(cc), (16, D)).astype(bf16)

    def mod_items(lo, hi):
        box = []

        def first():
            box.append(_dot(sc, wm[:, lo:hi]))

        def tile(j):
            r0 = lo + j * 128
            row = box[0][0:1, j * 128:(j + 1) * 128]
            col = r0 + jax.lax.broadcasted_iota(jnp.int32, (1, 128), 1)
            is_scale = ((col >= D) & (col < 2 * D)) | ((col >= 4 * D) & (col < 5 * D))
            row = row * jnp.where(col >= 5 * D, 0.5, 1.0) + jnp.where(is_scale, 1.0, 0.0)
            tbl[r0:r0 + 128, :] = jnp.broadcast_to(row, (128, 128)).T

        return [first] + [functools.partial(tile, j) for j in range((hi - lo) // 128)]

    with scope("wait_wm0"):
        cp_wm0.wait()
    with scope("mod0"):
        for it in mod_items(512, 1152):
            it()

    ones = jnp.ones((16, D), bf16)
    rsq = lambda v: jax.lax.rsqrt(v + EPS)

    def finish(k, fn):
        for t in range(NT):
            stat[k, t] = jnp.broadcast_to(fn(jnp.sum(stat[k, t], axis=0, keepdims=True) * (1.0 / D)), (8, 128))

    def x_rows(t, r):
        v = pltpu.bitcast(xT[t, 8 * (r // 2):8 * (r // 2) + 8, :], bf16).astype(f32)
        return v[8 * (r % 2):8 * (r % 2) + 8]

    def b_mean(tp, k):
        t = 2 * tp + k
        xs = []
        for r in range(D // 16):
            v = xw[tp, 16 * r:16 * r + 16, 128 * k:128 * k + 128]
            xT[t, 8 * r:8 * r + 8, :] = pltpu.bitcast(v, u32)
            v = v.astype(f32)
            xs += [v[0:8], v[8:16]]
        mnb[t] = jnp.broadcast_to(_colsum(xs, 3) * (1.0 / D), (8, 128))

    def radix9_store(t, load):
        for j in range(8):
            y0, ys = _radix9_fwd([load(8 * n9 + j) for n9 in range(9)])
            ybuf[t, 4, 16 * j:16 * j + 16, :] = _rows16(y0, jnp.zeros_like(y0))
            for g in range(4):
                ybuf[t, g, 16 * j:16 * j + 16, :] = _rows16(*ys[g])

    def b_vpu(t):
        mean = mnb[t]
        accs = [None] * 3

        def load(r):
            xc = x_rows(t, r) - mean
            k = (r // 8) % 3
            accs[k] = xc * xc if accs[k] is None else accs[k] + xc * xc
            return xc * tbl[D + 8 * r:D + 8 * r + 8, :]

        radix9_store(t, load)
        stat[0, t] = _tree(accs)

    def b_pair(tp, _):
        pltpu.make_async_copy(xT_h.at[:, 0:256], xw.at[tp], sem.at[xsem + tp]).wait()
        b_mean(tp, 0)
        b_mean(tp, 1)
        b_vpu(2 * tp)
        b_vpu(2 * tp + 1)

    with scope("B"):
        jax.lax.fori_loop(0, NT // 2, b_pair, None)
    finish(0, rsq)
    for d in cp_w1:
        d.start()

    def d_fwd(g, t):
        rows = 128 if g < 4 else 80
        return _dot(_as_bf16(df[g, 0:rows // 2, :]), ybuf[t, g])

    def phase_c():
        span = opt.get("span", 2)
        for g, grp in enumerate(_SETS):
            for c_lo in range(0, len(grp), span):
                sets = grp[c_lo:c_lo + span]
                nr = sum(16 if c0 == 288 else 32 for c0 in sets)
                lhs = _as_bf16(df[g, 16 * c_lo:16 * c_lo + nr // 2, :])
                xs = [_dot(lhs, ybuf[t + (zero[c_lo] if span < 4 else 0), g]) for t in range(NT)]
                for k, c0 in enumerate(sets):
                    y = [_radix16([(xs[t][r0:r0 + 8] * stat[0, t], xs[t][r0 + 8:r0 + 16] * stat[0, t])
                                   for t in range(NT)], -1)
                         for r0 in ((32 * k,) if c0 == 288 else (32 * k, 32 * k + 16))]
                    p = 4 * g + c_lo + k
                    for b in range(NT):
                        (lr, li), (hr, hi) = y[0][b], y[-1][b]
                        cbuf[b, 0, 16 * p:16 * p + 16, :] = _rows16(lr + li, hr + hi)
                        cbuf[b, 1, 16 * p:16 * p + 16, :] = _rows16(lr, hr)
                        cbuf[b, 2, 16 * p:16 * p + 16, :] = _rows16(li, hi)

    P = functools.partial
    qs = lambda g: range(8 * g, min(8 * g + 8, 2 * NP - 1))

    def region(fn):
        jax.lax.fori_loop(0, one, lambda i, _: fn(), None)

    cp_z.wait()
    one = jnp.minimum(zsm[0], 1)
    zero = [zsm[1 + k] for k in range(7)]
    cp_df.wait()
    with scope("C"):
        region(phase_c)

    def sa_items():
        def last():
            for g, grp in enumerate(_SETS):
                r = d_fwd(g, NT) * float(S)
                for cc, c0 in enumerate(grp):
                    for mh in range(1 if c0 == 288 else 2):
                        for ri in range(2):
                            src, dst = 32 * cc + 16 * mh + 8 * ri, ri * NR + 16 * (4 * g + cc) + 8 * mh
                            sab[dst:dst + 8, :] = r[src:src + 8]
        return mod_items(0, 512) + [lambda: radix9_store(NT, lambda r: tbl[8 * r:8 * r + 8, :]), last]

    lane = jax.lax.broadcasted_iota(jnp.int32, (8, 128), 1)
    masks = [(lane & (1 << b)) != 0 for b in range(4)]

    def shuffle(vals):
        vals = [pltpu.roll(v, a, 1) if a else v for a, v in enumerate(vals)]
        vals = [vals[(-b) % 16] for b in range(16)]
        for b in range(4):
            vals = [jnp.where(masks[b], vals[(i - (1 << b)) % 16], vals[i]) for i in range(16)]
        return vals

    def w_rows(p, raw, r):
        if r < 18:
            vals = shuffle([pltpu.bitcast(raw[16 * r:16 * r + 16, a * 128:(a + 1) * 128], u32) for a in range(16)])
        else:
            last = jnp.broadcast_to(raw[288:289, :].astype(f32), (8, S))
            vals = shuffle([pltpu.bitcast(last[:, a * 128:(a + 1) * 128], u32) for a in range(16)])
        for b in range(16):
            wp[p, b, 8 * r:8 * r + 8, :] = vals[b]

    def phase_d1(b):
        fr, fi = sm[b, 0], sm[b, 1]
        dif = (fi.astype(f32) - fr.astype(f32)).astype(bf16)
        tot = (fr.astype(f32) + fi.astype(f32)).astype(bf16)
        sm3[b, 0] = dif
        sm3[b, 1] = tot
        k = [_dot(cbuf[b, p], m) for p, m in enumerate((fr, dif, tot))]
        xbuf[b, 0:NR, :] = k[0] - k[2]
        xbuf[b, NR:2 * NR, :] = k[0] + k[1]

    def w_group(p, b, c0, mh):
        if c0 == 288:
            return pltpu.bitcast(wp[p, b, 144:152, :], f32)
        return _half(wp[p, b, pl.ds(c0 // 2 + 72 * mh, 8, stride=9), :], c0 % 2)

    def phase_d2(b):
        zs = [[], [], []]
        for p, c0 in enumerate(_FLAT):
            z = []
            for mh in range(1 if c0 == 288 else 2):
                r0 = 16 * p + 8 * mh
                xr, xi = xbuf[b, r0:r0 + 8, :], xbuf[b, NR + r0:NR + r0 + 8, :]
                if b == 0:
                    xr = xr + jnp.where(lane == 0, sab[r0:r0 + 8, :], 0.0)
                    xi = xi + jnp.where(lane == 0, sab[NR + r0:NR + r0 + 8, :], 0.0)
                wr, wi = w_group(0, b, c0, mh), w_group(1, b, c0, mh)
                zr, zi = xr * wr - xi * wi, xr * wi + xi * wr
                z.append((zr + zi, zr, zi))
            for k in range(3):
                zs[k] += [z[0][k], z[-1][k]]
        k = [_dot_t(jnp.concatenate(z, axis=0).astype(bf16), m)
             for z, m in zip(zs, (sm[b, 0], sm3[b, 1], sm3[b, 0]))]
        zbuf[b, 0:NR, :] = k[0] + k[2]
        zbuf[b, NR:2 * NR, :] = k[0] - k[1]

    def w_items(i):
        rows = range(WSPLIT[i] // 16, -(-WSPLIT[i + 1] // 16))
        return [P(w_rows, p, raw, r) for r in rows for p, raw in enumerate((wraw_r, wraw_i))]

    ds1 = opt.get("ds1", (0, 8, 13, 16))
    cp_sm.wait()
    for i in range(len(ds1) - 1):
        with scope("wait_w"):
            for d in cp_w[i]:
                d.wait()
        with scope("D1"):
            region(lambda: _interleave([P(phase_d1, b) for b in range(ds1[i], ds1[i + 1])], w_items(i)))
    with scope("wait_wms"):
        cp_wms.wait()
    with scope("D2"):
        def phase_d():
            _interleave([P(phase_d2, b) for b in range(NT - 1, 0, -1)], sa_items())
            phase_d2(0)
        region(phase_d)
    with scope("wait_wm1"):
        cp_di.wait()
        cp_wm1.wait()
    for d in cp_w2:
        d.start()

    def phase_e(q):
        r0 = 8 * q
        y = _radix16([(zbuf[b, r0:r0 + 8, :], zbuf[b, NR + r0:NR + r0 + 8, :]) for b in range(NT)], 1)
        for t in range(NT):
            ybuf[t + zero[0], q // 8, (q % 8) * 16:(q % 8) * 16 + 16, :] = _rows16(*y[t])

    def f_mxu(g, t):
        if g < 4:
            xbuf[t, 128 * g:128 * (g + 1), :] = _dot(_as_bf16(di[g]), ybuf[t, g])
        else:
            xbuf[t, 512:576, :] = _dot(_as_bf16(di[4, 0:32, :])[:, 0:80], ybuf[t, 4, 0:80, :])

    def phase_ef():
        _interleave([P(phase_e, q) for q in qs(4)], mod_items(1152, 6 * D))
        for g in range(4):
            _interleave([P(f_mxu, (g - 1) % 5, t) for t in range(NT)], [P(phase_e, q) for q in qs(g)])
        _interleave([P(f_mxu, 3, t) for t in range(NT)], [center_sb])

    def center_sb():
        sb = [tbl[3 * D + 8 * r:3 * D + 8 * r + 8, :] for r in range(D // 8)]
        sbm = _colsum(sb) * (1.0 / D)
        for r in range(D // 8):
            sab[8 * r:8 * r + 8, :] = sb[r] - sbm

    with scope("E"):
        region(phase_ef)

    def f_p1(t, _):
        accs = [None] * 3
        for j in range(8):
            v = [(xbuf[t, 128 * g + 8 * j:128 * g + 8 * j + 8, :],
                  xbuf[t, 128 * g + 64 + 8 * j:128 * g + 72 + 8 * j, :]) for g in range(4)]
            ys = _radix9_inv(xbuf[t, 512 + 8 * j:520 + 8 * j, :], v)
            for n9 in range(9):
                r = 8 * n9 + j
                xv = x_rows(t, r) + ys[n9] * tbl[2 * D + 8 * r:2 * D + 8 * r + 8, :]
                x1[t, 8 * r:8 * r + 8, :] = xv
                accs[n9 % 3] = xv if accs[n9 % 3] is None else accs[n9 % 3] + xv
        stat[0, t] = _tree(accs)

    def f_p2(t, _):
        mean = stat[0, t]
        a2 = [None] * 2
        az = [None] * 2
        for r in range(D // 8):
            xc = x1[t, 8 * r:8 * r + 8, :] - mean
            z = xc * tbl[4 * D + 8 * r:4 * D + 8 * r + 8, :]
            xbuf[t, 8 * r:8 * r + 8, :] = z
            k = r % 2
            a2[k] = xc * xc if a2[k] is None else a2[k] + xc * xc
            az[k] = z if az[k] is None else az[k] + z
        stat[1, t] = _tree(a2)
        stat[2, t] = _tree(az)

    def f_p3(t, _):
        rs = stat[1, t]
        mz = stat[2, t]
        a2 = [None] * 2
        for r in range(D // 8):
            dv = (xbuf[t, 8 * r:8 * r + 8, :] - mz) * rs + sab[8 * r:8 * r + 8, :]
            zbuf[t, 8 * r:8 * r + 8, :] = dv
            k = r % 2
            a2[k] = dv * dv if a2[k] is None else a2[k] + dv * dv
        stat[3, t] = _tree(a2)

    with scope("F1"):
        jax.lax.fori_loop(0, NT, f_p1, None, unroll=2)
        finish(0, lambda v: v)
    with scope("F2"):
        jax.lax.fori_loop(0, NT, f_p2, None, unroll=2)
        finish(1, rsq)
        finish(2, lambda v: v)
    with scope("F3"):
        jax.lax.fori_loop(0, NT, f_p3, None, unroll=2)
        finish(3, rsq)

    cp_b1.wait()
    cp_b2.wait()
    tbl[0:40, :] = jnp.concatenate([b1v[...].astype(f32), jnp.zeros((4, 128), f32)], axis=0)
    tbl[40:56, :] = b2v[...].astype(f32) * 2.0

    def bias(r):
        return jnp.broadcast_to(tbl[pl.ds(r, 1), :], (8, 128))

    def left_rows(block, dst, slot, r0):
        ops = [_sa2([[block(r, c, r0 + 8 * h) for c in range(4)] for r in range(4)]) for h in range(2)]
        out = [_rows16(ops[0][j], ops[1][j]) for j in range(49)]
        for j in range(49):
            dst[j, slot, pl.ds(r0, 16), :] = out[j]
        return out

    def f_p4(k, _):
        rs = [stat[3, 4 * k + c] for c in range(4)]
        for r0 in range(0, H, 16):
            left_rows(lambda r, c, row: zbuf[4 * k + c, r * H + row:r * H + row + 8, :] * rs[c], aop, k, r0)

    with scope("F4"):
        jax.lax.fori_loop(0, NT // 4, f_p4, None)

    def wait_w(src, dst, sems, i):
        view = dst.at[pl.ds(4 * i, 4)]
        pltpu.make_async_copy(view, view, sems.at[i]).wait()

    def hidden_rows(i, r0):
        return left_rows(lambda r, c, row: _gelu2(xbuf[4 * r + c, pl.ds(row, 8), :] + bias(4 * i + c)), gop, i, r0)

    def mlp1_chunk(i):
        prev = jnp.where(i == 0, NF - 1, i - 1)
        first, step = opt.get("h0", 1), opt.get("h1", 2)

        def hook(n):
            if n >= first and (n - first) % step == 0 and (n - first) // step < H // 16:
                r0 = 16 * ((n - first) // step)
                aop[49 + zero[0], 0, 0:16, :] = hidden_rows(prev, r0)[0]

        m = _strassen2(
            lambda j: jnp.concatenate([aop[j, k] for k in range(4)], axis=1),
            lambda o, r, c: jnp.concatenate(
                [w1v[4 * i + c + zero[opt.get('zz1', range(7))[o]], 128 * (4 * k + r):128 * (4 * k + r + 1), :].astype(f32) for k in range(4)], axis=0),
            hook, opt.get("oo1", (1, 5, 2, 4, 0, 3, 6)), opt.get("io1", _ORDER))
        u = _sc2(m)
        for r in range(4):
            for c in range(4):
                xbuf[4 * r + c, 0:H, :] = u[r][c]

    u1 = opt.get("u1", 1)

    def mlp1_step(n, _):
        for k in range(u1):
            wait_w(w1_h, w1v, w1sem, u1 * n + k)
        for k in range(u1):
            mlp1_chunk(u1 * n + k)

    with scope("mlp1"):
        jax.lax.fori_loop(0, NF // u1, mlp1_step, None)

    def mlp2(i, lhs):
        m = _strassen2(lhs, lambda o, r, c: jnp.concatenate(
            [w2v[4 * i + c + zero[opt.get('zz2', range(7))[o]], 128 * (4 * k + r):128 * (4 * k + r + 1), :].astype(f32) for k in range(NF)], axis=0),
            None, opt.get("oo2", _ORDER), opt.get("io2", _ORDER))
        y = _sc2(m)
        for ro, co in ((1, 0), (0, 0), (0, 1), (1, 1)):
            for c in (2 * co, 2 * co + 1):
                t = 4 * i + c
                bc = tbl[pl.ds(40 + t, 1), :]
                for r in (2 * ro, 2 * ro + 1):
                    rows = slice(r * H, (r + 1) * H)
                    gb = tbl[5 * D + r * H:5 * D + (r + 1) * H, :]
                    obuf[t, rows, :] = (x1[t, rows, :] + gb * (y[r][c] + bc)).astype(bf16)
                rows = pl.ds(2 * H * ro, 2 * H)
                cols = pl.ds(pl.multiple_of(t * 128, 128), 128)
                pltpu.make_async_copy(obuf.at[t, rows], out_h.at[rows, cols], osem.at[i]).start()

    def mlp2_step(i, _):
        wait_w(w2_h, w2v, w2sem, i)
        mlp2(i, lambda j: jnp.concatenate([gop[j, k] for k in range(NF)], axis=1))

    with scope("post"):
        jax.lax.fori_loop(0, H // 16, lambda n, _: hidden_rows(NF - 1, pl.multiple_of(16 * n, 16)) and None, None)
    with scope("mlp2"):
        jax.lax.fori_loop(0, NS, mlp2_step, None)
    for i in range(NS):
        view = out_h.at[:, pl.ds(SC * i, SC)]
        pltpu.make_async_copy(view, view, osem.at[i]).wait()


@jax.jit
def pallas_adaLN_cond__spectral_gfnet__mixer_token_mlp__prompt_kernel(
    A_x: jax.Array,
    A_w_r: jax.Array,
    A_w_i: jax.Array,
    B_x: jax.Array,
    B_w1: jax.Array,
    B_b1: jax.Array,
    B_w2: jax.Array,
    B_b2: jax.Array,
    c: jax.Array,
    w_mod: jax.Array,
):
    del B_x
    any_spec = pl.BlockSpec(memory_space=pl.ANY)
    scratch = [
        pltpu.VMEM((NT // 2, D, 256), bf16),
        pltpu.VMEM((NT, D // 2, 128), u32),
        pltpu.VMEM((289, S), bf16),
        pltpu.VMEM((289, S), bf16),
        pltpu.VMEM((2, NT, 152, 128), u32),
        pltpu.VMEM((F // 128, S, 128), bf16),
        pltpu.VMEM((NT, F, 128), bf16),
        pltpu.VMEM((F // 128, 128), bf16),
        pltpu.VMEM((S // 128, 128), bf16),
        pltpu.VMEM((1, D), bf16),
        pltpu.VMEM((D, 6 * D), bf16),
        pltpu.VMEM((5, 64, 128), u32),
        pltpu.VMEM((5, 64, 128), u32),
        pltpu.VMEM((NT, 2, 128, 128), bf16),
        pltpu.VMEM((NT, 2, 128, 128), bf16),
        pltpu.VMEM((6 * D, 128), f32),
        pltpu.VMEM((NT + 1, 5, 128, 128), bf16),
        pltpu.VMEM((NT, 2 * NR, 128), f32),
        pltpu.VMEM((NT, 3, NR, 128), bf16),
        pltpu.VMEM((2 * NR, 128), f32),
        pltpu.VMEM((NT, 8, 128), f32),
        pltpu.VMEM((4, NT, 8, 128), f32),
        pltpu.VMEM((NT, 2 * NR, 128), f32),
        pltpu.VMEM((NT, D, 128), f32),
        pltpu.VMEM((50, 4, H, 128), bf16),
        pltpu.VMEM((49, NF, H, 128), bf16),
        pltpu.VMEM((NT, D, 128), bf16),
        pltpu.SMEM((8,), jnp.int32),
        pltpu.SemaphoreType.DMA((24,)),
        pltpu.SemaphoreType.DMA((NF,)),
        pltpu.SemaphoreType.DMA((NS,)),
        pltpu.SemaphoreType.DMA((NS,)),
    ]
    outT = pl.pallas_call(
        functools.partial(_kernel, scopes=False, opt={}),
        out_shape=jax.ShapeDtypeStruct((D, S), bf16),
        in_specs=[any_spec] * 13,
        out_specs=any_spec,
        scratch_shapes=scratch,
        compiler_params=pltpu.CompilerParams(vmem_limit_bytes=120 * 1024 * 1024),
        name="adaln_gfnet_mixer",
    )(np.array([1, 0, 0, 0, 0, 0, 0, 0], np.int32), A_x[0].T, A_w_r.T, A_w_i.T, B_w1, B_b1.reshape(F // 128, 128), B_w2,
      B_b2.reshape(S // 128, 128), c, w_mod, _DFWD, _DINV, _SMAT)
    return outT.T[None]
```

```python
import functools

import jax
import jax.numpy as jnp
import numpy as np
import jax.experimental.pallas as pl
import jax.experimental.pallas.tpu as pltpu

S, D, F = 2048, 576, 4608
DF = D // 2 + 1
NT = S // 128
NP = 19
NR = NP * 16
H = D // 4
NF = F // 512
NS = S // 512
WSPLIT = (0, 96, 192, DF)
EPS = 1e-5
f32, bf16, u32 = jnp.float32, jnp.bfloat16, jnp.uint32

_TH = 2 * np.pi / 9
C1, C2, C4 = float(np.cos(_TH)), float(np.cos(2 * _TH)), float(np.cos(4 * _TH))
S1, S3, S4 = float(np.sin(_TH)), float(np.sin(3 * _TH)), float(np.sin(4 * _TH))

_SETS = [[g, g + 9, 9 - g, 18 - g] for g in range(1, 5)] + [[0, 9, 288]]
_FLAT = [c for grp in _SETS for c in grp]


def _row_pairs(m):
    bits = m.astype(bf16).view(np.uint16).astype(np.uint32)
    return bits[..., 0::2, :] | (bits[..., 1::2, :] << 16)


def _d_mats():
    d2 = np.arange(64)
    fwd = np.zeros((5, 128, 128))
    inv = np.zeros((5, 128, 128))
    col = 16 * (d2 // 8) + d2 % 8
    for g, grp in enumerate(_SETS):
        res = (g + 1) % 5
        scale = (0.0, S1, S1, S3, S1)[res]
        for cc, c0 in enumerate(grp):
            for m in range(1 if c0 == 288 else 16):
                kx = c0 + 18 * m
                ph = 2 * np.pi * ((kx * d2) % D) / D
                c, s = np.cos(ph), np.sin(ph)
                if kx % 288 == 0:
                    s = np.zeros_like(s)
                sg = (1.0 if kx % 9 == res else -1.0) * scale
                row = 32 * cc + 16 * (m // 8) + m % 8
                fwd[g, row, col] = c
                fwd[g, row + 8, col] = -s
                fwd[g, row, col + 8] = -sg * s
                fwd[g, row + 8, col + 8] = -sg * c
                w = (1.0 if kx % 288 == 0 else 2.0) / (S * D)
                inv[g, d2, row] = w * c
                inv[g, d2, row + 8] = -w * s
                inv[g, 64 + d2, row] = sg * w * s
                inv[g, 64 + d2, row + 8] = sg * w * c
    return _row_pairs(fwd), _row_pairs(inv)


def _s_mats():
    m = np.zeros((NT, 2, 128, 128))
    lane = np.arange(128)
    for b in range(NT):
        a = (lane - b) % 16
        k = 128 * a + (lane - a) % 128
        ph = 2 * np.pi * ((lane[:, None] * k[None, :]) % S) / S
        m[b] = np.cos(ph), -np.sin(ph)
    return m.astype(bf16)


_DFWD, _DINV = _d_mats()
_SMAT = _s_mats()
_SCALARS = np.array([1, 0, 0, 0, 0, 0, 0, 0], np.int32)


def _as_bf16(x):
    return pltpu.bitcast(x, bf16)


def _dot(a, b):
    return jnp.dot(a, b, preferred_element_type=f32)


def _dot_t(a, b):
    return jax.lax.dot_general(a, b, (((1,), (1,)), ((), ())), preferred_element_type=f32)


def _rows16(a, b):
    return jnp.concatenate([a, b], axis=0).astype(bf16)


def _half(x, i):
    return pltpu.bitcast(x & jnp.uint32(0xFFFF0000) if i else x << 16, f32)


def _radix9_fwd(a):
    p = [None] + [a[n] + a[9 - n] for n in range(1, 5)]
    m = [None] + [a[n] - a[9 - n] for n in range(1, 5)]
    t = p[1] + p[2] + p[4]
    u = a[0] + p[3]
    b = a[0] - 0.5 * p[3]
    e1 = p[1] - p[4]
    e2 = p[2] - p[4]
    r1 = C1 * e1 + C2 * e2
    r2 = C2 * e1 + C4 * e2
    f1 = m[1] + m[2]
    f2 = m[2] + m[4]
    f3 = m[1] - m[4]
    q1 = f1 + (S4 / S1) * f2
    q2 = f3 + (S4 / S1) * f1
    n3 = (S3 / S1) * m[3]
    return u + t, [(b + r1, q1 + n3), (b + r2, q2 - n3), (u - 0.5 * t, m[1] - m[2] + m[4]),
                   (b - (r1 + r2), (q2 - q1) + n3)]


def _radix9_inv(v0, v):
    (x1, i1), (x2, i2), (x3, i3), (x4, i4) = v
    t = x1 + x2 + x4
    u = v0 + x3
    b = v0 - 0.5 * x3
    e1 = x1 - x4
    e2 = x2 - x4
    r1 = C1 * e1 + C2 * e2
    r2 = C2 * e1 + C4 * e2
    a1, a2, a3, a4 = b + r1, b + r2, u - 0.5 * t, b - (r1 + r2)
    f1 = i1 + i2
    f2 = i2 + i4
    f3 = i1 - i4
    q1 = f1 + (S4 / S1) * f2
    q2 = f3 + (S4 / S1) * f1
    b1, b2, b4 = q1 + i3, q2 - i3, (q2 - q1) + i3
    b3 = (S3 / S1) * (i1 - i2 + i4)
    return [u + t, a1 - b1, a2 - b2, a3 - b3, a4 - b4, a4 + b4, a3 + b3, a2 + b2, a1 + b1]


def _bfly4(a, b, c, d, sgn, c_rot=False):
    if c_rot:
        minus, plus = (a[0] + c[1], a[1] - c[0]), (a[0] - c[1], a[1] + c[0])
        t0, t1 = (minus, plus) if sgn < 0 else (plus, minus)
    else:
        t0 = (a[0] + c[0], a[1] + c[1])
        t1 = (a[0] - c[0], a[1] - c[1])
    t2 = (b[0] + d[0], b[1] + d[1])
    t3 = (b[0] - d[0], b[1] - d[1])
    x0 = (t0[0] + t2[0], t0[1] + t2[1])
    x2 = (t0[0] - t2[0], t0[1] - t2[1])
    xm = (t1[0] + t3[1], t1[1] - t3[0])
    xp = (t1[0] - t3[1], t1[1] + t3[0])
    return [x0, xm, x2, xp] if sgn < 0 else [x0, xp, x2, xm]


def _tw16(z, e, sgn):
    c = float(np.cos(2 * np.pi * e / 16))
    s = float(sgn * np.sin(2 * np.pi * e / 16))
    x, y = z
    if e % 2 == 0:
        if (c > 0) == (s > 0):
            return ((x - y) * c, (x + y) * c)
        return ((x + y) * c, (y - x) * c)
    return (x * c - y * s, x * s + y * c)


def _radix16(x, sgn):
    u = [_bfly4(x[n2], x[4 + n2], x[8 + n2], x[12 + n2], sgn) for n2 in range(4)]
    out = [None] * 16
    for k1 in range(4):
        v = [u[n2][k1] if k1 * n2 % 4 == 0 else _tw16(u[n2][k1], k1 * n2, sgn) for n2 in range(4)]
        for k2, y in enumerate(_bfly4(*v, sgn, c_rot=(k1 == 2))):
            out[k1 + 4 * k2] = y
    return out


def _sa(a11, a12, a21, a22):
    return [a11 + a22, a21 + a22, a11, a22, a11 + a12, a21 - a11, a12 - a22]


def _sb(b11, b12, b21, b22):
    return [b11 + b22, b11, b12 - b22, b21 - b11, b22, b11 + b12, b21 + b22]


def _sc(m):
    m1, m2, m3, m4, m5, m6, m7 = m
    return [m4 + m7 - m5 + m1, m5 + m3, m2 + m4, m1 - m2 + m3 + m6]


def _sa2(blk):
    lvl = [_sa(blk[ri][ci], blk[ri][2 + ci], blk[2 + ri][ci], blk[2 + ri][2 + ci])
           for ri in range(2) for ci in range(2)]
    return [x for o in range(7) for x in _sa(*[q[o] for q in lvl])]


def _sc2(m):
    p = [_sc(m[7 * o:7 * o + 7]) for o in range(7)]
    out = [[None] * 4 for _ in range(4)]
    for ii in range(4):
        for oi, v in enumerate(_sc([p[o][ii] for o in range(7)])):
            out[2 * (oi // 2) + ii // 2][2 * (oi % 2) + ii % 2] = v
    return out


_SB_TERMS = (((1, 0, 0), (1, 1, 1)), ((1, 0, 0),), ((1, 0, 1), (-1, 1, 1)), ((1, 1, 0), (-1, 0, 0)),
             ((1, 1, 1),), ((1, 0, 0), (1, 0, 1)), ((1, 1, 0), (1, 1, 1)))
_ORDER = (1, 3, 6, 4, 0, 2, 5)


def _strassen2(lhs, raw, outer, before=None):
    m = [None] * 49
    for n, o in enumerate(outer):
        quad = []
        for ri in range(2):
            for ci in range(2):
                acc = None
                for sg, ro, co in _SB_TERMS[o]:
                    v = raw(o, 2 * ro + ri, 2 * co + ci)
                    acc = v if acc is None else (acc + v if sg > 0 else acc - v)
                quad.append(acc)
        ops = _sb(*quad)
        for k, j in enumerate(_ORDER):
            if before is not None:
                before(7 * n + k)
            rhs = ops[j].astype(bf16)
            m[7 * o + j] = _dot(lhs(7 * o + j), rhs)
    return m


def _gelu2(u):
    k0 = 0.7978845608028654
    z = u * (k0 + (k0 * 0.044715) * (u * u))
    return u * jnp.tanh(z) + u


class _Sum:
    def __init__(self, chains):
        self.accs = [None] * chains

    def add(self, k, v):
        k %= len(self.accs)
        self.accs[k] = v if self.accs[k] is None else self.accs[k] + v

    def total(self):
        return functools.reduce(lambda a, b: a + b, self.accs)


def _interleave(*lists):
    items = [((k + 0.5) / len(lst), ci, k, fn) for ci, lst in enumerate(lists) for k, fn in enumerate(lst)]
    for item in sorted(items, key=lambda x: x[:3]):
        item[3]()


def _kernel(z_h, xT_h, wr_h, wi_h, w1_h, b1_h, w2_h, b2_h, c_h, wm_h, df_h, di_h, sm_h, out_h,
            xw, xT, wraw_r, wraw_i, wp, w1v, w2v, b1v, b2v, cv, wm, df, di, sm, sm3, tbl,
            ybuf, ebuf, xbuf, cbuf, sab, mnb, stat, zbuf, x1, aop, gop, obuf, zsm,
            sem, w1sem, w2sem, osem):
    P = functools.partial
    used = []

    def cp(src, dst):
        used.append(pltpu.make_async_copy(src, dst, sem.at[len(used)]))
        return used[-1]

    cp_c = cp(c_h, cv)
    cp_wm0 = cp(wm_h.at[:, 512:1152], wm.at[:, 512:1152])
    xsem = len(used)
    for i in range(NT // 2):
        cp(xT_h.at[:, i * 256:(i + 1) * 256], xw.at[i])
    cp_z = cp(z_h, zsm)
    cp_df = cp(df_h, df)
    cp_sm = cp(sm_h, sm)
    cp_w = [[cp(src.at[lo:hi], dst.at[lo:hi]) for src, dst in ((wr_h, wraw_r), (wi_h, wraw_i))]
            for lo, hi in zip(WSPLIT[:-1], WSPLIT[1:])]
    cp_wms = cp(wm_h.at[:, 0:512], wm.at[:, 0:512])
    cp_di = cp(di_h, di)
    cp_wm1 = cp(wm_h.at[:, 1152:6 * D], wm.at[:, 1152:6 * D])
    cp_b1 = cp(b1_h, b1v)
    cp_b2 = cp(b2_h, b2v)
    for d in used:
        d.start()

    def start_strips(src, dst, sems):
        for j in range(dst.shape[0]):
            pltpu.make_async_copy(src.at[:, j * 128:(j + 1) * 128], dst.at[j], sems.at[j // 4]).start()

    def wait_strips(dst, sems, i):
        view = dst.at[pl.ds(4 * i, 4)]
        pltpu.make_async_copy(view, view, sems.at[i]).wait()

    def mean_of(v):
        return jnp.sum(v, axis=0, keepdims=True) * (1.0 / D)

    def rsq(v):
        return jax.lax.rsqrt(v + EPS)

    def finish(k, fn):
        for t in range(NT):
            stat[k, t] = jnp.broadcast_to(fn(mean_of(stat[k, t])), (8, 128))

    cp_c.wait()
    cc = cv[...].astype(f32)
    silu = jnp.broadcast_to(cc * jax.nn.sigmoid(cc), (16, D)).astype(bf16)

    def mod_items(lo, hi):
        box = []

        def tile(j):
            r0 = lo + j * 128
            col = r0 + jax.lax.broadcasted_iota(jnp.int32, (1, 128), 1)
            is_scale = ((col >= D) & (col < 2 * D)) | ((col >= 4 * D) & (col < 5 * D))
            row = box[0][0:1, j * 128:(j + 1) * 128]
            row = row * jnp.where(col >= 5 * D, 0.5, 1.0) + jnp.where(is_scale, 1.0, 0.0)
            tbl[r0:r0 + 128, :] = jnp.broadcast_to(row, (128, 128)).T

        return [lambda: box.append(_dot(silu, wm[:, lo:hi]))] + [P(tile, j) for j in range((hi - lo) // 128)]

    def mod_rows(k, r):
        return tbl[k * D + 8 * r:k * D + 8 * r + 8, :]

    cp_wm0.wait()
    _interleave(mod_items(512, 1152))

    def x_rows(t, r):
        v = _as_bf16(xT[t, 8 * (r // 2):8 * (r // 2) + 8, :]).astype(f32)
        return v[8 * (r % 2):8 * (r % 2) + 8]

    def radix9_store(t, load):
        for j in range(8):
            y0, ys = _radix9_fwd([load(8 * n + j) for n in range(9)])
            ybuf[t, 4, 8 * j:8 * j + 8, :] = pltpu.bitcast(_rows16(y0, jnp.zeros_like(y0)), u32)
            for g in range(4):
                ybuf[t, g, 8 * j:8 * j + 8, :] = pltpu.bitcast(_rows16(*ys[g]), u32)

    def token_mean(tp, k):
        acc = _Sum(3)
        for r in range(D // 16):
            v = xw[tp, 16 * r:16 * r + 16, 128 * k:128 * k + 128]
            xT[2 * tp + k, 8 * r:8 * r + 8, :] = pltpu.bitcast(v, u32)
            v = v.astype(f32)
            acc.add(2 * r, v[0:8])
            acc.add(2 * r + 1, v[8:16])
        mnb[2 * tp + k] = jnp.broadcast_to(mean_of(acc.total()), (8, 128))

    def first_butterfly(t):
        mean = mnb[t]
        acc = _Sum(3)

        def load(r):
            xc = x_rows(t, r) - mean
            acc.add(r // 8, xc * xc)
            return xc * mod_rows(1, r)

        radix9_store(t, load)
        stat[0, t] = acc.total()

    def tile_pair(tp, _):
        pltpu.make_async_copy(xT_h.at[:, 0:256], xw.at[tp], sem.at[xsem + tp]).wait()
        token_mean(tp, 0)
        token_mean(tp, 1)
        first_butterfly(2 * tp)
        first_butterfly(2 * tp + 1)

    jax.lax.fori_loop(0, NT // 2, tile_pair, None)
    finish(0, rsq)
    start_strips(w1_h, w1v, w1sem)

    cp_z.wait()
    one = jnp.minimum(zsm[0], 1)
    zero = [zsm[1 + k] for k in range(7)]

    def phase(fn):
        jax.lax.fori_loop(0, one, lambda i, _: fn(), None)

    def forward_d():
        for p, c0 in enumerate(_FLAT):
            g, k = divmod(p, 4)
            halves = 1 if c0 == 288 else 2
            lhs = _as_bf16(df[g, 16 * k:16 * k + 8 * halves, :])
            xs = [_dot(lhs, _as_bf16(ybuf[t + zero[k], g])) for t in range(NT)]
            y = [_radix16([(xs[t][16 * h:16 * h + 8] * stat[0, t], xs[t][16 * h + 8:16 * h + 16] * stat[0, t])
                           for t in range(NT)], -1) for h in range(halves)]
            for b in range(NT):
                (lr, li), (hr, hi) = y[0][b], y[-1][b]
                cbuf[b, 0, 16 * p:16 * p + 16, :] = _rows16(lr + li, hr + hi)
                cbuf[b, 1, 16 * p:16 * p + 16, :] = _rows16(lr, hr)
                cbuf[b, 2, 16 * p:16 * p + 16, :] = _rows16(li, hi)

    cp_df.wait()
    phase(forward_d)

    lane = jax.lax.broadcasted_iota(jnp.int32, (8, 128), 1)
    masks = [(lane & (1 << b)) != 0 for b in range(4)]

    def filter_rows(plane, raw, r):
        if r < 18:
            vals = [pltpu.bitcast(raw[16 * r:16 * r + 16, a * 128:(a + 1) * 128], u32) for a in range(NT)]
        else:
            last = jnp.broadcast_to(raw[288:289, :].astype(f32), (8, S))
            vals = [pltpu.bitcast(last[:, a * 128:(a + 1) * 128], u32) for a in range(NT)]
        vals = [pltpu.roll(v, a, 1) if a else v for a, v in enumerate(vals)]
        vals = [vals[(-b) % NT] for b in range(NT)]
        for b in range(4):
            vals = [jnp.where(masks[b], vals[(i - (1 << b)) % NT], vals[i]) for i in range(NT)]
        for b in range(NT):
            wp[plane, b, 8 * r:8 * r + 8, :] = vals[b]

    def filter_set(plane, b, c0, h):
        if c0 == 288:
            return pltpu.bitcast(wp[plane, b, 144:152, :], f32)
        return _half(wp[plane, b, pl.ds(c0 // 2 + 72 * h, 8, stride=9), :], c0 % 2)

    def forward_s(b):
        fr, fi = sm[b, 0], sm[b, 1]
        dif = (fi.astype(f32) - fr.astype(f32)).astype(bf16)
        tot = (fr.astype(f32) + fi.astype(f32)).astype(bf16)
        sm3[b, 0] = dif
        sm3[b, 1] = tot
        k = [_dot(cbuf[b, p], m) for p, m in enumerate((fr, dif, tot))]
        xbuf[b, 0:NR, :] = k[0] - k[2]
        xbuf[b, NR:2 * NR, :] = k[0] + k[1]

    cp_sm.wait()
    for i, (lo, hi) in enumerate(((0, 8), (8, 13), (13, NT))):
        for d in cp_w[i]:
            d.wait()
        phase(P(_interleave, [P(forward_s, b) for b in range(lo, hi)],
                [P(filter_rows, plane, raw, r) for r in range(WSPLIT[i] // 16, -(-WSPLIT[i + 1] // 16))
                 for plane, raw in enumerate((wraw_r, wraw_i))]))

    def shift_spectrum():
        for g, grp in enumerate(_SETS):
            r = _dot(_as_bf16(df[g, 0:64 if g < 4 else 40, :]), _as_bf16(ybuf[NT, g])) * float(S)
            for k, c0 in enumerate(grp):
                for h in range(1 if c0 == 288 else 2):
                    for ri in range(2):
                        src, dst = 32 * k + 16 * h + 8 * ri, ri * NR + 16 * (4 * g + k) + 8 * h
                        sab[dst:dst + 8, :] = r[src:src + 8]

    def filter_inverse_s(b):
        zs = [[], [], []]
        for p, c0 in enumerate(_FLAT):
            z = []
            for h in range(1 if c0 == 288 else 2):
                r0 = 16 * p + 8 * h
                xr, xi = xbuf[b, r0:r0 + 8, :], xbuf[b, NR + r0:NR + r0 + 8, :]
                if b == 0:
                    xr = xr + jnp.where(lane == 0, sab[r0:r0 + 8, :], 0.0)
                    xi = xi + jnp.where(lane == 0, sab[NR + r0:NR + r0 + 8, :], 0.0)
                wr, wi = filter_set(0, b, c0, h), filter_set(1, b, c0, h)
                zr, zi = xr * wr - xi * wi, xr * wi + xi * wr
                z.append((zr + zi, zr, zi))
            for k in range(3):
                zs[k] += [z[0][k], z[-1][k]]
        k = [_dot_t(jnp.concatenate(z, axis=0).astype(bf16), m)
             for z, m in zip(zs, (sm[b, 0], sm3[b, 1], sm3[b, 0]))]
        zbuf[b, 0:NR, :] = k[0] + k[2]
        zbuf[b, NR:2 * NR, :] = k[0] - k[1]

    def inverse_s():
        _interleave([P(filter_inverse_s, b) for b in range(NT - 1, 0, -1)],
                    mod_items(0, 512) + [P(radix9_store, NT, P(mod_rows, 0)), shift_spectrum])
        filter_inverse_s(0)

    cp_wms.wait()
    phase(inverse_s)
    start_strips(w2_h, w2v, w2sem)

    def second_butterfly(q):
        y = _radix16([(zbuf[b, 8 * q:8 * q + 8, :], zbuf[b, NR + 8 * q:NR + 8 * q + 8, :]) for b in range(NT)], 1)
        for t in range(NT):
            ebuf[t + zero[0], q // 8, (q % 8) * 16:(q % 8) * 16 + 16, :] = _rows16(*y[t])

    def inverse_d(g, t):
        if g < 4:
            xbuf[t, 128 * g:128 * (g + 1), :] = _dot(_as_bf16(di[g]), ebuf[t, g])
        else:
            xbuf[t, 512:576, :] = _dot(_as_bf16(di[4, 0:32, :])[:, 0:80], ebuf[t, 4, 0:80, :])

    def center_shift():
        acc = _Sum(4)
        for r in range(D // 8):
            acc.add(r, mod_rows(3, r))
        mean = mean_of(acc.total())
        for r in range(D // 8):
            sab[8 * r:8 * r + 8, :] = mod_rows(3, r) - mean

    early = 6

    def inverse_d_all():
        for g in range(4):
            _interleave([P(inverse_d, (g - 1) % 5, t) for t in range(NT)],
                        [P(second_butterfly, q) for q in range(max(8 * g, early), 8 * g + 8)],
                        *([mod_items(1152, 6 * D)] if g == 0 else []))
        _interleave([P(inverse_d, 3, t) for t in range(NT)], [center_shift])

    phase(P(_interleave, [P(second_butterfly, q) for q in [*range(32, 2 * NP - 1), *range(early)]]))
    cp_di.wait()
    cp_wm1.wait()
    phase(inverse_d_all)

    def residual(t, _):
        acc = _Sum(3)
        for j in range(8):
            v = [(xbuf[t, 128 * g + 8 * j:128 * g + 8 * j + 8, :],
                  xbuf[t, 128 * g + 64 + 8 * j:128 * g + 72 + 8 * j, :]) for g in range(4)]
            for n, y in enumerate(_radix9_inv(xbuf[t, 512 + 8 * j:520 + 8 * j, :], v)):
                r = 8 * n + j
                xv = x_rows(t, r) + y * mod_rows(2, r)
                x1[t, 8 * r:8 * r + 8, :] = xv
                acc.add(n, xv)
        stat[0, t] = acc.total()

    def center_scale(t, _):
        mean = stat[0, t]
        sq, tot = _Sum(2), _Sum(2)
        for r in range(D // 8):
            xc = x1[t, 8 * r:8 * r + 8, :] - mean
            z = xc * mod_rows(4, r)
            xbuf[t, 8 * r:8 * r + 8, :] = z
            sq.add(r, xc * xc)
            tot.add(r, z)
        stat[1, t] = sq.total()
        stat[2, t] = tot.total()

    def center_again(t, _):
        rs, mz = stat[1, t], stat[2, t]
        sq = _Sum(2)
        for r in range(D // 8):
            v = (xbuf[t, 8 * r:8 * r + 8, :] - mz) * rs + sab[8 * r:8 * r + 8, :]
            zbuf[t, 8 * r:8 * r + 8, :] = v
            sq.add(r, v * v)
        stat[3, t] = sq.total()

    jax.lax.fori_loop(0, NT, residual, None, unroll=2)
    finish(0, lambda v: v)
    jax.lax.fori_loop(0, NT, center_scale, None, unroll=2)
    finish(1, rsq)
    finish(2, lambda v: v)
    jax.lax.fori_loop(0, NT, center_again, None, unroll=2)
    finish(3, rsq)

    cp_b1.wait()
    cp_b2.wait()
    tbl[0:40, :] = jnp.concatenate([b1v[...].astype(f32), jnp.zeros((4, 128), f32)], axis=0)
    tbl[40:56, :] = b2v[...].astype(f32) * 2.0

    def left_rows(block, dst, slot, r0):
        ops = [_sa2([[block(r, c, r0 + 8 * h) for c in range(4)] for r in range(4)]) for h in range(2)]
        out = [_rows16(ops[0][j], ops[1][j]) for j in range(49)]
        for j in range(49):
            dst[j, slot, pl.ds(r0, 16), :] = out[j]
        return out

    def input_ops(k, _):
        rs = [stat[3, 4 * k + c] for c in range(4)]
        for r0 in range(0, H, 16):
            left_rows(lambda r, c, row: zbuf[4 * k + c, r * H + row:r * H + row + 8, :] * rs[c], aop, k, r0)

    jax.lax.fori_loop(0, NT // 4, input_ops, None)

    def hidden_ops(i, r0):
        def block(r, c, row):
            bias = jnp.broadcast_to(tbl[pl.ds(4 * i + c, 1), :], (8, 128))
            return _gelu2(xbuf[4 * r + c, pl.ds(row, 8), :] + bias)

        return left_rows(block, gop, i, r0)

    def weight_block(wv, i, tiles, o, r, c):
        return jnp.concatenate(
            [wv[4 * i + c + zero[o], 128 * (4 * k + r):128 * (4 * k + r + 1), :].astype(f32) for k in range(tiles)],
            axis=0)

    def first_matmul(i, _):
        wait_strips(w1v, w1sem, i)
        prev = jnp.where(i == 0, NF - 1, i - 1)

        def before(n):
            if n % 2 == 1 and n // 2 < H // 16:
                aop[49 + zero[0], 0, 0:16, :] = hidden_ops(prev, 16 * (n // 2))[0]

        u = _sc2(_strassen2(lambda j: jnp.concatenate([aop[j, k] for k in range(4)], axis=1),
                            P(weight_block, w1v, i, 4), (1, 5, 2, 4, 0, 3, 6), before))
        for r in range(4):
            for c in range(4):
                xbuf[4 * r + c, 0:H, :] = u[r][c]

    def last_hidden(n, _):
        hidden_ops(NF - 1, pl.multiple_of(16 * n, 16))

    jax.lax.fori_loop(0, NF, first_matmul, None)
    jax.lax.fori_loop(0, H // 16, last_hidden, None)

    def second_matmul(i, _):
        wait_strips(w2v, w2sem, i)
        y = _sc2(_strassen2(lambda j: jnp.concatenate([gop[j, k] for k in range(NF)], axis=1),
                            P(weight_block, w2v, i, NF), _ORDER))
        for ro, co in ((1, 0), (0, 0), (0, 1), (1, 1)):
            for c in (2 * co, 2 * co + 1):
                t = 4 * i + c
                bias = tbl[pl.ds(40 + t, 1), :]
                for r in (2 * ro, 2 * ro + 1):
                    rows = slice(r * H, (r + 1) * H)
                    gate = tbl[5 * D + r * H:5 * D + (r + 1) * H, :]
                    obuf[t, rows, :] = (x1[t, rows, :] + gate * (y[r][c] + bias)).astype(bf16)
                rows = pl.ds(2 * H * ro, 2 * H)
                cols = pl.ds(pl.multiple_of(t * 128, 128), 128)
                pltpu.make_async_copy(obuf.at[t, rows], out_h.at[rows, cols], osem.at[i]).start()

    jax.lax.fori_loop(0, NS, second_matmul, None)
    for i in range(NS):
        view = out_h.at[:, 512 * i:512 * (i + 1)]
        pltpu.make_async_copy(view, view, osem.at[i]).wait()


@jax.jit
def pallas_adaLN_cond__spectral_gfnet__mixer_token_mlp__prompt_kernel(
    A_x: jax.Array,
    A_w_r: jax.Array,
    A_w_i: jax.Array,
    B_x: jax.Array,
    B_w1: jax.Array,
    B_b1: jax.Array,
    B_w2: jax.Array,
    B_b2: jax.Array,
    c: jax.Array,
    w_mod: jax.Array,
):
    del B_x
    any_spec = pl.BlockSpec(memory_space=pl.ANY)
    scratch = [
        pltpu.VMEM((NT // 2, D, 256), bf16),
        pltpu.VMEM((NT, D // 2, 128), u32),
        pltpu.VMEM((DF, S), bf16),
        pltpu.VMEM((DF, S), bf16),
        pltpu.VMEM((2, NT, 152, 128), u32),
        pltpu.VMEM((F // 128, S, 128), bf16),
        pltpu.VMEM((NT, F, 128), bf16),
        pltpu.VMEM((F // 128, 128), bf16),
        pltpu.VMEM((S // 128, 128), bf16),
        pltpu.VMEM((1, D), bf16),
        pltpu.VMEM((D, 6 * D), bf16),
        pltpu.VMEM((5, 64, 128), u32),
        pltpu.VMEM((5, 64, 128), u32),
        pltpu.VMEM((NT, 2, 128, 128), bf16),
        pltpu.VMEM((NT, 2, 128, 128), bf16),
        pltpu.VMEM((6 * D, 128), f32),
        pltpu.VMEM((NT + 1, 5, 64, 128), u32),
        pltpu.VMEM((NT, 5, 128, 128), bf16),
        pltpu.VMEM((NT, 2 * NR, 128), f32),
        pltpu.VMEM((NT, 3, NR, 128), bf16),
        pltpu.VMEM((2 * NR, 128), f32),
        pltpu.VMEM((NT, 8, 128), f32),
        pltpu.VMEM((4, NT, 8, 128), f32),
        pltpu.VMEM((NT, 2 * NR, 128), f32),
        pltpu.VMEM((NT, D, 128), f32),
        pltpu.VMEM((50, 4, H, 128), bf16),
        pltpu.VMEM((49, NF, H, 128), bf16),
        pltpu.VMEM((NT, D, 128), bf16),
        pltpu.SMEM((8,), jnp.int32),
        pltpu.SemaphoreType.DMA((24,)),
        pltpu.SemaphoreType.DMA((NF,)),
        pltpu.SemaphoreType.DMA((NS,)),
        pltpu.SemaphoreType.DMA((NS,)),
    ]
    out = pl.pallas_call(
        _kernel,
        out_shape=jax.ShapeDtypeStruct((D, S), bf16),
        in_specs=[any_spec] * 13,
        out_specs=any_spec,
        scratch_shapes=scratch,
        compiler_params=pltpu.CompilerParams(vmem_limit_bytes=120 * 1024 * 1024),
        name="adaln_gfnet_mixer",
    )(_SCALARS, A_x[0].T, A_w_r.T, A_w_i.T, B_w1, B_b1.reshape(F // 128, 128), B_w2,
      B_b2.reshape(S // 128, 128), c, w_mod, _DFWD, _DINV, _SMAT)
    return out.T[None]
```
